```python
import jax
import jax.numpy as jnp

def _softmax(x, axis=-1):
    return jax.nn.softmax(x, axis=axis)
def _gelu(x):
    return jax.nn.gelu(x, approximate=True)
def _silu(x):
    return jax.nn.silu(x)
def _sigmoid(x):
    return jax.nn.sigmoid(x)
def _layernorm(x, axis=-1, eps=1e-5):
    m = jnp.mean(x, axis=axis, keepdims=True)
    v = jnp.var(x, axis=axis, keepdims=True)
    return (x - m) / jnp.sqrt(v + eps)
def _scatter_add(tgt, idx, src, axis=0):
    return tgt.at[idx].add(src)
def _segment_sum(src, seg, n):
    return jax.ops.segment_sum(src, seg, n)
class _Rng:
    def __init__(self, key):
        self._k = key
    def _next(self):
        self._k, sub = jax.random.split(self._k)
        return sub
    def normal(self, shape):
        return jax.random.normal(self._next(), shape, dtype=jnp.bfloat16)
    def randint(self, lo, hi, shape):
        return jax.random.randint(self._next(), shape, lo, hi, dtype=jnp.int32)
    def uniform(self, shape, lo=0.0, hi=1.0):
        return jax.random.uniform(self._next(), shape, jnp.bfloat16, lo, hi)
    def permutation(self, n):
        return jax.random.permutation(self._next(), n)


kernel_name = 'gated_mix__compressed_kv_cla__moe_arch_mod__prompt'

def setup_inputs():
    _rng = _Rng(jax.random.key(int.from_bytes(__import__("os").urandom(4), "little")))
    _w = (lambda a: (lambda t: t.astype(jnp.bfloat16) if jnp.issubdtype(t.dtype, jnp.floating) else t)(jnp.asarray(a)))
    def _A_setup():
        B, H, Sq, Sk, D, M = 1, 16, 2048, 2048, 256, 448
        Dc = 4 * D
        return {
            "x": _w((lambda *s: _rng.normal(s) * 0.05)(B, Sq, M)),
            "c_kv": _w((lambda *s: _rng.normal(s) * 0.05)(B, Sk, Dc)),
            "w_q": _w((lambda *s: _rng.normal(s) * 0.05)(M, H, D) * (M ** -0.5)),
            "w_uk": _w((lambda *s: _rng.normal(s) * 0.05)(Dc, H, D) * (Dc ** -0.5)),
            "w_uv": _w((lambda *s: _rng.normal(s) * 0.05)(Dc, H, D) * (Dc ** -0.5)),
            "w_o": _w((lambda *s: _rng.normal(s) * 0.05)(H, D, M) * ((H * D) ** -0.5)),
        }
    _A_in = _A_setup()

    def _B_setup():
        B, S, D, F, C = 1, 2048, 448, 1792, 2
        return {
            "x": _w((lambda *s: _rng.normal(s) * 0.05)(B, S, D)),
            "w_r": _w((lambda *s: _rng.normal(s) * 0.05)(D)),
            "w_gate": _w((lambda *s: _rng.normal(s) * 0.05)(D, F)),
            "w_up": _w((lambda *s: _rng.normal(s) * 0.05)(D, F)),
            "w_down": _w((lambda *s: _rng.normal(s) * 0.05)(F, D)),
        }
    _B_in = _B_setup()

    return {
        "A_x": _A_in["x"],
        "A_c_kv": _A_in["c_kv"],
        "A_w_q": _A_in["w_q"],
        "A_w_uk": _A_in["w_uk"],
        "A_w_uv": _A_in["w_uv"],
        "A_w_o": _A_in["w_o"],
        "B_x": _B_in["x"],
        "B_w_r": _B_in["w_r"],
        "B_w_gate": _B_in["w_gate"],
        "B_w_up": _B_in["w_up"],
        "B_w_down": _B_in["w_down"],
        "gate_w": _w((lambda *s: _rng.normal(s) * 0.05)(448)),
    }

def reference(A_x, A_c_kv, A_w_q, A_w_uk, A_w_uv, A_w_o, B_x, B_w_r, B_w_gate, B_w_up, B_w_down, gate_w):
    def _A_ref(x, c_kv, w_q, w_uk, w_uv, w_o):
        B, Sq, M = x.shape[0], x.shape[1], x.shape[2]
        Sk = c_kv.shape[1]
        H, D = w_q.shape[1], w_q.shape[2]
        q = jnp.einsum("bqm,mhd->bhqd", x, w_q)
        k = jnp.einsum("bkc,chd->bhkd", c_kv, w_uk)
        v = jnp.einsum("bkc,chd->bhkd", c_kv, w_uv)
        scores = jnp.einsum("bhqd,bhkd->bhqk", q, k) * (D ** -0.5)
        off = Sk - Sq
        qi = jnp.arange(Sq)[:, None]
        kj = jnp.arange(Sk)[None, :]
        cmask = kj <= (qi + off)
        scores = jnp.where(cmask[None, None], scores, -1e9)
        p = _softmax(scores, axis=-1)
        ctx = jnp.einsum("bhqk,bhkd->bhqd", p, v)
        return jnp.einsum("bhqd,hdm->bqm", ctx, w_o)

    def _B_ref(x, w_r, w_gate, w_up, w_down):
        B, S, D = x.shape
        C = 2
        r = x @ w_r
        idx = jnp.argsort(-r, axis=-1)[:, :C]
        idx_e = jnp.repeat(idx.reshape(B, C, 1), D, axis=2)
        x_sel = jnp.take_along_axis(x, idx_e, axis=1)
        g = _silu(x_sel @ w_gate)
        u = x_sel @ w_up
        y = (g * u) @ w_down
        r_sel = _sigmoid(jnp.take_along_axis(r, idx, axis=1))
        y = y * r_sel.reshape(B, C, 1)
        b_off = (jnp.arange(B) * S).reshape(B, 1)
        flat_idx = (idx + b_off).reshape(B * C)
        zero = (x * 0.0).reshape(B * S, D)
        upd = _scatter_add(zero, flat_idx, y.reshape(B * C, D), axis=0)
        return x + upd.reshape(B, S, D)

    x = A_x
    g = _sigmoid((x * gate_w).sum(-1, keepdims=True))
    a = _A_ref(x, A_c_kv, A_w_q, A_w_uk, A_w_uv, A_w_o)
    b = _B_ref(x, B_w_r, B_w_gate, B_w_up, B_w_down)
    return g * a + (1 - g) * b
```

```python
import math

import jax
import jax.numpy as jnp
from jax import lax
import jax.experimental.pallas as pl
import jax.experimental.pallas.tpu as pltpu

F32, BF16, U32, I32 = jnp.float32, jnp.bfloat16, jnp.uint32, jnp.int32
_NT = (((1,), (1,)), ((), ()))
_NEG = -1e30
_B = 256
_T = 128
_LAG = 2


def _mm(a, b):
    return jnp.dot(a, b, preferred_element_type=F32)


def _mm_nt(a, b):
    return lax.dot_general(a, b, _NT, preferred_element_type=F32)


def _sigmoid(x):
    return 1.0 / (1.0 + jnp.exp(-x))


def _make_kernel(S, M, C, H, D, FF):
    NB = S // _B
    q_scale = math.log2(math.e) * (D ** -0.5)

    def kernel(xT_ref, c_ref, wq_hbm, wk_hbm, wv_hbm, woT_ref, wr_ref, gw_ref,
               wg_hbm, wu_hbm, wdT_hbm, o_ref,
               wq_buf, wk_buf, wv_buf, wqT_s, wk_s, wvT_s, k_s, vT_s, acc, g_s, r_s,
               wg_s, wu_s, wdT_s, w_sem, f_sem):
        h = pl.program_id(0)

        def w_copies(p, slot):
            return [
                pltpu.make_async_copy(src.bitcast(U32).at[:, p, :], dst.at[slot], w_sem.at[slot, i])
                for i, (src, dst) in enumerate(((wq_hbm, wq_buf), (wk_hbm, wk_buf), (wv_hbm, wv_buf)))
            ]

        def f_copies():
            return [
                pltpu.make_async_copy(src, dst, f_sem.at[i])
                for i, (src, dst) in enumerate(((wg_hbm, wg_s), (wu_hbm, wu_s), (wdT_hbm, wdT_s)))
            ]

        def prep_weights(hh):
            slot = (hh // 2) % 2
            sh = ((1 - hh % 2) * 16).astype(U32)

            def unpack(buf):
                w = (buf[slot] << sh) & jnp.uint32(0xFFFF0000)
                return lax.bitcast_convert_type(w, F32)

            wqT_s[...] = unpack(wq_buf).T.astype(BF16)
            wk_s[...] = unpack(wk_buf).astype(BF16)
            wvT_s[...] = unpack(wv_buf).T.astype(BF16)

        @pl.when(h == 0)
        def _():
            for cp in w_copies(0, 0):
                cp.start()
            for cp in w_copies(1, 1):
                cp.start()
            for cp in f_copies():
                cp.start()
            row = lax.broadcasted_iota(I32, (16, M), 0)
            wr = wr_ref[...].astype(F32).reshape(1, M)
            gw = gw_ref[...].astype(F32).reshape(1, M)
            lhs = jnp.where(row == 0, wr, jnp.where(row == 1, gw, 0.0)).astype(BF16)
            rg = _mm(lhs, xT_ref[...])
            r_s[...] = rg[0:1, :].astype(BF16).astype(F32)
            g = _sigmoid(rg[1:2, :])
            g_s[...] = g
            acc[...] = (1.0 - g) * xT_ref[...].astype(F32)
            for cp in w_copies(0, 0):
                cp.wait()
            prep_weights(h)

        @pl.when(jnp.logical_and(h % 2 == 1, h + 1 < H))
        def _():
            for cp in w_copies((h + 1) // 2, ((h + 1) // 2) % 2):
                cp.wait()

        @pl.when(jnp.logical_and(jnp.logical_and(h % 2 == 0, h > 0), h + 2 < H))
        def _():
            for cp in w_copies(h // 2 + 1, (h // 2 + 1) % 2):
                cp.start()

        @pl.when(h == 1)
        def _():
            for cp in f_copies():
                cp.wait()
            r = r_s[...]
            lane = lax.broadcasted_iota(I32, (1, S), 1)
            idxs, cur = [], r
            for _ in range(2):
                mx = jnp.max(cur, axis=1, keepdims=True)
                ii = jnp.min(jnp.where(cur == mx, lane, S - 1))
                idxs.append(ii)
                cur = jnp.where(lane == ii, -jnp.inf, cur)
            row16 = lax.broadcasted_iota(I32, (16, _T), 0)
            lane16 = lax.broadcasted_iota(I32, (16, _T), 1)
            xs = None
            for n, ii in enumerate(idxs):
                t0 = pl.multiple_of((ii // _T) * _T, _T)
                oh = jnp.where(jnp.logical_and(row16 == n, lane16 == ii % _T), 1.0, 0.0).astype(BF16)
                xr = _mm_nt(oh, xT_ref[:, pl.ds(t0, _T)])
                xs = xr if xs is None else xs + xr
            xs = xs.astype(BF16)
            gt = _mm(xs, wg_s[...])
            up = _mm(xs, wu_s[...])
            hid = (gt * _sigmoid(gt) * up).astype(BF16)
            hid128 = jnp.concatenate([hid, jnp.zeros((_T - 16, FF), BF16)], axis=0)
            yT = _mm_nt(wdT_s[...], hid128)
            lane1 = lax.broadcasted_iota(I32, (1, _T), 1)
            for n, ii in enumerate(idxs):
                t0 = pl.multiple_of((ii // _T) * _T, _T)
                sc = _sigmoid(r_s[:, pl.ds(t0, _T)]) * (1.0 - g_s[:, pl.ds(t0, _T)])
                sc = jnp.where(lane1 == ii % _T, sc, 0.0)
                acc[:, pl.ds(t0, _T)] += yT[:, n:n + 1] * sc

        key = lax.broadcasted_iota(I32, (_T, _T), 0)
        qry = lax.broadcasted_iota(I32, (_T, _T), 1)
        tri = key <= qry
        qT = {}

        def pQ(j, t):
            c0 = j * _B + t * _T
            qT[(j, t)] = (_mm(wqT_s[...], xT_ref[:, c0:c0 + _T]) * q_scale).astype(BF16)

        def pK(j, t):
            k_s[j * _B:(j + 1) * _B, t * _T:(t + 1) * _T] = _mm(
                c_ref[j * _B:(j + 1) * _B, :], wk_s[:, t * _T:(t + 1) * _T]).astype(BF16)

        def pV(j, t):
            c0 = j * _B + t * _T
            vT_s[:, c0:c0 + _T] = _mm_nt(wvT_s[...], c_ref[c0:c0 + _T, :]).astype(BF16)

        done = set()

        def piece(name, j, t):
            if j < NB and (name, j, t) not in done:
                done.add((name, j, t))
                {'Q': pQ, 'K': pK, 'V': pV}[name](j, t)

        items = [(j, c) for j in range(NB) for c in range(j + 1)]
        state, scores = {}, {}

        def QK(j, c):
            for t in range(2):
                piece('Q', j, t)
            for t in range(2):
                piece('K', c, t)
            k0 = c * _B
            q = jnp.concatenate([qT[(j, 0)], qT[(j, 1)]], axis=1)
            if c < j:
                s = _mm(k_s[k0:k0 + _B, :], q)
                scores[(j, c)] = (s[:, :_T], s[:, _T:])
            else:
                s = _mm(k_s[k0:k0 + _T, :], q)
                s2 = _mm(k_s[k0 + _T:k0 + _B, :], qT[(j, 1)])
                scores[(j, c)] = (
                    jnp.where(tri, s[:, :_T], _NEG),
                    jnp.concatenate([s[:, _T:], jnp.where(tri, s2, _NEG)], axis=0))

        def PV(j, c):
            for t in range(2):
                piece('V', c, t)
            k0 = c * _B
            ss = scores.pop((j, c))
            first = j not in state
            ps, ms, al, ls = [], [], [], []
            for t in range(2):
                m = jnp.max(ss[t], axis=0, keepdims=True)
                if not first:
                    m = jnp.maximum(state[j][0][t], m)
                    al.append(jnp.exp2(state[j][0][t] - m))
                p = jnp.exp2(ss[t] - m)
                lc = jnp.sum(p, axis=0, keepdims=True)
                ls.append(lc if first else state[j][1][t] * al[t] + lc)
                ms.append(m)
                ps.append(p.astype(BF16))
            if c < j:
                o = _mm(vT_s[:, k0:k0 + _B], jnp.concatenate(ps, axis=1))
                os_ = [o[:, :_T], o[:, _T:]]
            else:
                o = _mm(vT_s[:, k0:k0 + _T], jnp.concatenate([ps[0], ps[1][:_T]], axis=1))
                o2 = _mm(vT_s[:, k0 + _T:k0 + _B], ps[1][_T:])
                os_ = [o[:, :_T], o[:, _T:] + o2]
            if not first:
                os_ = [state[j][2][t] * al[t] + os_[t] for t in range(2)]
            state[j] = (ms, ls, os_)

        def WO(j):
            _, ls, os_ = state.pop(j)
            ctxT = jnp.concatenate(
                [(os_[t] * (g_s[:, j * _B + t * _T:j * _B + (t + 1) * _T] / ls[t])).astype(BF16)
                 for t in range(2)], axis=1)
            acc[:, j * _B:(j + 1) * _B] += _mm(woT_ref[0], ctxT)

        pend = []
        n_it = len(items)
        for i in range(n_it + _LAG):
            if i < n_it:
                j, c = items[i]
                QK(j, c)
                pcs = [('V', j, 0), ('V', j, 1), ('Q', j + 1, 0), ('Q', j + 1, 1),
                       ('K', j + 1, 0), ('K', j + 1, 1)]
                lo, hi = len(pcs) * c // (j + 1), len(pcs) * (c + 1) // (j + 1)
                for pc in pcs[lo:hi]:
                    piece(*pc)
            for jw in pend:
                WO(jw)
            pend = []
            if i >= _LAG:
                j, c = items[i - _LAG]
                PV(j, c)
                if c == j:
                    pend.append(j)
        for jw in pend:
            WO(jw)

        prep_weights(jnp.minimum(h + 1, H - 1))

        @pl.when(h == H - 1)
        def _():
            o_ref[...] = acc[...].astype(BF16)

    return kernel


@jax.jit
def pallas_gated_mix__compressed_kv_cla__moe_arch_mod__prompt_kernel(
    A_x: jax.Array,
    A_c_kv: jax.Array,
    A_w_q: jax.Array,
    A_w_uk: jax.Array,
    A_w_uv: jax.Array,
    A_w_o: jax.Array,
    B_x: jax.Array,
    B_w_r: jax.Array,
    B_w_gate: jax.Array,
    B_w_up: jax.Array,
    B_w_down: jax.Array,
    gate_w: jax.Array,
):
    _, S, M = A_x.shape
    C = A_c_kv.shape[2]
    H, D = A_w_q.shape[1], A_w_q.shape[2]
    FF = B_w_gate.shape[1]
    xT = A_x[0].T
    woT = jnp.transpose(A_w_o, (0, 2, 1))
    wdT = B_w_down.T
    any_spec = pl.BlockSpec(memory_space=pl.ANY)
    outT = pl.pallas_call(
        _make_kernel(S, M, C, H, D, FF),
        grid=(H,),
        in_specs=[
            pl.BlockSpec((M, S), lambda h: (0, 0)),
            pl.BlockSpec((S, C), lambda h: (0, 0)),
            any_spec, any_spec, any_spec,
            pl.BlockSpec((1, M, D), lambda h: (h, 0, 0)),
            pl.BlockSpec((M,), lambda h: (0,)),
            pl.BlockSpec((M,), lambda h: (0,)),
            any_spec, any_spec, any_spec,
        ],
        out_specs=pl.BlockSpec((M, S), lambda h: (0, 0)),
        out_shape=jax.ShapeDtypeStruct((M, S), BF16),
        scratch_shapes=[
            pltpu.VMEM((2, M, D), U32), pltpu.VMEM((2, C, D), U32), pltpu.VMEM((2, C, D), U32),
            pltpu.VMEM((D, M), BF16), pltpu.VMEM((C, D), BF16), pltpu.VMEM((D, C), BF16),
            pltpu.VMEM((S, D), BF16), pltpu.VMEM((D, S), BF16),
            pltpu.VMEM((M, S), F32), pltpu.VMEM((1, S), F32), pltpu.VMEM((1, S), F32),
            pltpu.VMEM((M, FF), BF16), pltpu.VMEM((M, FF), BF16), pltpu.VMEM((M, FF), BF16),
            pltpu.SemaphoreType.DMA((2, 3)), pltpu.SemaphoreType.DMA((3,)),
        ],
        compiler_params=pltpu.CompilerParams(
            vmem_limit_bytes=100 << 20, dimension_semantics=("arbitrary",)),
    )(xT, A_c_kv[0], A_w_q, A_w_uk, A_w_uv, woT, B_w_r, gate_w, B_w_gate, B_w_up, wdT)
    return outT.T[None]
```

```python
import math

import jax
import jax.numpy as jnp
from jax import lax
import jax.experimental.pallas as pl
import jax.experimental.pallas.tpu as pltpu

F32, BF16, U32, I32 = jnp.float32, jnp.bfloat16, jnp.uint32, jnp.int32
_NT = (((1,), (1,)), ((), ()))
_NEG = -1e30
_B = 256
_T = 128
_LAG = 3
_NS = 6
_TREE = 1
_HI = 0xFFFF0000
_SREF = 1
_AREF = 0
_BFT = 0
_PF32 = 0
_TIE = 1
_KVAL = 2
_VVAL = 1


def _red(x, op, fn):
    n = _TREE
    if n > 1 and x.shape[0] % (8 * n) == 0:
        r = x.shape[0] // n
        parts = [x[i * r:(i + 1) * r] for i in range(n)]
        while len(parts) > 1:
            parts = [op(parts[i], parts[i + 1]) for i in range(0, len(parts), 2)]
        x = parts[0]
    return fn(x, axis=0, keepdims=True)


def _mm(a, b):
    return jnp.dot(a, b, preferred_element_type=F32)


def _mm_nt(a, b):
    return lax.dot_general(a, b, _NT, preferred_element_type=F32)


def _sigmoid(x):
    return 1.0 / (1.0 + jnp.exp(-x))


def _as_f32(u):
    return lax.bitcast_convert_type(u, F32)


def _cat(parts):
    return parts[0] if len(parts) == 1 else jnp.concatenate(parts, axis=1)


def _ld(ref, *lead, rows=None):
    u = ref.bitcast(U32)
    idx = lead if rows is None else lead + (slice(rows[0] // 2, (rows[0] + rows[1]) // 2),)
    return pltpu.bitcast(u[idx], BF16)


def _make_kernel(S, M, C, H, D, FF):
    NB = S // _B
    NP = H // 2
    NS_T, NC_T, ND_T = S // _T, C // _T, D // _T
    MF = M // _T
    assert NP == NB and ND_T == 2
    q_scale = math.log2(math.e) * (D ** -0.5)

    def kernel(xT_hbm, c_hbm, wq_hbm, wk_hbm, wv_hbm, woT_hbm, wr_hbm, gw_hbm,
               wg_hbm, wu_hbm, wdT_hbm, o_hbm,
               xT_s, c_s, wq_buf, wk_buf, wv_buf, woT_s, wr_s, gw_s, wg_s, wu_s, wdT_s,
               wqT_s, wk_s, wvT_s, lhs_s, qc_s, k_s, vT_s, g_s, r_s, y_s, o_s, s_s, a_s, idx_s,
               sem, q_sem, kv_sem, o_sem):
        def tiled(src, dst, n):
            return [(src.at[..., t * _T:(t + 1) * _T], dst.at[t]) for t in range(n)]

        misc = dict(x=tiled(xT_hbm, xT_s, NS_T), c=tiled(c_hbm, c_s, NC_T),
                    wo=tiled(woT_hbm, woT_s, ND_T), wr=[(wr_hbm, wr_s)], gw=[(gw_hbm, gw_s)],
                    wg=[(wg_hbm, wg_s)], wu=[(wu_hbm, wu_s)], wd=[(wdT_hbm, wdT_s)])

        def cps(name):
            s = sem.at[list(misc).index(name)]
            return [pltpu.make_async_copy(src, dst, s) for src, dst in misc[name]]

        def start(*names):
            for n in names:
                for d in cps(n):
                    d.start()

        def wait(*names):
            for n in names:
                for d in cps(n):
                    d.wait()

        def q_cp(p):
            return pltpu.make_async_copy(wq_hbm.bitcast(U32).at[:, p, :], wq_buf.at[p], q_sem.at[p])

        def kv_cps(p):
            return [pltpu.make_async_copy(src.bitcast(U32).at[:, p, :], dst.at[p & 1], kv_sem.at[p & 1, i])
                    for i, (src, dst) in enumerate(((wk_hbm, wk_buf), (wv_hbm, wv_buf)))]

        def o_cp(j):
            c0 = pl.multiple_of(j * _B, _B)
            return pltpu.make_async_copy(o_s.at[j & 1], o_hbm.at[:, pl.ds(c0, _B)], o_sem.at[j & 1])

        def prep_q(p):
            w = wq_buf[p].T
            for half, u in enumerate((w << 16, w & jnp.uint32(_HI))):
                wb = _as_f32(u).astype(BF16)
                for t in range(MF):
                    wqT_s[t, half * D:(half + 1) * D, :] = wb[:, t * _T:(t + 1) * _T]
                wqT_s[MF, half * D:(half + 1) * D, 0:M - MF * _T] = wb[:, MF * _T:]

        def wqT():
            return _cat([_ld(wqT_s, t) for t in range(MF)] + [_ld(wqT_s, MF)[:, 0:M - MF * _T]])

        def prep_kv(hh):
            slot = (hh >> 1) & 1
            sh = jnp.asarray((1 - (hh & 1)) * 16).astype(U32)
            wkf = _as_f32((wk_buf[slot] << sh) & jnp.uint32(_HI))
            wk = wkf.astype(BF16)
            for t in range(ND_T):
                wk_s[t] = wk[:, t * _T:(t + 1) * _T]
            wv = _as_f32((wv_buf[slot] << sh) & jnp.uint32(_HI))
            wvT = wv.astype(BF16).T if _BFT else wv.T.astype(BF16)
            for t in range(NC_T):
                wvT_s[t] = wvT[:, t * _T:(t + 1) * _T]
            return wkf, wk, wvT

        q_cp(0).start()
        start('wr', 'gw', 'x')
        q_cp(0).wait()
        q_cp(1).start()
        wqT_s[MF] = jnp.zeros((2 * D, _T), BF16)
        prep_q(0)
        wait('wr', 'gw')
        row = lax.broadcasted_iota(I32, (16, M), 0)
        wr = wr_s[...].astype(F32).reshape(1, M)
        gw = gw_s[...].astype(F32).reshape(1, M)
        lhs_s[...] = jnp.where(row == 0, wr, jnp.where(row == 1, gw, 0.0)).astype(BF16)
        idx_s[2] = 0
        wait('x')

        def phase_q(p, carry):
            @pl.when(p + 1 < NP)
            def _():
                q_cp(p + 1).wait()

            @pl.when(p + 2 < NP)
            def _():
                q_cp(p + 2).start()

            @pl.when(p == 0)
            def _():
                start('c')

            @pl.when(p == 1)
            def _():
                for d in kv_cps(0):
                    d.start()
                start('wg')

            @pl.when(p == 2)
            def _():
                start('wu', 'wd')

            @pl.when(p == 3)
            def _():
                for d in kv_cps(1):
                    d.start()

            @pl.when(p == 4)
            def _():
                start('wo')

            for t in range(NS_T):
                q = _mm(wqT(), _ld(xT_s, t)) * q_scale
                qc_s[2 * p, t] = q[:D].astype(BF16)
                qc_s[2 * p + 1, t] = q[D:].astype(BF16)
                if t == 1:
                    rg = _mm(lhs_s[...], _cat([_ld(xT_s, 2 * p), _ld(xT_s, 2 * p + 1)]))
                    c0 = pl.multiple_of(p * _B, _B)
                    r_s[:, pl.ds(c0, _B)] = rg[0:1, :].astype(BF16).astype(F32)
                    g_s[:, pl.ds(c0, _B)] = _sigmoid(rg[1:2, :])
            prep_q(jnp.minimum(p + 1, NP - 1))
            return carry

        lax.fori_loop(0, NP, phase_q, 0)

        wait('wg', 'wu', 'wd', 'c')
        for d in kv_cps(0):
            d.wait()
        lane = lax.broadcasted_iota(I32, (1, S), 1)
        idxs, cur = [], r_s[...]
        for n in range(2):
            mx = jnp.max(cur, axis=1, keepdims=True)
            ii = jnp.min(jnp.where(cur == mx, lane, S - 1))
            idxs.append(ii)
            idx_s[n] = ii
            cur = jnp.where(lane == ii, -jnp.inf, cur)
        row16 = lax.broadcasted_iota(I32, (16, _T), 0)
        lane16 = lax.broadcasted_iota(I32, (16, _T), 1)
        xs = None
        for n, ii in enumerate(idxs):
            oh = jnp.where(jnp.logical_and(row16 == n, lane16 == (ii & (_T - 1))), 1.0, 0.0).astype(BF16)
            xr = _mm_nt(oh, xT_s[ii >> 7])
            xs = xr if xs is None else xs + xr
        xs = xs.astype(BF16)
        gt = _mm(xs, wg_s[...])
        up = _mm(xs, wu_s[...])
        hid = (gt * _sigmoid(gt) * up).astype(BF16)
        hid128 = jnp.concatenate([hid, jnp.zeros((_T - 16, FF), BF16)], axis=0)
        yT = _mm_nt(wdT_s[...], hid128)
        for n in range(2):
            y_s[n] = jnp.broadcast_to(yT[:, n:n + 1], (M, _T))

        zz = idx_s[2]
        for rf in list(s_s) + list(a_s):
            rf[zz, 0:8, :] = jnp.zeros((8, _B), F32)

        def head(h, carry):
            wkf0, wk0, wvT0 = prep_kv(h)
            key = lax.broadcasted_iota(I32, (_T, _T), 0)
            qry = lax.broadcasted_iota(I32, (_T, _T), 1)
            tri = key <= qry

            def c_rows(r0, n):
                return _cat([_ld(c_s, t, rows=(r0, n)) for t in range(NC_T)])

            def k_rows(r0, n):
                return _cat([_ld(k_s, t, rows=(r0, n)) for t in range(ND_T)])

            def pK(j, t):
                if _KVAL and j == 0:
                    w = (wkf0 if _KVAL == 2 else wk0)[:, t * _T:(t + 1) * _T]
                else:
                    w = _ld(wk_s, t)
                k_s[t, j * _B:(j + 1) * _B, :] = _mm(c_rows(j * _B, _B), w).astype(BF16)

            def pV(j, t):
                if _VVAL and j == 0 and t < _VVAL:
                    wvT = wvT0
                else:
                    wvT = _cat([_ld(wvT_s, u) for u in range(NC_T)])
                vT_s[2 * j + t] = _mm_nt(wvT, c_rows(j * _B + t * _T, _T)).astype(BF16)

            done = set()

            def piece(name, j, t):
                if j < NB and (name, j, t) not in done:
                    done.add((name, j, t))
                    {'K': pK, 'V': pV}[name](j, t)

            items = [(j, c) for j in range(NB) for c in range(j + 1)]
            state, scores = {}, {}

            def cvt(p):
                return p if _PF32 else p.astype(BF16)

            def QK(j, c):
                for t in range(2):
                    piece('K', c, t)
                k0 = c * _B
                q1 = _ld(qc_s, h, 2 * j + 1)
                q = _cat([_ld(qc_s, h, 2 * j), q1])
                if c < j:
                    s = _mm(k_rows(k0, _B), q)
                    s2 = None
                    mc = _red(s, jnp.maximum, jnp.max)
                else:
                    s = _mm(k_rows(k0, _T), q)
                    hh = _T // 2
                    s2 = jnp.concatenate([_mm(k_rows(k0 + _T, hh), q1),
                                          _mm(k_rows(k0 + _T + hh, hh), q1)], axis=0)
                    s = jnp.concatenate([jnp.where(tri, s[:, :_T], _NEG), s[:, _T:]], axis=1)
                    s2 = jnp.where(tri, s2, _NEG)
                    mc = _red(s, jnp.maximum, jnp.max)
                    m2 = _red(s2, jnp.maximum, jnp.max)
                    mc = jnp.concatenate([mc[:, :_T], jnp.maximum(mc[:, _T:], m2)], axis=1)
                if _SREF:
                    slot = items.index((j, c)) % _NS
                    s_s[slot][0, 0:s.shape[0], :] = s
                    if s2 is not None:
                        s_s[slot][0, _T:, _T:] = s2
                scores[(j, c)] = (s, s2, mc)

            def PV(j, c):
                for t in range(2):
                    piece('V', c, t)
                s, s2, m = scores.pop((j, c))
                if _SREF:
                    slot = items.index((j, c)) % _NS
                    s = s_s[slot][0, 0:s.shape[0], :]
                    if s2 is not None:
                        s2 = s_s[slot][0, _T:, _T:]
                first = j not in state
                if not first:
                    m0, l0, o0 = state[j]
                    m = jnp.maximum(m0, m)
                    al = jnp.exp2(m0 - m)
                p = jnp.exp2(s - m)
                l = _red(p, jnp.add, jnp.sum)
                if c < j:
                    o = _mm(_cat([_ld(vT_s, 2 * c), _ld(vT_s, 2 * c + 1)]), cvt(p))
                else:
                    p2 = jnp.exp2(s2 - m[:, _T:])
                    l = jnp.concatenate([l[:, :_T], l[:, _T:] + _red(p2, jnp.add, jnp.sum)], axis=1)
                    pa = cvt(p)
                    pb = cvt(p2)
                    o = jnp.concatenate([_mm(_ld(vT_s, 2 * c, rows=(r, D // 2)), pa)
                                         for r in range(0, D, D // 2)], axis=0)
                    o2 = jnp.concatenate([_mm(_ld(vT_s, 2 * c + 1, rows=(r, D // 4)), pb)
                                          for r in range(0, D, D // 4)], axis=0)
                    o = jnp.concatenate([o[:, :_T], o[:, _T:] + o2], axis=1)
                if _TIE:
                    l = jnp.where(o[0:1] != o[0:1], o[0:1], l)
                if not first:
                    l = l0 * al + l
                    o = (a_s[j % 2][0] if _AREF else o0) * al + o
                if _AREF and c < j:
                    a_s[j % 2][0] = o
                state[j] = (m, l, o)
                if c == j:
                    state.pop(j)
                    ctx = (o * (1.0 / l)).astype(BF16)
                    for t in range(2):
                        qc_s[h, 2 * j + t] = ctx[:, t * _T:(t + 1) * _T]

            n_it = len(items)
            for i in range(n_it + _LAG):
                if i < n_it:
                    j, c = items[i]
                    QK(j, c)
                    pcs = [('V', j, 0), ('V', j, 1), ('K', j + 1, 0), ('K', j + 1, 1)]
                    lo, hi = len(pcs) * c // (j + 1), len(pcs) * (c + 1) // (j + 1)
                    for pc in pcs[lo:hi]:
                        piece(*pc)
                if i >= _LAG:
                    PV(*items[i - _LAG])

            @pl.when(jnp.logical_and((h & 1) == 1, h + 1 < H))
            def _():
                for d in kv_cps((h + 1) >> 1):
                    d.wait()

            @pl.when(jnp.logical_and((h & 1) == 1, h + 3 < H))
            def _():
                for d in kv_cps((h + 3) >> 1):
                    d.start()
            return carry

        lax.fori_loop(0, H, head, 0)

        wait('wo')

        def phase_o(j, carry):
            @pl.when(j >= 2)
            def _():
                o_cp(j - 2).wait()

            c0 = pl.multiple_of(j * _B, _B)
            a = None
            for hh in range(0, H, 2):
                w2 = _cat([_ld(woT_s, t, hh + u) for u in range(2) for t in range(ND_T)])
                x2 = jnp.concatenate([_cat([_ld(qc_s, hh + u, 2 * j), _ld(qc_s, hh + u, 2 * j + 1)])
                                      for u in range(2)], axis=0)
                part = _mm(w2, x2)
                a = part if a is None else a + part
            g = g_s[:, pl.ds(c0, _B)]
            rs = _sigmoid(r_s[:, pl.ds(c0, _B)])
            col = lax.broadcasted_iota(I32, (1, _B), 1) + j * _B
            b = _cat([xT_s[2 * j], xT_s[2 * j + 1]]).astype(F32)
            for n in range(2):
                y2 = jnp.concatenate([y_s[n], y_s[n]], axis=1)
                b = b + y2 * jnp.where(col == idx_s[n], rs, 0.0)
            o_s[j & 1] = (g * a + (1.0 - g) * b).astype(BF16)
            o_cp(j).start()
            return carry

        lax.fori_loop(0, NB, phase_o, 0)
        o_cp(NB - 2).wait()
        o_cp(NB - 1).wait()

    return kernel


@jax.jit
def pallas_gated_mix__compressed_kv_cla__moe_arch_mod__prompt_kernel(
    A_x: jax.Array,
    A_c_kv: jax.Array,
    A_w_q: jax.Array,
    A_w_uk: jax.Array,
    A_w_uv: jax.Array,
    A_w_o: jax.Array,
    B_x: jax.Array,
    B_w_r: jax.Array,
    B_w_gate: jax.Array,
    B_w_up: jax.Array,
    B_w_down: jax.Array,
    gate_w: jax.Array,
):
    _, S, M = A_x.shape
    C = A_c_kv.shape[2]
    H, D = A_w_q.shape[1], A_w_q.shape[2]
    FF = B_w_gate.shape[1]
    xT = A_x[0].T
    woT = jnp.transpose(A_w_o, (0, 2, 1))
    wdT = B_w_down.T
    any_spec = pl.BlockSpec(memory_space=pl.ANY)
    V = pltpu.VMEM
    outT = pl.pallas_call(
        _make_kernel(S, M, C, H, D, FF),
        in_specs=[any_spec] * 11,
        out_specs=any_spec,
        out_shape=jax.ShapeDtypeStruct((M, S), BF16),
        scratch_shapes=[
            V((S // _T, M, _T), BF16), V((C // _T, S, _T), BF16),
            V((H // 2, M, D), U32), V((2, C, D), U32), V((2, C, D), U32),
            V((D // _T, H, M, _T), BF16), V((M,), BF16), V((M,), BF16),
            V((M, FF), BF16), V((M, FF), BF16), V((M, FF), BF16),
            V((pl.cdiv(M, _T), 2 * D, _T), BF16), V((D // _T, C, _T), BF16), V((C // _T, D, _T), BF16),
            V((16, M), BF16),
            V((H, S // _T, D, _T), BF16), V((D // _T, S, _T), BF16), V((S // _T, D, _T), BF16),
            V((1, S), F32), V((1, S), F32), V((2, M, _T), F32), V((2, M, _B), BF16),
            [V((1, _B, _B), F32)] * _NS, [V((1, D, _B), F32)] * 2,
            pltpu.SMEM((3,), I32),
            pltpu.SemaphoreType.DMA((8,)), pltpu.SemaphoreType.DMA((H // 2,)),
            pltpu.SemaphoreType.DMA((2, 2)), pltpu.SemaphoreType.DMA((2,)),
        ],
        compiler_params=pltpu.CompilerParams(vmem_limit_bytes=100 << 20),
    )(xT, A_c_kv[0], A_w_q, A_w_uk, A_w_uv, woT, B_w_r, gate_w, B_w_gate, B_w_up, wdT)
    return outT.T[None]
```

```python
import math

import jax
import jax.numpy as jnp
from jax import lax
import jax.experimental.pallas as pl
import jax.experimental.pallas.tpu as pltpu

F32, BF16, U32, I32 = jnp.float32, jnp.bfloat16, jnp.uint32, jnp.int32
_NT = (((1,), (1,)), ((), ()))
_NEG = -1e30
_HI = 0xFFFF0000
_T = 128
_B = 256
_LAG = 4
_NS = 6
_XA, _XB = 2, 7


def _mm(a, b):
    return jnp.dot(a, b, preferred_element_type=F32)


def _mm_nt(a, b):
    return lax.dot_general(a, b, _NT, preferred_element_type=F32)


def _sigmoid(x):
    return 1.0 / (1.0 + jnp.exp(-x))


def _as_f32(u):
    return lax.bitcast_convert_type(u, F32)


def _cat(parts, axis=1):
    return parts[0] if len(parts) == 1 else jnp.concatenate(parts, axis=axis)


def _ld(ref, *lead, rows=None):
    u = ref.bitcast(U32)
    idx = lead if rows is None else lead + (slice(rows[0] // 2, (rows[0] + rows[1]) // 2),)
    return pltpu.bitcast(u[idx], BF16)


def _make_kernel(S, M, C, H, D, FF):
    NB, NP = S // _B, H // 2
    NS_T, NC_T, ND_T, NF_T = S // _T, C // _T, D // _T, FF // _T
    MF, MR = M // _T, M % _T
    assert ND_T == 2 and MR > 0 and _NS > _LAG
    q_scale = math.log2(math.e) * (D ** -0.5)

    def kernel(xT_hbm, c_hbm, wq_hbm, wk_hbm, wv_hbm, woT_hbm, wr_hbm, gw_hbm,
               wg_hbm, wu_hbm, wdT_hbm, o_hbm,
               xT_s, c_s, wq_buf, wk_buf, wv_buf, woT_s, wr_s, gw_s, wg_s, wu_s, wdT_s,
               wqT_s, wk_s, wvT_s, lhs_s, qc_s, k_s, vT_s, g_s, r_s, y_s, o_s, s_s, idx_s,
               sem, q_sem, kv_sem, o_sem):
        def tiled(src, dst, n):
            return [(src.at[..., t * _T:(t + 1) * _T], dst.at[t]) for t in range(n)]

        xt = tiled(xT_hbm, xT_s, NS_T)
        groups = dict(xa=[(wr_hbm, wr_s), (gw_hbm, gw_s)] + xt[:_XA], xb=xt[_XA:_XB], xc=xt[_XB:],
                      ffn=[(wg_hbm, wg_s), (wu_hbm, wu_s), (wdT_hbm, wdT_s)],
                      c=tiled(c_hbm, c_s, NC_T), wo=tiled(woT_hbm, woT_s, ND_T))

        def group(name):
            s = sem.at[list(groups).index(name)]
            return [pltpu.make_async_copy(src, dst, s) for src, dst in groups[name]]

        def q_cp(p):
            return [pltpu.make_async_copy(wq_hbm.bitcast(U32).at[:, p, :], wq_buf.at[p], q_sem.at[p])]

        def kv_cp(p):
            return [pltpu.make_async_copy(src.bitcast(U32).at[:, p, :], dst.at[p & 1], kv_sem.at[p & 1])
                    for src, dst in ((wk_hbm, wk_buf), (wv_hbm, wv_buf))]

        def o_cp(j):
            c0 = pl.multiple_of(j * _B, _B)
            return [pltpu.make_async_copy(o_s.at[j & 1], o_hbm.at[:, pl.ds(c0, _B)], o_sem.at[j & 1])]

        def start(cps):
            for d in cps:
                d.start()

        def wait(cps):
            for d in cps:
                d.wait()

        def prep_q(p):
            w = wq_buf[p].T
            for half, u in enumerate((w << 16, w & jnp.uint32(_HI))):
                wb = _as_f32(u).astype(BF16)
                for t in range(MF):
                    wqT_s[t, half * D:(half + 1) * D, :] = wb[:, t * _T:(t + 1) * _T]
                wqT_s[MF, half * D:(half + 1) * D, 0:MR] = wb[:, MF * _T:]

        def q_tile(p, t):
            wqT = _cat([_ld(wqT_s, u) for u in range(MF)] + [_ld(wqT_s, MF)[:, 0:MR]])
            q = _mm(wqT, _ld(xT_s, t)) * q_scale
            qc_s[2 * p, t] = q[:D].astype(BF16)
            qc_s[2 * p + 1, t] = q[D:].astype(BF16)

        def q_first(t0, t1):
            for t in range(t0, t1):
                q_tile(0, t)
                rg = _mm(lhs_s[...], _ld(xT_s, t))
                r_s[:, t * _T:(t + 1) * _T] = rg[0:1, :].astype(BF16).astype(F32)
                g_s[:, t * _T:(t + 1) * _T] = _sigmoid(rg[1:2, :])

        start(q_cp(0) + group('xa') + group('xb') + group('xc'))
        for p in range(1, NP):
            start(q_cp(p))
        start(group('ffn') + group('c') + kv_cp(0) + kv_cp(1) + group('wo'))
        wqT_s[MF] = jnp.zeros((2 * D, _T), BF16)
        idx_s[2] = 0
        wait(q_cp(0))
        prep_q(0)
        wait(group('xa'))
        row = lax.broadcasted_iota(I32, (16, M), 0)
        wr = wr_s[...].astype(F32).reshape(1, M)
        gw = gw_s[...].astype(F32).reshape(1, M)
        lhs_s[...] = jnp.where(row == 0, wr, jnp.where(row == 1, gw, 0.0)).astype(BF16)
        q_first(0, _XA)
        wait(group('xb'))
        q_first(_XA, _XB)
        wait(group('xc') + q_cp(1))
        q_first(_XB, NS_T)
        prep_q(1)
        wait(q_cp(2))

        def phase_q(i, carry):
            p = i + 1
            for t in range(NS_T):
                q_tile(p, t)
            prep_q(p + 1)
            pl.when(p + 2 < NP)(lambda: wait(q_cp(p + 2)))
            return carry

        lax.fori_loop(0, NP - 2, phase_q, 0)
        wait(group('ffn'))

        lane = lax.broadcasted_iota(I32, (1, S), 1)
        idxs, cur = [], r_s[...]
        for n in range(2):
            mx = jnp.max(cur, axis=1, keepdims=True)
            ii = jnp.min(jnp.where(cur == mx, lane, S - 1))
            idxs.append(ii)
            idx_s[n] = ii
            cur = jnp.where(lane == ii, -jnp.inf, cur)
        ffn = {}

        def ffn_select():
            row16 = lax.broadcasted_iota(I32, (16, _T), 0)
            lane16 = lax.broadcasted_iota(I32, (16, _T), 1)
            xs = None
            for n, ii in enumerate(idxs):
                oh = jnp.logical_and(row16 == n, lane16 == (ii & (_T - 1)))
                xr = _mm_nt(jnp.where(oh, 1.0, 0.0).astype(BF16), _ld(xT_s, ii // _T))
                xs = xr if xs is None else xs + xr
            ffn['x'] = xs.astype(BF16)

        def ffn_hidden(f):
            gt = _mm(ffn['x'], wg_s[:, f * _T:(f + 1) * _T])
            up = _mm(ffn['x'], wu_s[:, f * _T:(f + 1) * _T])
            ffn[f] = (gt * _sigmoid(gt) * up).astype(BF16)

        def ffn_down(f):
            y = _mm_nt(ffn[f], wdT_s[:, f * _T:(f + 1) * _T])
            ffn['y'] = y if 'y' not in ffn else ffn['y'] + y

        after = {3: [ffn_select]}
        for f in range(NF_T):
            after.setdefault(4 + f * 10 // NF_T, []).append(lambda f=f: ffn_hidden(f))
            after.setdefault(5 + f * 10 // NF_T, []).append(lambda f=f: ffn_down(f))
        for t in range(NS_T):
            q_tile(NP - 1, t)
            for fn in after.get(t, []):
                fn()
        yp = jnp.concatenate([ffn['y'], jnp.zeros((16, (MF + 1) * _T - M), F32)], axis=1)
        yT = jnp.concatenate([yp, jnp.zeros((_T - 16, (MF + 1) * _T), F32)], axis=0).T[:M]
        for n in range(2):
            y_s[n] = jnp.broadcast_to(yT[:, n:n + 1], (M, _T))

        zero = idx_s[2]
        for ref in s_s:
            ref[zero, 0:8, :] = jnp.zeros((8, _B), F32)
        wait(group('c') + kv_cp(0))

        def head(h, carry):
            slot = (h >> 1) & 1
            sh = ((1 - (h & 1)) * 16).astype(U32)
            wk = _as_f32((wk_buf[slot] << sh) & jnp.uint32(_HI))
            for t in range(ND_T):
                wk_s[t] = wk[:, t * _T:(t + 1) * _T].astype(BF16)
            wvT = _as_f32((wv_buf[slot] << sh) & jnp.uint32(_HI)).T.astype(BF16)
            for t in range(NC_T):
                wvT_s[t] = wvT[:, t * _T:(t + 1) * _T]
            tri = (lax.broadcasted_iota(I32, (_T, _T), 0) <= lax.broadcasted_iota(I32, (_T, _T), 1))

            def c_rows(r0, n):
                return _cat([_ld(c_s, t, rows=(r0, n)) for t in range(NC_T)])

            def k_rows(r0, n):
                return _cat([_ld(k_s, t, rows=(r0, n)) for t in range(ND_T)])

            def proj_k(j, t):
                w = wk[:, t * _T:(t + 1) * _T] if j == 0 else _ld(wk_s, t)
                k_s[t, j * _B:(j + 1) * _B, :] = _mm(c_rows(j * _B, _B), w).astype(BF16)

            def proj_v(j, t):
                w = wvT if (j, t) == (0, 0) else _cat([_ld(wvT_s, u) for u in range(NC_T)])
                vT_s[2 * j + t] = _mm_nt(w, c_rows(j * _B + t * _T, _T)).astype(BF16)

            done = set()

            def piece(fn, j, t):
                if j < NB and (fn, j, t) not in done:
                    done.add((fn, j, t))
                    fn(j, t)

            items = [(j, c) for j in range(NB) for c in range(j + 1)]
            state, cmax = {}, {}

            def qk(i):
                j, c = items[i]
                for t in range(2):
                    piece(proj_k, c, t)
                k0, st = c * _B, s_s[i % _NS]
                q1 = _ld(qc_s, h, 2 * j + 1)
                q = _cat([_ld(qc_s, h, 2 * j), q1])
                if c < j:
                    s = _mm(k_rows(k0, _B), q)
                    st[0] = s
                    cmax[i] = jnp.max(s, axis=0, keepdims=True)
                else:
                    s = _mm(k_rows(k0, _T), q)
                    s2 = _cat([_mm(k_rows(k0 + _T + r, _T // 2), q1) for r in (0, _T // 2)], axis=0)
                    s = _cat([jnp.where(tri, s[:, :_T], _NEG), s[:, _T:]])
                    s2 = jnp.where(tri, s2, _NEG)
                    st[0, 0:_T, :] = s
                    st[0, _T:, _T:] = s2
                    m = jnp.max(s, axis=0, keepdims=True)
                    cmax[i] = _cat([m[:, :_T], jnp.maximum(m[:, _T:], jnp.max(s2, axis=0, keepdims=True))])

            def pv(i):
                j, c = items[i]
                for t in range(2):
                    piece(proj_v, c, t)
                st, m = s_s[i % _NS], cmax.pop(i)
                if c > 0:
                    m0, l0, o0 = state[j]
                    m = jnp.maximum(m0, m)
                    alpha = jnp.exp2(m0 - m)
                if c < j:
                    p = jnp.exp2(st[0] - m)
                    l = jnp.sum(p, axis=0, keepdims=True)
                    o = _mm(_cat([_ld(vT_s, 2 * c), _ld(vT_s, 2 * c + 1)]), p.astype(BF16))
                else:
                    p = jnp.exp2(st[0, 0:_T, :] - m)
                    p2 = jnp.exp2(st[0, _T:, _T:] - m[:, _T:])
                    l = jnp.sum(p, axis=0, keepdims=True)
                    l = _cat([l[:, :_T], l[:, _T:] + jnp.sum(p2, axis=0, keepdims=True)])
                    p, p2 = p.astype(BF16), p2.astype(BF16)
                    o = _cat([_mm(_ld(vT_s, 2 * c, rows=(r, D // 2)), p)
                              for r in range(0, D, D // 2)], axis=0)
                    o2 = _cat([_mm(_ld(vT_s, 2 * c + 1, rows=(r, D // 4)), p2)
                               for r in range(0, D, D // 4)], axis=0)
                    o = _cat([o[:, :_T], o[:, _T:] + o2])
                l = jnp.where(o[0:1] != o[0:1], o[0:1], l)
                if c > 0:
                    l = l0 * alpha + l
                    o = o0 * alpha + o
                state[j] = (m, l, o)
                if c == j:
                    ctx = (o * (1.0 / l)).astype(BF16)
                    for t in range(2):
                        qc_s[h, 2 * j + t] = ctx[:, t * _T:(t + 1) * _T]

            for i in range(len(items) + _LAG):
                if i < len(items):
                    qk(i)
                    j, c = items[i]
                    fill = [(proj_v, j, 0), (proj_v, j, 1), (proj_k, j + 1, 0), (proj_k, j + 1, 1)]
                    for pc in fill[len(fill) * c // (j + 1):len(fill) * (c + 1) // (j + 1)]:
                        piece(*pc)
                if i >= _LAG:
                    pv(i - _LAG)

            odd = (h & 1) == 1
            pl.when(jnp.logical_and(odd, h + 3 < H))(lambda: start(kv_cp((h + 3) >> 1)))
            pl.when(jnp.logical_and(odd, h + 1 < H))(lambda: wait(kv_cp((h + 1) >> 1)))
            return carry

        lax.fori_loop(0, H, head, 0)
        wait(group('wo'))

        def phase_o(j, carry):
            pl.when(j >= 2)(lambda: wait(o_cp(j - 2)))
            c0 = pl.multiple_of(j * _B, _B)
            a = None
            for hh in range(0, H, 2):
                w2 = _cat([_ld(woT_s, t, hh + u) for u in range(2) for t in range(ND_T)])
                x2 = _cat([_cat([_ld(qc_s, hh + u, 2 * j), _ld(qc_s, hh + u, 2 * j + 1)])
                           for u in range(2)], axis=0)
                part = _mm(w2, x2)
                a = part if a is None else a + part
            g = g_s[:, pl.ds(c0, _B)]
            rs = _sigmoid(r_s[:, pl.ds(c0, _B)])
            col = lax.broadcasted_iota(I32, (1, _B), 1) + j * _B
            b = _cat([xT_s[2 * j], xT_s[2 * j + 1]]).astype(F32)
            for n in range(2):
                b = b + _cat([y_s[n], y_s[n]]) * jnp.where(col == idx_s[n], rs, 0.0)
            o_s[j & 1] = (g * a + (1.0 - g) * b).astype(BF16)
            start(o_cp(j))
            return carry

        lax.fori_loop(0, NB, phase_o, 0)
        wait(o_cp(NB - 2) + o_cp(NB - 1))

    return kernel


@jax.jit
def pallas_gated_mix__compressed_kv_cla__moe_arch_mod__prompt_kernel(
    A_x: jax.Array,
    A_c_kv: jax.Array,
    A_w_q: jax.Array,
    A_w_uk: jax.Array,
    A_w_uv: jax.Array,
    A_w_o: jax.Array,
    B_x: jax.Array,
    B_w_r: jax.Array,
    B_w_gate: jax.Array,
    B_w_up: jax.Array,
    B_w_down: jax.Array,
    gate_w: jax.Array,
):
    _, S, M = A_x.shape
    C = A_c_kv.shape[2]
    H, D = A_w_q.shape[1], A_w_q.shape[2]
    FF = B_w_gate.shape[1]
    xT = A_x[0].T
    woT = jnp.transpose(A_w_o, (0, 2, 1))
    wdT = B_w_down.T
    any_spec = pl.BlockSpec(memory_space=pl.ANY)
    V = pltpu.VMEM
    outT = pl.pallas_call(
        _make_kernel(S, M, C, H, D, FF),
        in_specs=[any_spec] * 11,
        out_specs=any_spec,
        out_shape=jax.ShapeDtypeStruct((M, S), BF16),
        scratch_shapes=[
            V((S // _T, M, _T), BF16), V((C // _T, S, _T), BF16),
            V((H // 2, M, D), U32), V((2, C, D), U32), V((2, C, D), U32),
            V((D // _T, H, M, _T), BF16), V((M,), BF16), V((M,), BF16),
            V((M, FF), BF16), V((M, FF), BF16), V((M, FF), BF16),
            V((pl.cdiv(M, _T), 2 * D, _T), BF16), V((D // _T, C, _T), BF16),
            V((C // _T, D, _T), BF16), V((16, M), BF16),
            V((H, S // _T, D, _T), BF16),
            V((D // _T, S, _T), BF16), V((S // _T, D, _T), BF16),
            V((1, S), F32), V((1, S), F32), V((2, M, _T), F32), V((2, M, _B), BF16),
            [V((1, _B, _B), F32)] * _NS,
            pltpu.SMEM((3,), I32),
            pltpu.SemaphoreType.DMA((6,)), pltpu.SemaphoreType.DMA((H // 2,)),
            pltpu.SemaphoreType.DMA((2,)), pltpu.SemaphoreType.DMA((2,)),
        ],
        compiler_params=pltpu.CompilerParams(vmem_limit_bytes=100 << 20),
    )(xT, A_c_kv[0], A_w_q, A_w_uk, A_w_uv, woT, B_w_r, gate_w, B_w_gate, B_w_up, wdT)
    return outT.T[None]
```

```python
import math

import jax
import jax.numpy as jnp
from jax import lax
import jax.experimental.pallas as pl
import jax.experimental.pallas.tpu as pltpu

F32, BF16, U32, I32 = jnp.float32, jnp.bfloat16, jnp.uint32, jnp.int32
_NT = (((1,), (1,)), ((), ()))
_NEG = -1e30
_HI = 0xFFFF0000
_T = 128
_B = 256
_LAG = 4
_NS = 6
_XA, _XB = 2, 7


def _mm(a, b):
    return jnp.dot(a, b, preferred_element_type=F32)


def _mm_nt(a, b):
    return lax.dot_general(a, b, _NT, preferred_element_type=F32)


def _sigmoid(x):
    return 1.0 / (1.0 + jnp.exp(-x))


def _as_f32(u):
    return lax.bitcast_convert_type(u, F32)


def _cat(parts, axis=1):
    return parts[0] if len(parts) == 1 else jnp.concatenate(parts, axis=axis)


def _ld(ref, *lead, rows=None):
    u = ref.bitcast(U32)
    idx = lead if rows is None else lead + (slice(rows[0] // 2, (rows[0] + rows[1]) // 2),)
    return pltpu.bitcast(u[idx], BF16)


def _make_kernel(S, M, C, H, D, FF):
    NB, NP = S // _B, H // 2
    NS_T, NC_T, ND_T, NF_T = S // _T, C // _T, D // _T, FF // _T
    MF, MR = M // _T, M % _T
    assert ND_T == 2 and MR > 0 and _NS > _LAG
    q_scale = math.log2(math.e) * (D ** -0.5)

    def kernel(xT_hbm, c_hbm, wq_hbm, wk_hbm, wv_hbm, woT_hbm, wr_hbm, gw_hbm,
               wg_hbm, wu_hbm, wdT_hbm, o_hbm,
               xT_s, c_s, wq_buf, wk_buf, wv_buf, woT_s, wr_s, gw_s, wg_s, wu_s, wdT_s,
               wqT_s, wk_s, wvT_s, lhs_s, qc_s, q_s, k_s, vT_s, g_s, r_s, y_s, o_s, s_s, idx_s,
               sem, q_sem, kv_sem, o_sem):
        def tiled(src, dst, n):
            return [(src.at[..., t * _T:(t + 1) * _T], dst.at[t]) for t in range(n)]

        xt = tiled(xT_hbm, xT_s, NS_T)
        groups = dict(xa=[(wr_hbm, wr_s), (gw_hbm, gw_s)] + xt[:_XA], xb=xt[_XA:_XB], xc=xt[_XB:],
                      ffn=[(wg_hbm, wg_s), (wu_hbm, wu_s), (wdT_hbm, wdT_s)],
                      c=tiled(c_hbm, c_s, NC_T), wo=tiled(woT_hbm, woT_s, ND_T))

        def group(name):
            s = sem.at[list(groups).index(name)]
            return [pltpu.make_async_copy(src, dst, s) for src, dst in groups[name]]

        def q_cp(p):
            return [pltpu.make_async_copy(wq_hbm.bitcast(U32).at[:, p, :], wq_buf.at[p], q_sem.at[p])]

        def kv_cp(p):
            return [pltpu.make_async_copy(src.bitcast(U32).at[:, p, :], dst.at[p], kv_sem)
                    for src, dst in ((wk_hbm, wk_buf), (wv_hbm, wv_buf))]

        def o_cp(j):
            c0 = pl.multiple_of(j * _B, _B)
            return [pltpu.make_async_copy(o_s.at[j & 1], o_hbm.at[:, pl.ds(c0, _B)], o_sem.at[j & 1])]

        def start(cps):
            for d in cps:
                d.start()

        def wait(cps):
            for d in cps:
                d.wait()

        def prep_q(p, b):
            w = wq_buf[p].T
            for half, u in enumerate((w << 16, w & jnp.uint32(_HI))):
                wb = _as_f32(u)
                for t in range(MF):
                    wqT_s[b][t, half * D:(half + 1) * D, :] = wb[:, t * _T:(t + 1) * _T].astype(BF16)
                wqT_s[b][MF, half * D:(half + 1) * D, 0:MR] = wb[:, MF * _T:].astype(BF16)

        def q_tile(p, t, b):
            wqT = _cat([_ld(wqT_s[b], u) for u in range(MF)] + [_ld(wqT_s[b], MF)[:, 0:MR]])
            q = _mm(wqT, _ld(xT_s, t)) * q_scale
            qc_s[2 * p, t] = q[:D].astype(BF16)
            qc_s[2 * p + 1, t] = q[D:].astype(BF16)

        def q_first(t0, t1):
            for t in range(t0, t1):
                q_tile(0, t, 0)
                rg = _mm(lhs_s[...], _ld(xT_s, t))
                r_s[:, t * _T:(t + 1) * _T] = rg[0:1, :].astype(BF16).astype(F32)
                g_s[:, t * _T:(t + 1) * _T] = _sigmoid(rg[1:2, :])

        def run_pre():
            start(q_cp(0) + group('xa') + group('xb') + group('xc'))
            pl.loop(1, NP)(lambda p: start(q_cp(p)))
            start(group('ffn') + group('c'))
            pl.loop(0, NP)(lambda p: start(kv_cp(p)))
            start(group('wo'))
            for b in range(2):
                wqT_s[b][MF] = jnp.zeros((2 * D, _T), BF16)
            idx_s[2] = 0
            wait(q_cp(0))
            prep_q(0, 0)
            wait(group('xa'))
            row = lax.broadcasted_iota(I32, (16, M), 0)
            wr = wr_s[...].astype(F32).reshape(1, M)
            gw = gw_s[...].astype(F32).reshape(1, M)
            lhs_s[...] = jnp.where(row == 0, wr, jnp.where(row == 1, gw, 0.0)).astype(BF16)
            q_first(0, _XA)
            wait(group('xb'))
            q_first(_XA, _XB)
            wait(group('xc') + q_cp(1))
            prep_q(1, 1)
            q_first(_XB, NS_T)
            wait(q_cp(2) + q_cp(3))

            def phase_q(i, carry):
                p = 2 * i + 1
                prep_q(p + 1, 0)
                for t in range(NS_T):
                    q_tile(p, t, 1)
                prep_q(p + 2, 1)
                for t in range(NS_T):
                    q_tile(p + 1, t, 0)
                pl.when(p + 4 < NP)(lambda: wait(q_cp(p + 3) + q_cp(p + 4)))
                return carry

            lax.fori_loop(0, (NP - 2) // 2, phase_q, 0)
            wait(group('ffn'))

            lane = lax.broadcasted_iota(I32, (1, S), 1)
            idxs, cur = [], r_s[...]
            for n in range(2):
                mx = jnp.max(cur, axis=1, keepdims=True)
                ii = jnp.min(jnp.where(cur == mx, lane, S - 1))
                idxs.append(ii)
                idx_s[n] = ii
                cur = jnp.where(lane == ii, -jnp.inf, cur)
            ffn = {}

            def ffn_select():
                row16 = lax.broadcasted_iota(I32, (16, _T), 0)
                lane16 = lax.broadcasted_iota(I32, (16, _T), 1)
                xs = None
                for n, ii in enumerate(idxs):
                    oh = jnp.logical_and(row16 == n, lane16 == (ii & (_T - 1)))
                    xr = _mm_nt(jnp.where(oh, 1.0, 0.0).astype(BF16), _ld(xT_s, ii // _T))
                    xs = xr if xs is None else xs + xr
                ffn['x'] = xs.astype(BF16)

            def ffn_hidden(f):
                gt = _mm(ffn['x'], wg_s[:, f * _T:(f + 1) * _T])
                up = _mm(ffn['x'], wu_s[:, f * _T:(f + 1) * _T])
                ffn[f] = (gt * _sigmoid(gt) * up).astype(BF16)

            def ffn_down(f):
                y = _mm_nt(ffn[f], wdT_s[:, f * _T:(f + 1) * _T])
                ffn['y'] = y if 'y' not in ffn else ffn['y'] + y

            after = {3: [ffn_select]}
            for f in range(NF_T):
                after.setdefault(5 + f // 2, []).append(lambda f=f: ffn_hidden(f))
            for f in range(NF_T):
                after.setdefault(6 + f // 2, []).insert(0, lambda f=f: ffn_down(f))
            for t in range(NS_T):
                q_tile(NP - 1, t, 1)
                for fn in after.get(t, []):
                    fn()
            yp = jnp.concatenate([ffn['y'], jnp.zeros((16, (MF + 1) * _T - M), F32)], axis=1)
            yT = jnp.concatenate([yp, jnp.zeros((_T - 16, (MF + 1) * _T), F32)], axis=0).T[:M]
            for n in range(2):
                y_s[n] = jnp.broadcast_to(yT[:, n:n + 1], (M, _T))

            zero = idx_s[2]
            for ref in s_s:
                ref[zero, 0:8, :] = jnp.zeros((8, _B), F32)
            q_s[zero, 0:8, :] = jnp.zeros((8, _T), U32)
            wait(group('c'))
            pl.loop(0, NP)(lambda p: wait(kv_cp(p)))

        def head(h, carry):
            slot = h >> 1
            sh = ((1 - (h & 1)) * 16).astype(U32)
            wk = _as_f32((wk_buf[slot] << sh) & jnp.uint32(_HI))
            for t in range(ND_T):
                wk_s[t] = wk[:, t * _T:(t + 1) * _T].astype(BF16)
            wvT = _as_f32((wv_buf[slot] << sh) & jnp.uint32(_HI)).T.astype(BF16)
            for t in range(NC_T):
                wvT_s[t] = wvT[:, t * _T:(t + 1) * _T]
            for t in range(NS_T):
                q_s[t] = qc_s.bitcast(U32)[h, t]
            tri = (lax.broadcasted_iota(I32, (_T, _T), 0) <= lax.broadcasted_iota(I32, (_T, _T), 1))

            def c_rows(r0, n):
                return _cat([_ld(c_s, t, rows=(r0, n)) for t in range(NC_T)])

            def k_rows(r0, n):
                return _cat([_ld(k_s, t, rows=(r0, n)) for t in range(ND_T)])

            def proj_k(j, t):
                w = wk[:, t * _T:(t + 1) * _T] if j == 0 else _ld(wk_s, t)
                k_s[t, j * _B:(j + 1) * _B, :] = _mm(c_rows(j * _B, _B), w).astype(BF16)

            def proj_v(j, t):
                w = wvT if (j, t) == (0, 0) else _cat([_ld(wvT_s, u) for u in range(NC_T)])
                vT_s[2 * j + t] = _mm_nt(w, c_rows(j * _B + t * _T, _T)).astype(BF16)

            done = set()

            def piece(fn, j, t):
                if j < NB and (fn, j, t) not in done:
                    done.add((fn, j, t))
                    fn(j, t)

            items = [(j, c) for j in range(NB) for c in range(j + 1)]
            state, cmax = {}, {}

            def qk(i):
                j, c = items[i]
                for t in range(2):
                    piece(proj_k, c, t)
                k0, st = c * _B, s_s[i % _NS]
                q1 = pltpu.bitcast(q_s[2 * j + 1], BF16)
                q = _cat([pltpu.bitcast(q_s[2 * j], BF16), q1])
                if c < j:
                    s = _mm(k_rows(k0, _B), q)
                    st[0] = s
                    cmax[i] = jnp.max(s, axis=0, keepdims=True)
                else:
                    s = _mm(k_rows(k0, _T), q)
                    s2 = _cat([_mm(k_rows(k0 + _T + r, _T // 2), q1) for r in (0, _T // 2)], axis=0)
                    s = _cat([jnp.where(tri, s[:, :_T], _NEG), s[:, _T:]])
                    s2 = jnp.where(tri, s2, _NEG)
                    st[0, 0:_T, :] = s
                    st[0, _T:, _T:] = s2
                    m = jnp.max(s, axis=0, keepdims=True)
                    cmax[i] = _cat([m[:, :_T], jnp.maximum(m[:, _T:], jnp.max(s2, axis=0, keepdims=True))])

            def pv(i):
                j, c = items[i]
                for t in range(2):
                    piece(proj_v, c, t)
                st, m = s_s[i % _NS], cmax.pop(i)
                if c > 0:
                    m0, l0, o0 = state[j]
                    m = jnp.maximum(m0, m)
                    alpha = jnp.exp2(m0 - m)
                if c < j:
                    p = jnp.exp2(st[0] - m)
                    l = jnp.sum(p, axis=0, keepdims=True)
                    o = _mm(_cat([_ld(vT_s, 2 * c), _ld(vT_s, 2 * c + 1)]), p.astype(BF16))
                else:
                    p = jnp.exp2(st[0, 0:_T, :] - m)
                    p2 = jnp.exp2(st[0, _T:, _T:] - m[:, _T:])
                    l = jnp.sum(p, axis=0, keepdims=True)
                    l = _cat([l[:, :_T], l[:, _T:] + jnp.sum(p2, axis=0, keepdims=True)])
                    p, p2 = p.astype(BF16), p2.astype(BF16)
                    o = _cat([_mm(_ld(vT_s, 2 * c, rows=(r, D // 2)), p)
                              for r in range(0, D, D // 2)], axis=0)
                    o2 = _cat([_mm(_ld(vT_s, 2 * c + 1, rows=(r, D // 4)), p2)
                               for r in range(0, D, D // 4)], axis=0)
                    o = _cat([o[:, :_T], o[:, _T:] + o2])
                l = jnp.where(o[0:1] != o[0:1], o[0:1], l)
                if c > 0:
                    l = l0 * alpha + l
                    o = o0 * alpha + o
                state[j] = (m, l, o)
                if c == j:
                    ctx = o * (1.0 / l)
                    for t in range(2):
                        qc_s[h, 2 * j + t] = ctx[:, t * _T:(t + 1) * _T].astype(BF16)

            for i in range(len(items) + _LAG):
                if i < len(items):
                    qk(i)
                    j, c = items[i]
                    fill = [(proj_v, j, 0), (proj_v, j, 1), (proj_k, j + 1, 0), (proj_k, j + 1, 1)]
                    if j < NB - 1:
                        for pc in fill[len(fill) * c // (j + 1):len(fill) * (c + 1) // (j + 1)]:
                            piece(*pc)
                elif (i - len(items)) % 2 == 0:
                    piece(proj_v, NB - 1, (i - len(items)) // 2)
                if i >= _LAG:
                    pv(i - _LAG)

            return carry

        def run_heads():
            lax.fori_loop(0, H, head, 0)
            wait(group('wo'))

        def phase_o(j, carry):
            pl.when(j >= 2)(lambda: wait(o_cp(j - 2)))
            c0 = pl.multiple_of(j * _B, _B)
            a = None
            for hh in range(0, H, 2):
                w2 = _cat([_ld(woT_s, t, hh + u) for u in range(2) for t in range(ND_T)])
                x2 = _cat([_cat([_ld(qc_s, hh + u, 2 * j), _ld(qc_s, hh + u, 2 * j + 1)])
                           for u in range(2)], axis=0)
                part = _mm(w2, x2)
                a = part if a is None else a + part
            g = g_s[:, pl.ds(c0, _B)]
            rs = _sigmoid(r_s[:, pl.ds(c0, _B)])
            col = lax.broadcasted_iota(I32, (1, _B), 1) + j * _B
            b = _cat([xT_s[2 * j], xT_s[2 * j + 1]]).astype(F32)
            for n in range(2):
                b = b + _cat([y_s[n], y_s[n]]) * jnp.where(col == idx_s[n], rs, 0.0)
            o_s[j & 1] = (g * a + (1.0 - g) * b).astype(BF16)
            start(o_cp(j))
            return carry

        def run_o():
            lax.fori_loop(0, NB, phase_o, 0)

        def stage(k, carry):
            for i, fn in enumerate((run_pre, run_heads, run_o)):
                pl.when(k == i)(fn)
            return carry

        lax.fori_loop(0, 3, stage, 0)
        wait(o_cp(NB - 2) + o_cp(NB - 1))

    return kernel


@jax.jit
def pallas_gated_mix__compressed_kv_cla__moe_arch_mod__prompt_kernel(
    A_x: jax.Array,
    A_c_kv: jax.Array,
    A_w_q: jax.Array,
    A_w_uk: jax.Array,
    A_w_uv: jax.Array,
    A_w_o: jax.Array,
    B_x: jax.Array,
    B_w_r: jax.Array,
    B_w_gate: jax.Array,
    B_w_up: jax.Array,
    B_w_down: jax.Array,
    gate_w: jax.Array,
):
    _, S, M = A_x.shape
    C = A_c_kv.shape[2]
    H, D = A_w_q.shape[1], A_w_q.shape[2]
    FF = B_w_gate.shape[1]
    xT = A_x[0].T
    woT = jnp.transpose(A_w_o, (0, 2, 1))
    wdT = B_w_down.T
    any_spec = pl.BlockSpec(memory_space=pl.ANY)
    V = pltpu.VMEM
    outT = pl.pallas_call(
        _make_kernel(S, M, C, H, D, FF),
        in_specs=[any_spec] * 11,
        out_specs=any_spec,
        out_shape=jax.ShapeDtypeStruct((M, S), BF16),
        scratch_shapes=[
            V((S // _T, M, _T), BF16), V((C // _T, S, _T), BF16),
            V((H // 2, M, D), U32), V((H // 2, C, D), U32), V((H // 2, C, D), U32),
            V((D // _T, H, M, _T), BF16), V((M,), BF16), V((M,), BF16),
            V((M, FF), BF16), V((M, FF), BF16), V((M, FF), BF16),
            [V((pl.cdiv(M, _T), 2 * D, _T), BF16)] * 2, V((D // _T, C, _T), BF16),
            V((C // _T, D, _T), BF16), V((16, M), BF16),
            V((H, S // _T, D, _T), BF16), V((S // _T, D // 2, _T), U32),
            V((D // _T, S, _T), BF16), V((S // _T, D, _T), BF16),
            V((1, S), F32), V((1, S), F32), V((2, M, _T), F32), V((2, M, _B), BF16),
            [V((1, _B, _B), F32)] * _NS,
            pltpu.SMEM((3,), I32),
            pltpu.SemaphoreType.DMA((6,)), pltpu.SemaphoreType.DMA((H // 2,)),
            pltpu.SemaphoreType.DMA(()), pltpu.SemaphoreType.DMA((2,)),
        ],
        compiler_params=pltpu.CompilerParams(vmem_limit_bytes=100 << 20),
    )(xT, A_c_kv[0], A_w_q, A_w_uk, A_w_uv, woT, B_w_r, gate_w, B_w_gate, B_w_up, wdT)
    return outT.T[None]
```

```python
import math

import jax
import jax.numpy as jnp
from jax import lax
import jax.experimental.pallas as pl
import jax.experimental.pallas.tpu as pltpu

F32, BF16, U32, I32 = jnp.float32, jnp.bfloat16, jnp.uint32, jnp.int32
_NT = (((1,), (1,)), ((), ()))
_NEG = -1e30
_HI = 0xFFFF0000
_T = 128
_B = 256
_LAG = 4
_NS = 6
_G = 64
_XA, _XB = 2, 7


def _mm(a, b):
    return jnp.dot(a, b, preferred_element_type=F32)


def _mm_nt(a, b):
    return lax.dot_general(a, b, _NT, preferred_element_type=F32)


def _sigmoid(x):
    return 1.0 / (1.0 + jnp.exp(-x))


def _as_f32(u):
    return lax.bitcast_convert_type(u, F32)


def _cat(parts, axis=1):
    return parts[0] if len(parts) == 1 else jnp.concatenate(parts, axis=axis)


def _colmax(x):
    return jnp.max(x, axis=0, keepdims=True)


def _ld(ref, *lead, rows=None):
    u = ref.bitcast(U32)
    idx = lead if rows is None else lead + (slice(rows[0] // 2, (rows[0] + rows[1]) // 2),)
    return pltpu.bitcast(u[idx], BF16)


def _make_kernel(S, M, C, H, D, FF):
    NB, NP = S // _B, H // 2
    NS_T, NC_T, ND_T, NF_T = S // _T, C // _T, D // _T, FF // _T
    MF, MR = M // _T, M % _T
    assert ND_T == 2 and MR > 0 and _NS > _LAG
    q_scale = math.log2(math.e) * (D ** -0.5)

    def kernel(xT_hbm, c_hbm, wq_hbm, wk_hbm, wv_hbm, woT_hbm, wr_hbm, gw_hbm,
               wg_hbm, wu_hbm, wdT_hbm, o_hbm,
               xT_s, c_s, wq_buf, wk_buf, wv_buf, woT_s, wr_s, gw_s, wg_s, wu_s, wdT_s,
               wqT_s, wk_s, wvT_s, lhs_s, qc_s, q_s, k_s, vT_s, g_s, r_s, y_s, o_s, s_s, z_s, side_s, qn_s, idx_s,
               sem, q_sem, kv_sem, o_sem):
        def tiled(src, dst, n):
            return [(src.at[..., t * _T:(t + 1) * _T], dst.at[t]) for t in range(n)]

        xt = tiled(xT_hbm, xT_s, NS_T)
        groups = dict(xa=[(wr_hbm, wr_s), (gw_hbm, gw_s)] + xt[:_XA], xb=xt[_XA:_XB], xc=xt[_XB:],
                      ffn=[(wg_hbm, wg_s), (wu_hbm, wu_s), (wdT_hbm, wdT_s)],
                      c=tiled(c_hbm, c_s, NC_T), wo=tiled(woT_hbm, woT_s, ND_T))

        def group(name):
            s = sem.at[list(groups).index(name)]
            return [pltpu.make_async_copy(src, dst, s) for src, dst in groups[name]]

        def q_cp(p):
            return [pltpu.make_async_copy(wq_hbm.bitcast(U32).at[:, p, :], wq_buf.at[p], q_sem.at[p])]

        def kv_cp(p):
            return [pltpu.make_async_copy(src.bitcast(U32).at[:, p, :], dst.at[p], kv_sem)
                    for src, dst in ((wk_hbm, wk_buf), (wv_hbm, wv_buf))]

        def o_cp(j):
            c0 = pl.multiple_of(j * _B, _B)
            return [pltpu.make_async_copy(o_s.at[j & 1], o_hbm.at[:, pl.ds(c0, _B)], o_sem.at[j & 1])]

        def start(cps):
            for d in cps:
                d.start()

        def wait(cps):
            for d in cps:
                d.wait()

        def prep_q(p, b):
            w = wq_buf[p].T
            for half, u in enumerate((w << 16, w & jnp.uint32(_HI))):
                wb = _as_f32(u)
                for t in range(MF):
                    wqT_s[b][t, half * D:(half + 1) * D, :] = wb[:, t * _T:(t + 1) * _T].astype(BF16)
                wqT_s[b][MF, half * D:(half + 1) * D, 0:MR] = wb[:, MF * _T:].astype(BF16)

        def q_tile(p, t, b):
            wqT = _cat([_ld(wqT_s[b], u) for u in range(MF)] + [_ld(wqT_s[b], MF)[:, 0:MR]])
            q = _mm(wqT, _ld(xT_s, t)) * q_scale
            qc_s[2 * p, t] = q[:D].astype(BF16)
            qc_s[2 * p + 1, t] = q[D:].astype(BF16)

        def q_first(t0, t1):
            for t in range(t0, t1):
                q_tile(0, t, 0)
                rg = _mm(lhs_s[...], _ld(xT_s, t))
                r_s[:, t * _T:(t + 1) * _T] = rg[0:1, :].astype(BF16).astype(F32)
                g_s[:, t * _T:(t + 1) * _T] = _sigmoid(rg[1:2, :])

        def run_pre():
            start(q_cp(0) + group('xa') + group('xb') + group('xc'))
            pl.loop(1, NP)(lambda p: start(q_cp(p)))
            start(group('ffn') + group('c'))
            pl.loop(0, NP)(lambda p: start(kv_cp(p)))
            start(group('wo'))
            for b in range(2):
                wqT_s[b][MF] = jnp.zeros((2 * D, _T), BF16)
            idx_s[2] = 0
            wait(q_cp(0))
            prep_q(0, 0)
            wait(group('xa'))
            row = lax.broadcasted_iota(I32, (16, M), 0)
            wr = wr_s[...].astype(F32).reshape(1, M)
            gw = gw_s[...].astype(F32).reshape(1, M)
            lhs_s[...] = jnp.where(row == 0, wr, jnp.where(row == 1, gw, 0.0)).astype(BF16)
            q_first(0, _XA)
            wait(group('xb'))
            q_first(_XA, _XB)
            wait(group('xc') + q_cp(1))
            prep_q(1, 1)
            q_first(_XB, NS_T)
            wait(q_cp(2) + q_cp(3))

            def phase_q(i, carry):
                p = 2 * i + 1
                prep_q(p + 1, 0)
                for t in range(NS_T):
                    q_tile(p, t, 1)
                prep_q(p + 2, 1)
                for t in range(NS_T):
                    q_tile(p + 1, t, 0)
                pl.when(p + 4 < NP)(lambda: wait(q_cp(p + 3) + q_cp(p + 4)))
                return carry

            lax.fori_loop(0, (NP - 2) // 2, phase_q, 0)
            wait(group('ffn'))

            lane = lax.broadcasted_iota(I32, (1, S), 1)
            idxs, cur = [], r_s[...]
            for n in range(2):
                mx = jnp.max(cur, axis=1, keepdims=True)
                ii = jnp.min(jnp.where(cur == mx, lane, S - 1))
                idxs.append(ii)
                idx_s[n] = ii
                cur = jnp.where(lane == ii, -jnp.inf, cur)
            ffn = {}

            def ffn_select():
                row16 = lax.broadcasted_iota(I32, (16, _T), 0)
                lane16 = lax.broadcasted_iota(I32, (16, _T), 1)
                xs = None
                for n, ii in enumerate(idxs):
                    oh = jnp.logical_and(row16 == n, lane16 == (ii & (_T - 1)))
                    xr = _mm_nt(jnp.where(oh, 1.0, 0.0).astype(BF16), _ld(xT_s, ii // _T))
                    xs = xr if xs is None else xs + xr
                ffn['x'] = xs.astype(BF16)

            def ffn_hidden(f):
                gt = _mm(ffn['x'], wg_s[:, f * _T:(f + 1) * _T])
                up = _mm(ffn['x'], wu_s[:, f * _T:(f + 1) * _T])
                ffn[f] = (gt * _sigmoid(gt) * up).astype(BF16)

            def ffn_down(f):
                y = _mm_nt(ffn[f], wdT_s[:, f * _T:(f + 1) * _T])
                ffn['y'] = y if 'y' not in ffn else ffn['y'] + y

            after = {3: [ffn_select]}
            for f in range(NF_T):
                after.setdefault(5 + f // 2, []).append(lambda f=f: ffn_hidden(f))
            for f in range(NF_T):
                after.setdefault(6 + f // 2, []).insert(0, lambda f=f: ffn_down(f))
            for t in range(NS_T):
                q_tile(NP - 1, t, 1)
                for fn in after.get(t, []):
                    fn()
            yp = jnp.concatenate([ffn['y'], jnp.zeros((16, (MF + 1) * _T - M), F32)], axis=1)
            yT = jnp.concatenate([yp, jnp.zeros((_T - 16, (MF + 1) * _T), F32)], axis=0).T[:M]
            for n in range(2):
                y_s[n] = jnp.broadcast_to(yT[:, n:n + 1], (M, _T))

            zero = idx_s[2]
            for ref in s_s:
                ref[zero, 0:8, :] = jnp.zeros((8, _B), F32)
            q_s[zero, 0:8, :] = jnp.zeros((8, _T), U32)
            z_s[...] = jnp.zeros(z_s.shape, F32)
            z_s[zero, 0:8, :] = jnp.zeros((8, _T), F32)
            side_s[zero, 0:8, :] = jnp.zeros((8, _T), F32)
            wait(group('c'))
            pl.loop(0, NP)(lambda p: wait(kv_cp(p)))

        def head(h, carry):
            slot = h >> 1
            sh = ((1 - (h & 1)) * 16).astype(U32)
            wk = _as_f32((wk_buf[slot] << sh) & jnp.uint32(_HI))
            for t in range(ND_T):
                wk_s[t] = wk[:, t * _T:(t + 1) * _T].astype(BF16)
            wvT = _as_f32((wv_buf[slot] << sh) & jnp.uint32(_HI)).T.astype(BF16)
            for t in range(NC_T):
                wvT_s[t] = wvT[:, t * _T:(t + 1) * _T]
            for t in range(NS_T):
                q_s[t] = qc_s.bitcast(U32)[h, t]
            tri = (lax.broadcasted_iota(I32, (_T, _T), 0) <= lax.broadcasted_iota(I32, (_T, _T), 1))
            left = lax.broadcasted_iota(I32, (_T, _T), 1) < _G
            r64 = lax.broadcasted_iota(I32, (_G, _T), 0)
            l64 = lax.broadcasted_iota(I32, (_G, _T), 1)
            left_h, tri_u, tri_l = l64 < _G, r64 <= l64, r64 + _G <= l64
            qn = _ld(qc_s, h, NS_T - 1).astype(F32).T[_G:]
            for t in range(ND_T):
                qn_s[t] = qn[:, t * _T:(t + 1) * _T].astype(BF16)

            def c_rows(r0, n):
                return _cat([_ld(c_s, t, rows=(r0, n)) for t in range(NC_T)])

            def k_rows(r0, n):
                return _cat([_ld(k_s, t, rows=(r0, n)) for t in range(ND_T)])

            def proj_k(j, t):
                w = wk[:, t * _T:(t + 1) * _T] if j == 0 else _ld(wk_s, t)
                k_s[t, j * _B:(j + 1) * _B, :] = _mm(c_rows(j * _B, _B), w).astype(BF16)

            def proj_v(j, t):
                w = wvT if (j, t) == (0, 0) else _cat([_ld(wvT_s, u) for u in range(NC_T)])
                vT_s[2 * j + t] = _mm_nt(w, c_rows(j * _B + t * _T, _T)).astype(BF16)

            done = set()

            def piece(fn, j, t):
                if j < NB and (fn, j, t) not in done:
                    done.add((fn, j, t))
                    fn(j, t)

            items = [(j, c) for j in range(NB) for c in range(j + 1)]
            state, cmax = {}, {}

            def qk(i):
                j, c = items[i]
                for t in range(2):
                    piece(proj_k, c, t)
                k0, st, G = c * _B, s_s[i % _NS], _G
                q0u, q1u = q_s[2 * j], q_s[2 * j + 1]
                q0, q1 = pltpu.bitcast(q0u, BF16), pltpu.bitcast(q1u, BF16)
                q = _cat([q0, q1])

                def shared(qu):
                    return pltpu.bitcast(jnp.where(left, q_s[NS_T - 1], qu), BF16)

                if j == NB - 1:
                    k_odd = _cat([k_rows(k0 + G, G), k_rows(k0 + 3 * G, G)], axis=0)
                    qn = _cat([_ld(qn_s, t) for t in range(ND_T)])
                if c < j < NB - 1:
                    s = _mm(k_rows(k0, _B), q)
                    st[0] = s
                    cmax[i] = _colmax(s)
                elif c < j:
                    n1 = _B - G // 2
                    sa = _mm(k_rows(k0, n1), q0)
                    z_s[c, G:, :] = _mm_nt(qn, k_odd)
                    sb = _mm(k_rows(k0 + n1, _B - n1), q0)
                    su = _mm(_cat([k_rows(k0, G), k_rows(k0 + 2 * G, G)], axis=0), q1)
                    s0 = _cat([sa, sb], axis=0)
                    st[0, :, 0:_T] = s0
                    st[0, 0:G, _T:] = su[:G]
                    st[0, 2 * G:3 * G, _T:] = su[G:]
                    cmax[i] = _cat([_colmax(s0), _colmax(su)])
                elif j < NB - 1:
                    s_ua = _mm(k_rows(k0, G), q)
                    s_la = _mm(k_rows(k0 + G, G), _cat([shared(q0u), q1]))
                    s_ub = _mm(k_rows(k0 + 2 * G, G), q1)
                    s_lb = _mm(k_rows(k0 + 3 * G, G), shared(q1u))
                    side_s[2 * j] = s_la[:, :_T]
                    side_s[2 * j + 1] = s_lb
                    s = _cat([s_ua, s_la], axis=0)
                    s = _cat([jnp.where(tri, s[:, :_T], _NEG), s[:, _T:]])
                    s2 = jnp.where(tri, _cat([s_ub, s_lb], axis=0), _NEG)
                    st[0, 0:_T, :] = s
                    st[0, _T:, _T:] = s2
                    m = _colmax(s)
                    cmax[i] = _cat([m[:, :_T], jnp.maximum(m[:, _T:], _colmax(s2))])
                else:
                    z_s[c, G:, :] = _cat([_mm_nt(qn[r:r + G // 2], k_odd) for r in (0, G // 2)], axis=0)
                    s_ua = _mm(k_rows(k0, G), q)
                    s_la = _mm(k_rows(k0 + G, G), shared(q0u))
                    s_ub = _mm(k_rows(k0 + 2 * G, G), q1)
                    side_s[2 * j] = s_la
                    s0 = jnp.where(tri, _cat([s_ua[:, :_T], s_la], axis=0), _NEG)
                    s_ub = jnp.where(tri_u, s_ub, _NEG)
                    st[0, 0:_T, 0:_T] = s0
                    st[0, 0:G, _T:] = s_ua[:, _T:]
                    st[0, 2 * G:3 * G, _T:] = s_ub
                    cmax[i] = _cat([_colmax(s0), jnp.maximum(_colmax(s_ua[:, _T:]), _colmax(s_ub))])

            def pv(i):
                j, c = items[i]
                for t in range(2):
                    piece(proj_v, c, t)
                st, m, G = s_s[i % _NS], cmax.pop(i), _G
                if j == NB - 1:
                    zt = z_s[c].T
                    la = jnp.where(left_h, side_s[2 * c], zt[:G])
                    if c < j:
                        lb = jnp.where(left_h, side_s[2 * c + 1], zt[G:])
                    else:
                        lb = jnp.where(tri_l, zt[G:], _NEG)
                    st[0, G:2 * G, _T:] = la
                    st[0, 3 * G:, _T:] = lb
                    m = _cat([m[:, :_T], jnp.maximum(m[:, _T:], jnp.maximum(_colmax(la), _colmax(lb)))])
                if c > 0:
                    m0, l0, o0 = state[j]
                    m = jnp.maximum(m0, m)
                    alpha = jnp.exp2(m0 - m)
                if c < j:
                    p = jnp.exp2(st[0] - m)
                    l = jnp.sum(p, axis=0, keepdims=True)
                    o = _mm(_cat([_ld(vT_s, 2 * c), _ld(vT_s, 2 * c + 1)]), p.astype(BF16))
                else:
                    p = jnp.exp2(st[0, 0:_T, :] - m)
                    p2 = jnp.exp2(st[0, _T:, _T:] - m[:, _T:])
                    l = jnp.sum(p, axis=0, keepdims=True)
                    l = _cat([l[:, :_T], l[:, _T:] + jnp.sum(p2, axis=0, keepdims=True)])
                    p, p2 = p.astype(BF16), p2.astype(BF16)
                    o = _cat([_mm(_ld(vT_s, 2 * c, rows=(r, D // 2)), p)
                              for r in range(0, D, D // 2)], axis=0)
                    o2 = _cat([_mm(_ld(vT_s, 2 * c + 1, rows=(r, D // 4)), p2)
                               for r in range(0, D, D // 4)], axis=0)
                    o = _cat([o[:, :_T], o[:, _T:] + o2])
                l = jnp.where(o[0:1] != o[0:1], o[0:1], l)
                if c > 0:
                    l = l0 * alpha + l
                    o = o0 * alpha + o
                state[j] = (m, l, o)
                if c == j:
                    ctx = o * (1.0 / l)
                    for t in range(2):
                        qc_s[h, 2 * j + t] = ctx[:, t * _T:(t + 1) * _T].astype(BF16)

            for i in range(len(items) + _LAG):
                if i < len(items):
                    qk(i)
                    j, c = items[i]
                    fill = [(proj_v, j, 0), (proj_v, j, 1), (proj_k, j + 1, 0), (proj_k, j + 1, 1)]
                    if j < NB - 1:
                        for pc in fill[len(fill) * c // (j + 1):len(fill) * (c + 1) // (j + 1)]:
                            piece(*pc)
                elif (i - len(items)) % 2 == 0:
                    piece(proj_v, NB - 1, (i - len(items)) // 2)
                if i >= _LAG:
                    pv(i - _LAG)

            return carry

        def run_heads():
            lax.fori_loop(0, H, head, 0)
            wait(group('wo'))

        def phase_o(j, carry):
            pl.when(j >= 2)(lambda: wait(o_cp(j - 2)))
            c0 = pl.multiple_of(j * _B, _B)
            a = None
            for hh in range(0, H, 2):
                w2 = _cat([_ld(woT_s, t, hh + u) for u in range(2) for t in range(ND_T)])
                x2 = _cat([_cat([_ld(qc_s, hh + u, 2 * j), _ld(qc_s, hh + u, 2 * j + 1)])
                           for u in range(2)], axis=0)
                part = _mm(w2, x2)
                a = part if a is None else a + part
            g = g_s[:, pl.ds(c0, _B)]
            rs = _sigmoid(r_s[:, pl.ds(c0, _B)])
            col = lax.broadcasted_iota(I32, (1, _B), 1) + j * _B
            b = _cat([xT_s[2 * j], xT_s[2 * j + 1]]).astype(F32)
            for n in range(2):
                b = b + _cat([y_s[n], y_s[n]]) * jnp.where(col == idx_s[n], rs, 0.0)
            o_s[j & 1] = (g * a + (1.0 - g) * b).astype(BF16)
            start(o_cp(j))
            return carry

        def run_o():
            lax.fori_loop(0, NB, phase_o, 0)

        def stage(k, carry):
            for i, fn in enumerate((run_pre, run_heads, run_o)):
                pl.when(k == i)(fn)
            return carry

        lax.fori_loop(0, 3, stage, 0)
        wait(o_cp(NB - 2) + o_cp(NB - 1))

    return kernel


@jax.jit
def pallas_gated_mix__compressed_kv_cla__moe_arch_mod__prompt_kernel(
    A_x: jax.Array,
    A_c_kv: jax.Array,
    A_w_q: jax.Array,
    A_w_uk: jax.Array,
    A_w_uv: jax.Array,
    A_w_o: jax.Array,
    B_x: jax.Array,
    B_w_r: jax.Array,
    B_w_gate: jax.Array,
    B_w_up: jax.Array,
    B_w_down: jax.Array,
    gate_w: jax.Array,
):
    _, S, M = A_x.shape
    C = A_c_kv.shape[2]
    H, D = A_w_q.shape[1], A_w_q.shape[2]
    FF = B_w_gate.shape[1]
    xT = A_x[0].T
    woT = jnp.transpose(A_w_o, (0, 2, 1))
    wdT = B_w_down.T
    any_spec = pl.BlockSpec(memory_space=pl.ANY)
    V = pltpu.VMEM
    outT = pl.pallas_call(
        _make_kernel(S, M, C, H, D, FF),
        in_specs=[any_spec] * 11,
        out_specs=any_spec,
        out_shape=jax.ShapeDtypeStruct((M, S), BF16),
        scratch_shapes=[
            V((S // _T, M, _T), BF16), V((C // _T, S, _T), BF16),
            V((H // 2, M, D), U32), V((H // 2, C, D), U32), V((H // 2, C, D), U32),
            V((D // _T, H, M, _T), BF16), V((M,), BF16), V((M,), BF16),
            V((M, FF), BF16), V((M, FF), BF16), V((M, FF), BF16),
            [V((pl.cdiv(M, _T), 2 * D, _T), BF16)] * 2, V((D // _T, C, _T), BF16),
            V((C // _T, D, _T), BF16), V((16, M), BF16),
            V((H, S // _T, D, _T), BF16), V((S // _T, D // 2, _T), U32),
            V((D // _T, S, _T), BF16), V((S // _T, D, _T), BF16),
            V((1, S), F32), V((1, S), F32), V((2, M, _T), F32), V((2, M, _B), BF16),
            [V((1, _B, _B), F32)] * _NS,
            V((S // _B, _T, _T), F32), V((S // _T, _G, _T), F32), V((D // _T, _G, _T), BF16),
            pltpu.SMEM((3,), I32),
            pltpu.SemaphoreType.DMA((6,)), pltpu.SemaphoreType.DMA((H // 2,)),
            pltpu.SemaphoreType.DMA(()), pltpu.SemaphoreType.DMA((2,)),
        ],
        compiler_params=pltpu.CompilerParams(vmem_limit_bytes=100 << 20),
    )(xT, A_c_kv[0], A_w_q, A_w_uk, A_w_uv, woT, B_w_r, gate_w, B_w_gate, B_w_up, wdT)
    return outT.T[None]
```

```python
import math

import jax
import jax.numpy as jnp
from jax import lax
import jax.experimental.pallas as pl
import jax.experimental.pallas.tpu as pltpu

F32, BF16, U32, I32 = jnp.float32, jnp.bfloat16, jnp.uint32, jnp.int32
_NT = (((1,), (1,)), ((), ()))
_NEG = -1e30
_HI = 0xFFFF0000
_T = 128
_B = 256
_LAG = 4
_NS = 6
_NG = 4
_G = _T // _NG
_XA, _XB = 2, 7


def _mm(a, b):
    return jnp.dot(a, b, preferred_element_type=F32)


def _mm_nt(a, b):
    return lax.dot_general(a, b, _NT, preferred_element_type=F32)


def _sigmoid(x):
    return 1.0 / (1.0 + jnp.exp(-x))


def _as_f32(u):
    return lax.bitcast_convert_type(u, F32)


def _cat(parts, axis=1):
    return parts[0] if len(parts) == 1 else jnp.concatenate(parts, axis=axis)


def _colmax(x):
    return jnp.max(x, axis=0, keepdims=True)


def _ld(ref, *lead, rows=None):
    u = ref.bitcast(U32)
    idx = lead if rows is None else lead + (slice(rows[0] // 2, (rows[0] + rows[1]) // 2),)
    return pltpu.bitcast(u[idx], BF16)


def _make_kernel(S, M, C, H, D, FF):
    NB, NP = S // _B, H // 2
    NS_T, NC_T, ND_T, NF_T = S // _T, C // _T, D // _T, FF // _T
    MF, MR = M // _T, M % _T
    assert ND_T == 2 and MR > 0 and _NS > _LAG >= 1 and _NG == 4 and NB % 2 == 0
    q_scale = math.log2(math.e) * (D ** -0.5)

    def kernel(xT_hbm, c_hbm, wq_hbm, wk_hbm, wv_hbm, woT_hbm, wr_hbm, gw_hbm,
               wg_hbm, wu_hbm, wdT_hbm, o_hbm,
               xT_s, c_s, wq_buf, wk_buf, wv_buf, woT_s, wr_s, gw_s, wg_s, wu_s, wdT_s,
               wqT_s, wk_s, wvT_s, lhs_s, qc_s, q_s, k_s, vT_s, g_s, r_s, y_s, o_s, s_s, z_s, zt_s, side_s, qn_s, idx_s,
               sem, q_sem, kv_sem, o_sem):
        def tiled(src, dst, n):
            return [(src.at[..., t * _T:(t + 1) * _T], dst.at[t]) for t in range(n)]

        xt = tiled(xT_hbm, xT_s, NS_T)
        groups = dict(xa=[(wr_hbm, wr_s), (gw_hbm, gw_s)] + xt[:_XA], xb=xt[_XA:_XB], xc=xt[_XB:],
                      ffn=[(wg_hbm, wg_s), (wu_hbm, wu_s), (wdT_hbm, wdT_s)],
                      c=tiled(c_hbm, c_s, NC_T), wo=tiled(woT_hbm, woT_s, ND_T))

        def group(name):
            s = sem.at[list(groups).index(name)]
            return [pltpu.make_async_copy(src, dst, s) for src, dst in groups[name]]

        def q_cp(p):
            return [pltpu.make_async_copy(wq_hbm.bitcast(U32).at[:, p, :], wq_buf.at[p], q_sem.at[p])]

        def kv_cp(p):
            return [pltpu.make_async_copy(src.bitcast(U32).at[:, p, :], dst.at[p], kv_sem)
                    for src, dst in ((wk_hbm, wk_buf), (wv_hbm, wv_buf))]

        def o_cp(j):
            c0 = pl.multiple_of(j * _B, _B)
            return [pltpu.make_async_copy(o_s.at[j & 1], o_hbm.at[:, pl.ds(c0, _B)], o_sem.at[j & 1])]

        def start(cps):
            for d in cps:
                d.start()

        def wait(cps):
            for d in cps:
                d.wait()

        def prep_q(p, b):
            w = wq_buf[p].T
            for half, u in enumerate((w << 16, w & jnp.uint32(_HI))):
                wb = _as_f32(u)
                for t in range(MF):
                    wqT_s[b][t, half * D:(half + 1) * D, :] = wb[:, t * _T:(t + 1) * _T].astype(BF16)
                wqT_s[b][MF, half * D:(half + 1) * D, 0:MR] = wb[:, MF * _T:].astype(BF16)

        def q_tile(p, t, b):
            wqT = _cat([_ld(wqT_s[b], u) for u in range(MF)] + [_ld(wqT_s[b], MF)[:, 0:MR]])
            q = _mm(wqT, _ld(xT_s, t)) * q_scale
            qc_s[2 * p, t] = q[:D].astype(BF16)
            qc_s[2 * p + 1, t] = q[D:].astype(BF16)

        def q_first(t0, t1):
            for t in range(t0, t1):
                q_tile(0, t, 0)
                rg = _mm(lhs_s[...], _ld(xT_s, t))
                r_s[:, t * _T:(t + 1) * _T] = rg[0:1, :].astype(BF16).astype(F32)
                g_s[:, t * _T:(t + 1) * _T] = _sigmoid(rg[1:2, :])

        def run_pre():
            start(q_cp(0) + group('xa') + group('xb') + group('xc'))
            pl.loop(1, NP)(lambda p: start(q_cp(p)))
            start(group('ffn') + group('c'))
            pl.loop(0, NP)(lambda p: start(kv_cp(p)))
            start(group('wo'))
            for b in range(2):
                wqT_s[b][MF] = jnp.zeros((2 * D, _T), BF16)
            idx_s[2] = 0
            wait(q_cp(0))
            prep_q(0, 0)
            wait(group('xa'))
            row = lax.broadcasted_iota(I32, (16, M), 0)
            wr = wr_s[...].astype(F32).reshape(1, M)
            gw = gw_s[...].astype(F32).reshape(1, M)
            lhs_s[...] = jnp.where(row == 0, wr, jnp.where(row == 1, gw, 0.0)).astype(BF16)
            q_first(0, _XA)
            wait(group('xb'))
            q_first(_XA, _XB)
            wait(group('xc') + q_cp(1))
            prep_q(1, 1)
            q_first(_XB, NS_T)
            wait(q_cp(2) + q_cp(3))

            def phase_q(i, carry):
                p = 2 * i + 1
                prep_q(p + 1, 0)
                for t in range(NS_T):
                    q_tile(p, t, 1)
                prep_q(p + 2, 1)
                for t in range(NS_T):
                    q_tile(p + 1, t, 0)
                pl.when(p + 4 < NP)(lambda: wait(q_cp(p + 3) + q_cp(p + 4)))
                return carry

            lax.fori_loop(0, (NP - 2) // 2, phase_q, 0)
            wait(group('ffn'))

            lane = lax.broadcasted_iota(I32, (1, S), 1)
            idxs, cur = [], r_s[...]
            for n in range(2):
                mx = jnp.max(cur, axis=1, keepdims=True)
                ii = jnp.min(jnp.where(cur == mx, lane, S - 1))
                idxs.append(ii)
                idx_s[n] = ii
                cur = jnp.where(lane == ii, -jnp.inf, cur)
            ffn = {}

            def ffn_select():
                row16 = lax.broadcasted_iota(I32, (16, _T), 0)
                lane16 = lax.broadcasted_iota(I32, (16, _T), 1)
                xs = None
                for n, ii in enumerate(idxs):
                    oh = jnp.logical_and(row16 == n, lane16 == (ii & (_T - 1)))
                    xr = _mm_nt(jnp.where(oh, 1.0, 0.0).astype(BF16), _ld(xT_s, ii // _T))
                    xs = xr if xs is None else xs + xr
                ffn['x'] = xs.astype(BF16)

            def ffn_hidden(f):
                gt = _mm(ffn['x'], wg_s[:, f * _T:(f + 1) * _T])
                up = _mm(ffn['x'], wu_s[:, f * _T:(f + 1) * _T])
                ffn[f] = (gt * _sigmoid(gt) * up).astype(BF16)

            def ffn_down(f):
                y = _mm_nt(ffn[f], wdT_s[:, f * _T:(f + 1) * _T])
                ffn['y'] = y if 'y' not in ffn else ffn['y'] + y

            after = {3: [ffn_select]}
            for f in range(NF_T):
                after.setdefault(5 + f // 2, []).append(lambda f=f: ffn_hidden(f))
            for f in range(NF_T):
                after.setdefault(6 + f // 2, []).insert(0, lambda f=f: ffn_down(f))
            for t in range(NS_T):
                q_tile(NP - 1, t, 1)
                for fn in after.get(t, []):
                    fn()
            yp = jnp.concatenate([ffn['y'], jnp.zeros((16, (MF + 1) * _T - M), F32)], axis=1)
            yT = jnp.concatenate([yp, jnp.zeros((_T - 16, (MF + 1) * _T), F32)], axis=0).T[:M]
            for n in range(2):
                y_s[n] = jnp.broadcast_to(yT[:, n:n + 1], (M, _T))

            zero = idx_s[2]
            for ref in s_s:
                ref[zero, 0:8, :] = jnp.zeros((8, _B), F32)
            q_s[zero, 0:8, :] = jnp.zeros((8, _T), U32)
            z_s[...] = jnp.zeros(z_s.shape, F32)
            z_s[zero, 0, 0:8, :] = jnp.zeros((8, _T), F32)
            side_s[zero, 0, 0:8, :] = jnp.zeros((8, _T), F32)
            zt_s[zero, 0:8, :] = jnp.zeros((8, _T), F32)
            wait(group('c'))
            pl.loop(0, NP)(lambda p: wait(kv_cp(p)))

        def head(h, carry):
            slot = h >> 1
            sh = ((1 - (h & 1)) * 16).astype(U32)
            wk = _as_f32((wk_buf[slot] << sh) & jnp.uint32(_HI))
            for t in range(ND_T):
                wk_s[t] = wk[:, t * _T:(t + 1) * _T].astype(BF16)
            wvT = _as_f32((wv_buf[slot] << sh) & jnp.uint32(_HI)).T.astype(BF16)
            for t in range(NC_T):
                wvT_s[t] = wvT[:, t * _T:(t + 1) * _T]
            for t in range(NS_T):
                q_s[t] = qc_s.bitcast(U32)[h, t]
            tri = (lax.broadcasted_iota(I32, (_T, _T), 0) <= lax.broadcasted_iota(I32, (_T, _T), 1))
            G, NG = _G, _NG
            lane_t = lax.broadcasted_iota(I32, (_T, _T), 1)
            row_g = lax.broadcasted_iota(I32, (G, _T), 0)
            lane_g = lax.broadcasted_iota(I32, (G, _T), 1)
            qn = _ld(qc_s, h, NS_T - 1).astype(F32).T
            for t in range(ND_T):
                qn_s[t] = qn[:, t * _T:(t + 1) * _T].astype(BF16)

            def c_rows(r0, n):
                return _cat([_ld(c_s, t, rows=(r0, n)) for t in range(NC_T)])

            def k_rows(r0, n):
                return _cat([_ld(k_s, t, rows=(r0, n)) for t in range(ND_T)])

            def proj_k(j, t):
                w = wk[:, t * _T:(t + 1) * _T] if j == 0 else _ld(wk_s, t)
                k_s[t, j * _B:(j + 1) * _B, :] = _mm(c_rows(j * _B, _B), w).astype(BF16)

            def proj_v(j, t):
                w = wvT if (j, t) == (0, 0) else _cat([_ld(wvT_s, u) for u in range(NC_T)])
                vT_s[2 * j + t] = _mm_nt(w, c_rows(j * _B + t * _T, _T)).astype(BF16)

            done = set()

            def piece(fn, j, t):
                if j < NB and (fn, j, t) not in done:
                    done.add((fn, j, t))
                    fn(j, t)

            items = [(j, c) for j in range(NB) for c in range(j + 1)]
            state, cmax = {}, {}

            def qk(i):
                j, c = items[i]
                for t in range(2):
                    piece(proj_k, c, t)
                k0, st = c * _B, s_s[i % _NS]
                q0u, q1u = q_s[2 * j], q_s[2 * j + 1]
                q0, q1 = pltpu.bitcast(q0u, BF16), pltpu.bitcast(q1u, BF16)
                q = _cat([q0, q1])

                def diag(r0, qu, g):
                    w = jnp.where(lane_t < g * G, q_s[NS_T - 1], qu) if g else qu
                    return _mm(k_rows(k0 + r0 + g * G, G), pltpu.bitcast(w, BF16))

                def z_parts():
                    u = c // 2
                    assert (proj_k, 2 * u + 1, 1) in done
                    for g in (1,) if c % 2 == 0 else (2, 3):
                        kg = _cat([k_rows((NG * u + p) * _T + g * G, G) for p in range(NG)], axis=0)
                        qg = _cat([_ld(qn_s, t, rows=(g * G, _T - g * G)) for t in range(ND_T)])
                        z_s[u, g - 1, g * G:, :] = _mm_nt(qg, kg)

                if c < j < NB - 1:
                    s = _mm(k_rows(k0, _B), q)
                    st[0] = s
                    cmax[i] = _colmax(s)
                elif c < j:
                    n1 = (_B + 5 * G) // 2
                    sa = _mm(k_rows(k0, n1), q0)
                    z_parts()
                    sb = _mm(k_rows(k0 + n1, _B - n1), q0)
                    su = _mm(_cat([k_rows(k0, G), k_rows(k0 + _T, G)], axis=0), q1)
                    s0 = _cat([sa, sb], axis=0)
                    st[0, :, 0:_T] = s0
                    st[0, 0:G, _T:] = su[:G]
                    st[0, _T:_T + G, _T:] = su[G:]
                    cmax[i] = _cat([_colmax(s0), _colmax(su)])
                elif j < NB - 1:
                    sab = _mm(k_rows(k0, _T), q1)
                    sa = [diag(0, q0u, g) for g in range(NG)]
                    sb = [diag(_T, q1u, g) for g in range(NG)]
                    for g in range(1, NG):
                        side_s[2 * j, g - 1] = sa[g]
                        side_s[2 * j + 1, g - 1] = sb[g]
                    s = _cat([jnp.where(tri, _cat(sa, axis=0), _NEG), sab])
                    s2 = jnp.where(tri, _cat(sb, axis=0), _NEG)
                    st[0, 0:_T, :] = s
                    st[0, _T:, _T:] = s2
                    m = _colmax(s)
                    cmax[i] = _cat([m[:, :_T], jnp.maximum(m[:, _T:], _colmax(s2))])
                else:
                    z_parts()
                    sa = [diag(0, q0u, 1)]
                    s_a0 = _mm(k_rows(k0, G), q)
                    sa += [diag(0, q0u, g) for g in range(2, NG)]
                    s_b0 = _cat([_mm(k_rows(k0 + _T + r, G // 2), q1) for r in (0, G // 2)], axis=0)
                    for g in range(1, NG):
                        side_s[2 * j, g - 1] = sa[g - 1]
                    s0 = jnp.where(tri, _cat([s_a0[:, :_T]] + sa, axis=0), _NEG)
                    s_b0 = jnp.where(row_g <= lane_g, s_b0, _NEG)
                    st[0, 0:_T, 0:_T] = s0
                    st[0, 0:G, _T:] = s_a0[:, _T:]
                    st[0, _T:_T + G, _T:] = s_b0
                    cmax[i] = _cat([_colmax(s0), jnp.maximum(_colmax(s_a0[:, _T:]), _colmax(s_b0))])

            def pv(i):
                j, c = items[i]
                for t in range(2):
                    piece(proj_v, c, t)
                st, m = s_s[i % _NS], cmax.pop(i)
                if j == NB - 1:
                    fix = []
                    for g in range(1, NG):
                        if c % 2 == 0:
                            zt = z_s[c // 2, g - 1].T
                            zt_s[g - 1] = zt[2 * G:]
                        else:
                            zt = zt_s[g - 1]
                        for r in range(2):
                            zr = zt[r * G:(r + 1) * G]
                            if 2 * c + r < NS_T - 1:
                                x = jnp.where(lane_g < g * G, side_s[2 * c + r, g - 1], zr)
                            else:
                                x = jnp.where(row_g + g * G <= lane_g, zr, _NEG)
                            st[0, r * _T + g * G:r * _T + (g + 1) * G, _T:] = x
                            fix.append(x)
                    m = _cat([m[:, :_T], jnp.maximum(m[:, _T:], _colmax(_cat(fix, axis=0)))])
                if c > 0:
                    m0, l0, o0 = state[j]
                    m = jnp.maximum(m0, m)
                    alpha = jnp.exp2(m0 - m)
                if c < j:
                    p = jnp.exp2(st[0] - m)
                    l = jnp.sum(p, axis=0, keepdims=True)
                    o = _mm(_cat([_ld(vT_s, 2 * c), _ld(vT_s, 2 * c + 1)]), p.astype(BF16))
                else:
                    p = jnp.exp2(st[0, 0:_T, :] - m)
                    p2 = jnp.exp2(st[0, _T:, _T:] - m[:, _T:])
                    l = jnp.sum(p, axis=0, keepdims=True)
                    l = _cat([l[:, :_T], l[:, _T:] + jnp.sum(p2, axis=0, keepdims=True)])
                    p, p2 = p.astype(BF16), p2.astype(BF16)
                    o = _cat([_mm(_ld(vT_s, 2 * c, rows=(r, D // 2)), p)
                              for r in range(0, D, D // 2)], axis=0)
                    o2 = _cat([_mm(_ld(vT_s, 2 * c + 1, rows=(r, D // 4)), p2)
                               for r in range(0, D, D // 4)], axis=0)
                    o = _cat([o[:, :_T], o[:, _T:] + o2])
                l = jnp.where(o[0:1] != o[0:1], o[0:1], l)
                if c > 0:
                    l = l0 * alpha + l
                    o = o0 * alpha + o
                state[j] = (m, l, o)
                if c == j:
                    ctx = o * (1.0 / l)
                    for t in range(2):
                        qc_s[h, 2 * j + t] = ctx[:, t * _T:(t + 1) * _T].astype(BF16)

            for i in range(len(items) + _LAG):
                if i < len(items):
                    qk(i)
                    j, c = items[i]
                    fill = [(proj_v, j, 0), (proj_v, j, 1), (proj_k, j + 1, 0), (proj_k, j + 1, 1)]
                    if j < NB - 1:
                        for pc in fill[len(fill) * c // (j + 1):len(fill) * (c + 1) // (j + 1)]:
                            piece(*pc)
                elif (i - len(items)) % 2 == 0:
                    piece(proj_v, NB - 1, (i - len(items)) // 2)
                if i >= _LAG:
                    pv(i - _LAG)

            return carry

        def run_heads():
            lax.fori_loop(0, H, head, 0)
            wait(group('wo'))

        def phase_o(j, carry):
            pl.when(j >= 2)(lambda: wait(o_cp(j - 2)))
            c0 = pl.multiple_of(j * _B, _B)
            a = None
            for hh in range(0, H, 2):
                w2 = _cat([_ld(woT_s, t, hh + u) for u in range(2) for t in range(ND_T)])
                x2 = _cat([_cat([_ld(qc_s, hh + u, 2 * j), _ld(qc_s, hh + u, 2 * j + 1)])
                           for u in range(2)], axis=0)
                part = _mm(w2, x2)
                a = part if a is None else a + part
            g = g_s[:, pl.ds(c0, _B)]
            rs = _sigmoid(r_s[:, pl.ds(c0, _B)])
            col = lax.broadcasted_iota(I32, (1, _B), 1) + j * _B
            b = _cat([xT_s[2 * j], xT_s[2 * j + 1]]).astype(F32)
            for n in range(2):
                b = b + _cat([y_s[n], y_s[n]]) * jnp.where(col == idx_s[n], rs, 0.0)
            o_s[j & 1] = (g * a + (1.0 - g) * b).astype(BF16)
            start(o_cp(j))
            return carry

        def run_o():
            lax.fori_loop(0, NB, phase_o, 0)

        def stage(k, carry):
            for i, fn in enumerate((run_pre, run_heads, run_o)):
                pl.when(k == i)(fn)
            return carry

        lax.fori_loop(0, 3, stage, 0)
        wait(o_cp(NB - 2) + o_cp(NB - 1))

    return kernel


@jax.jit
def pallas_gated_mix__compressed_kv_cla__moe_arch_mod__prompt_kernel(
    A_x: jax.Array,
    A_c_kv: jax.Array,
    A_w_q: jax.Array,
    A_w_uk: jax.Array,
    A_w_uv: jax.Array,
    A_w_o: jax.Array,
    B_x: jax.Array,
    B_w_r: jax.Array,
    B_w_gate: jax.Array,
    B_w_up: jax.Array,
    B_w_down: jax.Array,
    gate_w: jax.Array,
):
    _, S, M = A_x.shape
    C = A_c_kv.shape[2]
    H, D = A_w_q.shape[1], A_w_q.shape[2]
    FF = B_w_gate.shape[1]
    xT = A_x[0].T
    woT = jnp.transpose(A_w_o, (0, 2, 1))
    wdT = B_w_down.T
    any_spec = pl.BlockSpec(memory_space=pl.ANY)
    V = pltpu.VMEM
    outT = pl.pallas_call(
        _make_kernel(S, M, C, H, D, FF),
        in_specs=[any_spec] * 11,
        out_specs=any_spec,
        out_shape=jax.ShapeDtypeStruct((M, S), BF16),
        scratch_shapes=[
            V((S // _T, M, _T), BF16), V((C // _T, S, _T), BF16),
            V((H // 2, M, D), U32), V((H // 2, C, D), U32), V((H // 2, C, D), U32),
            V((D // _T, H, M, _T), BF16), V((M,), BF16), V((M,), BF16),
            V((M, FF), BF16), V((M, FF), BF16), V((M, FF), BF16),
            [V((pl.cdiv(M, _T), 2 * D, _T), BF16)] * 2, V((D // _T, C, _T), BF16),
            V((C // _T, D, _T), BF16), V((16, M), BF16),
            V((H, S // _T, D, _T), BF16), V((S // _T, D // 2, _T), U32),
            V((D // _T, S, _T), BF16), V((S // _T, D, _T), BF16),
            V((1, S), F32), V((1, S), F32), V((2, M, _T), F32), V((2, M, _B), BF16),
            [V((1, _B, _B), F32)] * _NS,
            V((S // _T // _NG, _NG - 1, _T, _T), F32), V((_NG - 1, 2 * _G, _T), F32),
            V((S // _T, _NG - 1, _G, _T), F32), V((D // _T, _T, _T), BF16),
            pltpu.SMEM((3,), I32),
            pltpu.SemaphoreType.DMA((6,)), pltpu.SemaphoreType.DMA((H // 2,)),
            pltpu.SemaphoreType.DMA(()), pltpu.SemaphoreType.DMA((2,)),
        ],
        compiler_params=pltpu.CompilerParams(vmem_limit_bytes=100 << 20),
    )(xT, A_c_kv[0], A_w_q, A_w_uk, A_w_uv, woT, B_w_r, gate_w, B_w_gate, B_w_up, wdT)
    return outT.T[None]
```

```python
import math

import jax
import jax.numpy as jnp
from jax import lax
import jax.experimental.pallas as pl
import jax.experimental.pallas.tpu as pltpu

F32, BF16, U32, I32 = jnp.float32, jnp.bfloat16, jnp.uint32, jnp.int32
_NT = (((1,), (1,)), ((), ()))
_NEG = -1e30
_HI = 0xFFFF0000
_T = 128
_B = 256
_LAG = 4
_NS = 6
_NG = 4
_G = _T // _NG
_XA, _XB = 2, 7


def _mm(a, b):
    return jnp.dot(a, b, preferred_element_type=F32)


def _mm_nt(a, b):
    return lax.dot_general(a, b, _NT, preferred_element_type=F32)


def _sigmoid(x):
    return 1.0 / (1.0 + jnp.exp(-x))


def _as_f32(u):
    return lax.bitcast_convert_type(u, F32)


def _cat(parts, axis=1):
    return parts[0] if len(parts) == 1 else jnp.concatenate(parts, axis=axis)


def _colmax(x):
    return jnp.max(x, axis=0, keepdims=True)


def _ld(ref, *lead, rows=None):
    u = ref.bitcast(U32)
    idx = lead if rows is None else lead + (slice(rows[0] // 2, (rows[0] + rows[1]) // 2),)
    return pltpu.bitcast(u[idx], BF16)


def _make_kernel(S, M, C, H, D, FF):
    NB, NP = S // _B, H // 2
    NS_T, NC_T, ND_T, NF_T = S // _T, C // _T, D // _T, FF // _T
    MF, MR = M // _T, M % _T
    assert ND_T == 2 and MR > 0 and _NS > _LAG >= 1 and _NG == 4 and NB % 2 == 0
    q_scale = math.log2(math.e) * (D ** -0.5)

    def kernel(xT_hbm, c_hbm, wq_hbm, wk_hbm, wv_hbm, woT_hbm, wr_hbm, gw_hbm,
               wg_hbm, wu_hbm, wdT_hbm, o_hbm,
               qc_s, wq_buf, wk_buf, wv_buf, xT_s, o_s, c_s, woT_s, wg_s, wu_s, wdT_s,
               wqT_s, wk_s, wvT_s, k_s, vT_s, y_s, s_s, z_s, zt_s, side_s, qn_s, wc_s,
               g_s, r_s, wr_s, gw_s, idx_s,
               sem, q_sem, kv_sem, o_sem):
        def tiled(src, dst, n):
            return [(src.at[..., t * _T:(t + 1) * _T], dst.at[t]) for t in range(n)]

        xt = tiled(xT_hbm, xT_s, NS_T)
        groups = dict(w=[(wr_hbm, wr_s), (gw_hbm, gw_s)], xa=xt[:_XA], xb=xt[_XA:_XB], xc=xt[_XB:],
                      ffn=[(wg_hbm, wg_s), (wu_hbm, wu_s), (wdT_hbm, wdT_s)],
                      c=tiled(c_hbm, c_s, NC_T), wo=tiled(woT_hbm, woT_s, ND_T))

        def group(name):
            s = sem.at[list(groups).index(name)]
            return [pltpu.make_async_copy(src, dst, s) for src, dst in groups[name]]

        def q_cp(p):
            return [pltpu.make_async_copy(wq_hbm.bitcast(U32).at[:, p, :], wq_buf.at[p], q_sem.at[p])]

        def kv_cp(p):
            return [pltpu.make_async_copy(src.bitcast(U32).at[:, p, :], dst.at[p], kv_sem)
                    for src, dst in ((wk_hbm, wk_buf), (wv_hbm, wv_buf))]

        def o_cp(j):
            c0 = pl.multiple_of(j * _B, _B)
            return [pltpu.make_async_copy(o_s.at[j & 1], o_hbm.at[:, pl.ds(c0, _B)], o_sem.at[j & 1])]

        def start(cps):
            for d in cps:
                d.start()

        def wait(cps):
            for d in cps:
                d.wait()

        def prep_q(p, b):
            w = wq_buf[p].T
            for half, u in enumerate((w << 16, w & jnp.uint32(_HI))):
                wb = _as_f32(u)
                for t in range(MF):
                    wqT_s[b][t, half * D:(half + 1) * D, :] = wb[:, t * _T:(t + 1) * _T].astype(BF16)
                wqT_s[b][MF, half * D:(half + 1) * D, 0:MR] = wb[:, MF * _T:].astype(BF16)

        def q_tile(p, t, b):
            wqT = _cat([_ld(wqT_s[b], u) for u in range(MF)] + [_ld(wqT_s[b], MF)[:, 0:MR]])
            q = _mm(wqT, _ld(xT_s, t)) * q_scale
            qc_s[2 * p, t] = q[:D].astype(BF16)
            qc_s[2 * p + 1, t] = q[D:].astype(BF16)

        def q_first(t0, t1):
            for t in range(t0, t1):
                q_tile(0, t, 0)
                xf = xT_s[t].astype(F32)
                r0, r1 = [jnp.sum(xf * wc_s[n], axis=0, keepdims=True) for n in range(2)]
                r_s[:, t * _T:(t + 1) * _T] = r0.astype(BF16).astype(F32)
                g_s[:, t * _T:(t + 1) * _T] = _sigmoid(r1)

        def run_pre():
            start(group('w') + q_cp(0) + group('xa') + group('xb') + group('xc'))
            pl.loop(1, NP)(lambda p: start(q_cp(p)))
            start(group('ffn') + group('c'))
            pl.loop(0, NP)(lambda p: start(kv_cp(p)))
            start(group('wo'))
            for b in range(2):
                wqT_s[b][MF] = jnp.zeros((2 * D, _T), BF16)
            idx_s[2] = 0
            wait(group('w'))
            for n, ref in enumerate((wr_s, gw_s)):
                wc_s[n] = jnp.broadcast_to(ref[...].astype(F32).reshape(1, M), (_T, M)).T
            wait(q_cp(0))
            prep_q(0, 0)
            wait(group('xa'))
            q_first(0, _XA)
            wait(group('xb'))
            q_first(_XA, _XB)
            wait(group('xc') + q_cp(1))
            prep_q(1, 1)
            q_first(_XB, NS_T)
            wait(q_cp(2) + q_cp(3))

            def phase_q(i, carry):
                p = 2 * i + 1
                prep_q(p + 1, 0)
                for t in range(NS_T):
                    q_tile(p, t, 1)
                prep_q(p + 2, 1)
                for t in range(NS_T):
                    q_tile(p + 1, t, 0)
                pl.when(p + 4 < NP)(lambda: wait(q_cp(p + 3) + q_cp(p + 4)))
                return carry

            lax.fori_loop(0, (NP - 2) // 2, phase_q, 0)
            wait(group('ffn'))

            lane = lax.broadcasted_iota(I32, (1, S), 1)
            idxs, cur = [], r_s[...]
            for n in range(2):
                mx = jnp.max(cur, axis=1, keepdims=True)
                ii = jnp.min(jnp.where(cur == mx, lane, S - 1))
                idxs.append(ii)
                idx_s[n] = ii
                cur = jnp.where(lane == ii, -jnp.inf, cur)
            ffn = {}

            def ffn_select(n):
                row16 = lax.broadcasted_iota(I32, (16, _T), 0)
                lane16 = lax.broadcasted_iota(I32, (16, _T), 1)
                oh = jnp.logical_and(row16 == n, lane16 == (idxs[n] & (_T - 1)))
                xr = _mm_nt(jnp.where(oh, 1.0, 0.0).astype(BF16), _ld(xT_s, idxs[n] // _T))
                ffn['x'] = xr if n == 0 else (ffn['x'] + xr).astype(BF16)

            def ffn_gate(f):
                ffn['g', f] = _mm(ffn['x'], wg_s[:, f * _T:(f + 1) * _T])

            def ffn_up(f):
                gt = ffn['g', f]
                ffn[f] = (gt * _sigmoid(gt) * _mm(ffn['x'], wu_s[:, f * _T:(f + 1) * _T])).astype(BF16)

            def ffn_down(f):
                y = _mm_nt(ffn[f], wdT_s[:, f * _T:(f + 1) * _T])
                ffn['y'] = y if 'y' not in ffn else ffn['y'] + y

            plain = [(fn, f) for f in range(NF_T) for fn in (ffn_gate, ffn_up)]
            after = {5: [(ffn_select, 0)], 6: [(ffn_select, 1)]}
            gap, nd, ready = 8, 0, {}
            while plain or nd < NF_T:
                slot = []
                if nd < NF_T and ready.get(nd, gap) < gap:
                    slot.append((ffn_down, nd))
                    nd += 1
                while len(slot) < 2 and plain:
                    fn, f = plain.pop(0)
                    slot.append((fn, f))
                    if fn is ffn_up:
                        ready[f] = gap
                after[gap] = slot
                gap += 1
            assert gap <= 2 * NS_T - 1, gap
            for t in range(NS_T):
                if 2 * t in after:
                    for half in range(2):
                        w = _cat([_ld(wqT_s[1], u, rows=(half * D, D)) for u in range(MF)]
                                 + [_ld(wqT_s[1], MF, rows=(half * D, D))[:, 0:MR]])
                        qc_s[2 * (NP - 1) + half, t] = (_mm(w, _ld(xT_s, t)) * q_scale).astype(BF16)
                        for fn, f in after.get(2 * t + half, []):
                            fn(f)
                else:
                    q_tile(NP - 1, t, 1)
                    for fn, f in after.get(2 * t + 1, []):
                        fn(f)
            yp = jnp.concatenate([ffn['y'], jnp.zeros((16, (MF + 1) * _T - M), F32)], axis=1)
            yT = jnp.concatenate([yp, jnp.zeros((_T - 16, (MF + 1) * _T), F32)], axis=0).T[:M]
            for n in range(2):
                y_s[n] = jnp.broadcast_to(yT[:, n:n + 1], (M, _T))

            zero = idx_s[2]
            for ref in s_s:
                ref[zero, 0:8, :] = jnp.zeros((8, _B), F32)
            z_s[...] = jnp.zeros(z_s.shape, F32)
            z_s[zero, 0, 0:8, :] = jnp.zeros((8, _T), F32)
            side_s[zero, 0, 0:8, :] = jnp.zeros((8, _T), F32)
            zt_s[zero, 0:8, :] = jnp.zeros((8, _T), F32)
            wait(group('c'))
            pl.loop(0, NP)(lambda p: wait(kv_cp(p)))

        def head(h, carry):
            slot = h >> 1
            sh = ((1 - (h & 1)) * 16).astype(U32)
            wk = _as_f32((wk_buf[slot] << sh) & jnp.uint32(_HI))
            for t in range(ND_T):
                wk_s[t] = wk[:, t * _T:(t + 1) * _T].astype(BF16)
            wvT = _as_f32((wv_buf[slot] << sh) & jnp.uint32(_HI)).T.astype(BF16)
            for t in range(NC_T):
                wvT_s[t] = wvT[:, t * _T:(t + 1) * _T]
            tri = (lax.broadcasted_iota(I32, (_T, _T), 0) <= lax.broadcasted_iota(I32, (_T, _T), 1))
            G, NG, q_u = _G, _NG, qc_s.bitcast(U32)
            lane_t = lax.broadcasted_iota(I32, (_T, _T), 1)
            row_g = lax.broadcasted_iota(I32, (G, _T), 0)
            lane_g = lax.broadcasted_iota(I32, (G, _T), 1)
            qn = _ld(qc_s, h, NS_T - 1).astype(F32).T
            for t in range(ND_T):
                qn_s[t] = qn[:, t * _T:(t + 1) * _T].astype(BF16)

            def c_rows(r0, n):
                return _cat([_ld(c_s, t, rows=(r0, n)) for t in range(NC_T)])

            def k_rows(r0, n):
                return _cat([_ld(k_s, t, rows=(r0, n)) for t in range(ND_T)])

            def proj_k(j, t):
                w = wk[:, t * _T:(t + 1) * _T] if j == 0 else _ld(wk_s, t)
                k_s[t, j * _B:(j + 1) * _B, :] = _mm(c_rows(j * _B, _B), w).astype(BF16)

            def proj_v(j, t):
                w = wvT if (j, t) == (0, 0) else _cat([_ld(wvT_s, u) for u in range(NC_T)])
                vT_s[2 * j + t] = _mm_nt(w, c_rows(j * _B + t * _T, _T)).astype(BF16)

            done = set()

            def piece(fn, j, t):
                if j < NB and (fn, j, t) not in done:
                    done.add((fn, j, t))
                    fn(j, t)

            items = [(j, c) for j in range(NB) for c in range(j + 1)]
            state, cmax = {}, {}

            def qk(i):
                j, c = items[i]
                for t in range(2):
                    piece(proj_k, c, t)
                k0, st = c * _B, s_s[i % _NS]
                q0u, q1u = q_u[h, 2 * j], q_u[h, 2 * j + 1]
                q0, q1 = pltpu.bitcast(q0u, BF16), pltpu.bitcast(q1u, BF16)
                q = _cat([q0, q1])

                def diag(r0, qu, g):
                    w = jnp.where(lane_t < g * G, q_u[h, NS_T - 1], qu) if g else qu
                    return _mm(k_rows(k0 + r0 + g * G, G), pltpu.bitcast(w, BF16))

                def z_parts():
                    u = c // 2
                    assert (proj_k, 2 * u + 1, 1) in done
                    for g in (1,) if c % 2 == 0 else (2, 3):
                        kg = _cat([k_rows((NG * u + p) * _T + g * G, G) for p in range(NG)], axis=0)
                        qg = _cat([_ld(qn_s, t, rows=(g * G, _T - g * G)) for t in range(ND_T)])
                        z_s[u, g - 1, g * G:, :] = _mm_nt(qg, kg)

                if c < j < NB - 1:
                    s = _mm(k_rows(k0, _B), q)
                    st[0] = s
                    cmax[i] = _colmax(s)
                elif c < j:
                    n1 = (_B + 5 * G) // 2
                    sa = _mm(k_rows(k0, n1), q0)
                    z_parts()
                    sb = _mm(k_rows(k0 + n1, _B - n1), q0)
                    su = _mm(_cat([k_rows(k0, G), k_rows(k0 + _T, G)], axis=0), q1)
                    s0 = _cat([sa, sb], axis=0)
                    st[0, :, 0:_T] = s0
                    st[0, 0:G, _T:] = su[:G]
                    st[0, _T:_T + G, _T:] = su[G:]
                    cmax[i] = _cat([_colmax(s0), _colmax(su)])
                elif j < NB - 1:
                    sab = _mm(k_rows(k0, _T), q1)
                    sa = [diag(0, q0u, g) for g in range(NG)]
                    sb = [diag(_T, q1u, g) for g in range(NG)]
                    for g in range(1, NG):
                        side_s[2 * j, g - 1] = sa[g]
                        side_s[2 * j + 1, g - 1] = sb[g]
                    s = _cat([jnp.where(tri, _cat(sa, axis=0), _NEG), sab])
                    s2 = jnp.where(tri, _cat(sb, axis=0), _NEG)
                    st[0, 0:_T, :] = s
                    st[0, _T:, _T:] = s2
                    m = _colmax(s)
                    cmax[i] = _cat([m[:, :_T], jnp.maximum(m[:, _T:], _colmax(s2))])
                else:
                    z_parts()
                    sa = [diag(0, q0u, 1)]
                    s_a0 = _mm(k_rows(k0, G), q)
                    sa += [diag(0, q0u, g) for g in range(2, NG)]
                    s_b0 = _cat([_mm(k_rows(k0 + _T + r, G // 2), q1) for r in (0, G // 2)], axis=0)
                    for g in range(1, NG):
                        side_s[2 * j, g - 1] = sa[g - 1]
                    s0 = jnp.where(tri, _cat([s_a0[:, :_T]] + sa, axis=0), _NEG)
                    s_b0 = jnp.where(row_g <= lane_g, s_b0, _NEG)
                    st[0, 0:_T, 0:_T] = s0
                    st[0, 0:G, _T:] = s_a0[:, _T:]
                    st[0, _T:_T + G, _T:] = s_b0
                    cmax[i] = _cat([_colmax(s0), jnp.maximum(_colmax(s_a0[:, _T:]), _colmax(s_b0))])

            def pv(i):
                j, c = items[i]
                for t in range(2):
                    piece(proj_v, c, t)
                st, m = s_s[i % _NS], cmax.pop(i)
                if j == NB - 1:
                    fix = []
                    for g in range(1, NG):
                        if c % 2 == 0:
                            zt = z_s[c // 2, g - 1].T
                            zt_s[g - 1] = zt[2 * G:]
                        else:
                            zt = zt_s[g - 1]
                        for r in range(2):
                            zr = zt[r * G:(r + 1) * G]
                            if 2 * c + r < NS_T - 1:
                                x = jnp.where(lane_g < g * G, side_s[2 * c + r, g - 1], zr)
                            else:
                                x = jnp.where(row_g + g * G <= lane_g, zr, _NEG)
                            st[0, r * _T + g * G:r * _T + (g + 1) * G, _T:] = x
                            fix.append(x)
                    m = _cat([m[:, :_T], jnp.maximum(m[:, _T:], _colmax(_cat(fix, axis=0)))])
                if c > 0:
                    m0, l0, o0 = state[j]
                    m = jnp.maximum(m0, m)
                    alpha = jnp.exp2(m0 - m)
                if c < j:
                    p = jnp.exp2(st[0] - m)
                    l = jnp.sum(p, axis=0, keepdims=True)
                    o = _mm(_cat([_ld(vT_s, 2 * c), _ld(vT_s, 2 * c + 1)]), p.astype(BF16))
                else:
                    p = jnp.exp2(st[0, 0:_T, :] - m)
                    p2 = jnp.exp2(st[0, _T:, _T:] - m[:, _T:])
                    l = jnp.sum(p, axis=0, keepdims=True)
                    l = _cat([l[:, :_T], l[:, _T:] + jnp.sum(p2, axis=0, keepdims=True)])
                    p, p2 = p.astype(BF16), p2.astype(BF16)
                    o = _cat([_mm(_ld(vT_s, 2 * c, rows=(r, D // 2)), p)
                              for r in range(0, D, D // 2)], axis=0)
                    o2 = _cat([_mm(_ld(vT_s, 2 * c + 1, rows=(r, D // 4)), p2)
                               for r in range(0, D, D // 4)], axis=0)
                    o = _cat([o[:, :_T], o[:, _T:] + o2])
                l = jnp.where(o[0:1] != o[0:1], o[0:1], l)
                if c > 0:
                    l = l0 * alpha + l
                    o = o0 * alpha + o
                state[j] = (m, l, o)
                if c == j:
                    ctx = o * (1.0 / l)
                    for t in range(2):
                        qc_s[h, 2 * j + t] = ctx[:, t * _T:(t + 1) * _T].astype(BF16)

            for i in range(len(items) + _LAG):
                if i < len(items):
                    qk(i)
                    j, c = items[i]
                    fill = [(proj_v, j, 0), (proj_v, j, 1), (proj_k, j + 1, 0), (proj_k, j + 1, 1)]
                    if j < NB - 1:
                        for pc in fill[len(fill) * c // (j + 1):len(fill) * (c + 1) // (j + 1)]:
                            piece(*pc)
                elif i - len(items) in (0, 2):
                    piece(proj_v, NB - 1, (i - len(items)) // 2)
                if i >= _LAG:
                    pv(i - _LAG)

            return carry

        def run_heads():
            lax.fori_loop(0, H, head, 0)
            wait(group('wo'))

        def phase_o(j, carry):
            pl.when(j >= 2)(lambda: wait(o_cp(j - 2)))
            c0 = pl.multiple_of(j * _B, _B)
            a = None
            for hh in range(0, H, 2):
                w2 = _cat([_ld(woT_s, t, hh + u) for u in range(2) for t in range(ND_T)])
                x2 = _cat([_cat([_ld(qc_s, hh + u, 2 * j), _ld(qc_s, hh + u, 2 * j + 1)])
                           for u in range(2)], axis=0)
                part = _mm(w2, x2)
                a = part if a is None else a + part
            g = g_s[:, pl.ds(c0, _B)]
            rs = _sigmoid(r_s[:, pl.ds(c0, _B)])
            col = lax.broadcasted_iota(I32, (1, _B), 1) + j * _B
            b = _cat([xT_s[2 * j], xT_s[2 * j + 1]]).astype(F32)
            for n in range(2):
                b = b + _cat([y_s[n], y_s[n]]) * jnp.where(col == idx_s[n], rs, 0.0)
            o_s[j & 1] = (g * a + (1.0 - g) * b).astype(BF16)
            start(o_cp(j))
            return carry

        def run_o():
            lax.fori_loop(0, NB, phase_o, 0)

        def stage(k, carry):
            for i, fn in enumerate((run_pre, run_heads, run_o)):
                pl.when(k == i)(fn)
            return carry

        lax.fori_loop(0, 3, stage, 0)
        wait(o_cp(NB - 2) + o_cp(NB - 1))

    return kernel


@jax.jit
def pallas_gated_mix__compressed_kv_cla__moe_arch_mod__prompt_kernel(
    A_x: jax.Array,
    A_c_kv: jax.Array,
    A_w_q: jax.Array,
    A_w_uk: jax.Array,
    A_w_uv: jax.Array,
    A_w_o: jax.Array,
    B_x: jax.Array,
    B_w_r: jax.Array,
    B_w_gate: jax.Array,
    B_w_up: jax.Array,
    B_w_down: jax.Array,
    gate_w: jax.Array,
):
    _, S, M = A_x.shape
    C = A_c_kv.shape[2]
    H, D = A_w_q.shape[1], A_w_q.shape[2]
    FF = B_w_gate.shape[1]
    xT = A_x[0].T
    woT = jnp.transpose(A_w_o, (0, 2, 1))
    wdT = B_w_down.T
    any_spec = pl.BlockSpec(memory_space=pl.ANY)
    V = pltpu.VMEM
    outT = pl.pallas_call(
        _make_kernel(S, M, C, H, D, FF),
        in_specs=[any_spec] * 11,
        out_specs=any_spec,
        out_shape=jax.ShapeDtypeStruct((M, S), BF16),
        scratch_shapes=[
            V((H, S // _T, D, _T), BF16),
            V((H // 2, M, D), U32), V((H // 2, C, D), U32), V((H // 2, C, D), U32),
            V((S // _T, M, _T), BF16), V((2, M, _B), BF16),
            V((C // _T, S, _T), BF16), V((D // _T, H, M, _T), BF16),
            V((M, FF), BF16), V((M, FF), BF16), V((M, FF), BF16),
            [V((pl.cdiv(M, _T), 2 * D, _T), BF16)] * 2, V((D // _T, C, _T), BF16),
            V((C // _T, D, _T), BF16),
            V((D // _T, S, _T), BF16), V((S // _T, D, _T), BF16), V((2, M, _T), F32),
            [V((1, _B, _B), F32)] * _NS,
            V((S // _T // _NG, _NG - 1, _T, _T), F32), V((_NG - 1, 2 * _G, _T), F32),
            V((S // _T, _NG - 1, _G, _T), F32), V((D // _T, _T, _T), BF16),
            V((2, M, _T), F32),
            V((1, S), F32), V((1, S), F32), V((M,), BF16), V((M,), BF16),
            pltpu.SMEM((3,), I32),
            pltpu.SemaphoreType.DMA((7,)), pltpu.SemaphoreType.DMA((H // 2,)),
            pltpu.SemaphoreType.DMA(()), pltpu.SemaphoreType.DMA((2,)),
        ],
        compiler_params=pltpu.CompilerParams(vmem_limit_bytes=100 << 20),
    )(xT, A_c_kv[0], A_w_q, A_w_uk, A_w_uv, woT, B_w_r, gate_w, B_w_gate, B_w_up, wdT)
    return outT.T[None]
```

```python
import math

import jax
import jax.numpy as jnp
from jax import lax
import jax.experimental.pallas as pl
import jax.experimental.pallas.tpu as pltpu

F32, BF16, U32, I32 = jnp.float32, jnp.bfloat16, jnp.uint32, jnp.int32
_NT = (((1,), (1,)), ((), ()))
_NEG = -1e30
_HI = 0xFFFF0000
_T = 128
_B = 256
_LAG = 5
_NS = 7
_NG = 4
_G = _T // _NG
_XA, _XB = 2, 7


def _mm(a, b):
    return jnp.dot(a, b, preferred_element_type=F32)


def _mm_nt(a, b):
    return lax.dot_general(a, b, _NT, preferred_element_type=F32)


def _sigmoid(x):
    return 1.0 / (1.0 + jnp.exp(-x))


def _as_f32(u):
    return lax.bitcast_convert_type(u, F32)


def _cat(parts, axis=1):
    return parts[0] if len(parts) == 1 else jnp.concatenate(parts, axis=axis)


def _colmax(x):
    return jnp.max(x, axis=0, keepdims=True)


def _ld(ref, *lead, rows=None):
    u = ref.bitcast(U32)
    idx = lead if rows is None else lead + (slice(rows[0] // 2, (rows[0] + rows[1]) // 2),)
    return pltpu.bitcast(u[idx], BF16)


def _make_kernel(S, M, C, H, D, FF):
    NB, NP = S // _B, H // 2
    NS_T, NC_T, ND_T, NF_T = S // _T, C // _T, D // _T, FF // _T
    MF, MR = M // _T, M % _T
    assert ND_T == 2 and MR > 0 and _NS > _LAG >= 1 and _NG == 4 and NB % 2 == 0
    q_scale = math.log2(math.e) * (D ** -0.5)

    def kernel(xT_hbm, c_hbm, wq_hbm, wk_hbm, wv_hbm, woT_hbm, wr_hbm, gw_hbm,
               wg_hbm, wu_hbm, wdT_hbm, o_hbm,
               qc_s, wq_buf, wk_buf, wv_buf, xT_s, o_s, c_s, woT_s, wg_s, wu_s, wdT_s,
               wqT_s, wk_s, wvT_s, k_s, vT_s, y_s, s_s, z_s, zt_s, side_s, qn_s, wc_s,
               g_s, r_s, wr_s, gw_s, idx_s,
               sem, q_sem, kv_sem, o_sem):
        def tiled(src, dst, n):
            return [(src.at[..., t * _T:(t + 1) * _T], dst.at[t]) for t in range(n)]

        xt = tiled(xT_hbm, xT_s, NS_T)
        groups = dict(w=[(wr_hbm, wr_s), (gw_hbm, gw_s)], xa=xt[:_XA], xb=xt[_XA:_XB], xc=xt[_XB:],
                      ffn=[(wg_hbm, wg_s), (wu_hbm, wu_s), (wdT_hbm, wdT_s)],
                      c=tiled(c_hbm, c_s, NC_T), wo=tiled(woT_hbm, woT_s, ND_T))

        def group(name):
            s = sem.at[list(groups).index(name)]
            return [pltpu.make_async_copy(src, dst, s) for src, dst in groups[name]]

        def q_cp(p):
            return [pltpu.make_async_copy(wq_hbm.bitcast(U32).at[:, p, :], wq_buf.at[p], q_sem.at[p])]

        def kv_cp(p):
            return [pltpu.make_async_copy(src.bitcast(U32).at[:, p, :], dst.at[p], kv_sem)
                    for src, dst in ((wk_hbm, wk_buf), (wv_hbm, wv_buf))]

        def o_cp(j):
            c0 = pl.multiple_of(j * _B, _B)
            return [pltpu.make_async_copy(o_s.at[j & 1], o_hbm.at[:, pl.ds(c0, _B)], o_sem.at[j & 1])]

        def start(cps):
            for d in cps:
                d.start()

        def wait(cps):
            for d in cps:
                d.wait()

        def prep_q(p, b):
            w = wq_buf[p].T
            for half, u in enumerate((w << 16, w & jnp.uint32(_HI))):
                wb = _as_f32(u)
                for t in range(MF):
                    wqT_s[b][t, half * D:(half + 1) * D, :] = wb[:, t * _T:(t + 1) * _T].astype(BF16)
                wqT_s[b][MF, half * D:(half + 1) * D, 0:MR] = wb[:, MF * _T:].astype(BF16)

        def q_tile(p, t, b):
            wqT = _cat([_ld(wqT_s[b], u) for u in range(MF)] + [_ld(wqT_s[b], MF)[:, 0:MR]])
            q = _mm(wqT, _ld(xT_s, t)) * q_scale
            qc_s[2 * p, t] = q[:D].astype(BF16)
            qc_s[2 * p + 1, t] = q[D:].astype(BF16)

        def q_first(t0, t1):
            for t in range(t0, t1):
                q_tile(0, t, 0)
                xf = xT_s[t].astype(F32)
                r0, r1 = [jnp.sum(xf * wc_s[n], axis=0, keepdims=True) for n in range(2)]
                r_s[:, t * _T:(t + 1) * _T] = r0.astype(BF16).astype(F32)
                g_s[:, t * _T:(t + 1) * _T] = _sigmoid(r1)

        def run_pre():
            start(group('w') + q_cp(0) + group('xa') + group('xb') + group('xc'))
            pl.loop(1, NP)(lambda p: start(q_cp(p)))
            start(group('ffn') + group('c'))
            pl.loop(0, NP)(lambda p: start(kv_cp(p)))
            start(group('wo'))
            for b in range(2):
                wqT_s[b][MF] = jnp.zeros((2 * D, _T), BF16)
            idx_s[2] = 0
            wait(group('w'))
            for n, ref in enumerate((wr_s, gw_s)):
                wc_s[n] = jnp.broadcast_to(ref[...].astype(F32).reshape(1, M), (_T, M)).T
            wait(q_cp(0))
            prep_q(0, 0)
            wait(group('xa'))
            q_first(0, _XA)
            wait(group('xb'))
            q_first(_XA, _XB)
            wait(group('xc') + q_cp(1))
            prep_q(1, 1)
            q_first(_XB, NS_T)
            wait(q_cp(2) + q_cp(3))

            def phase_q(i, carry):
                p = 2 * i + 1
                prep_q(p + 1, 0)
                for t in range(NS_T):
                    q_tile(p, t, 1)
                prep_q(p + 2, 1)
                for t in range(NS_T):
                    q_tile(p + 1, t, 0)
                pl.when(p + 4 < NP)(lambda: wait(q_cp(p + 3) + q_cp(p + 4)))
                return carry

            lax.fori_loop(0, (NP - 2) // 2, phase_q, 0)
            wait(group('ffn'))

            lane = lax.broadcasted_iota(I32, (1, S), 1)
            idxs, cur = [], r_s[...]
            for n in range(2):
                mx = jnp.max(cur, axis=1, keepdims=True)
                ii = jnp.min(jnp.where(cur == mx, lane, S - 1))
                idxs.append(ii)
                idx_s[n] = ii
                cur = jnp.where(lane == ii, -jnp.inf, cur)
            ffn = {}

            def ffn_select(n):
                row16 = lax.broadcasted_iota(I32, (16, _T), 0)
                lane16 = lax.broadcasted_iota(I32, (16, _T), 1)
                oh = jnp.logical_and(row16 == n, lane16 == (idxs[n] & (_T - 1)))
                xr = _mm_nt(jnp.where(oh, 1.0, 0.0).astype(BF16), _ld(xT_s, idxs[n] // _T))
                ffn['x'] = xr if n == 0 else (ffn['x'] + xr).astype(BF16)

            def ffn_gate(f):
                ffn['g', f] = _mm(ffn['x'], wg_s[:, f * _T:(f + 1) * _T])

            def ffn_up(f):
                gt = ffn['g', f]
                ffn[f] = (gt * _sigmoid(gt) * _mm(ffn['x'], wu_s[:, f * _T:(f + 1) * _T])).astype(BF16)

            def ffn_down(f):
                y = _mm_nt(ffn[f], wdT_s[:, f * _T:(f + 1) * _T])
                ffn['y'] = y if 'y' not in ffn else ffn['y'] + y

            plain = [(fn, f) for f in range(NF_T) for fn in (ffn_gate, ffn_up)]
            after = {5: [(ffn_select, 0)], 6: [(ffn_select, 1)]}
            gap, nd, ready = 7, 0, {}
            while plain or nd < NF_T:
                slot = []
                if nd < NF_T and ready.get(nd, gap) < gap:
                    slot.append((ffn_down, nd))
                    nd += 1
                while len(slot) < 2 and plain:
                    fn, f = plain.pop(0)
                    slot.append((fn, f))
                    if fn is ffn_up:
                        ready[f] = gap
                after[gap] = slot
                gap += 1
            assert gap <= 2 * NS_T - 1, gap
            for t in range(NS_T):
                if 2 * t in after:
                    for half in range(2):
                        w = _cat([_ld(wqT_s[1], u, rows=(half * D, D)) for u in range(MF)]
                                 + [_ld(wqT_s[1], MF, rows=(half * D, D))[:, 0:MR]])
                        qc_s[2 * (NP - 1) + half, t] = (_mm(w, _ld(xT_s, t)) * q_scale).astype(BF16)
                        for fn, f in after.get(2 * t + half, []):
                            fn(f)
                else:
                    q_tile(NP - 1, t, 1)
                    for fn, f in after.get(2 * t + 1, []):
                        fn(f)
            yp = jnp.concatenate([ffn['y'], jnp.zeros((16, (MF + 1) * _T - M), F32)], axis=1)
            yT = jnp.concatenate([yp, jnp.zeros((_T - 16, (MF + 1) * _T), F32)], axis=0).T[:M]
            for n in range(2):
                y_s[n] = jnp.broadcast_to(yT[:, n:n + 1], (M, _T))

            zero = idx_s[2]
            for ref in s_s:
                ref[zero, 0:8, :] = jnp.zeros((8, _B), F32)
            z_s[...] = jnp.zeros(z_s.shape, F32)
            z_s[zero, 0, 0:8, :] = jnp.zeros((8, _T), F32)
            side_s[zero, 0, 0:8, :] = jnp.zeros((8, _T), F32)
            zt_s[zero, 0:8, :] = jnp.zeros((8, _T), F32)
            wait(group('c'))
            pl.loop(0, NP)(lambda p: wait(kv_cp(p)))

        def head(h, carry):
            slot = h >> 1
            sh = ((1 - (h & 1)) * 16).astype(U32)
            wk = _as_f32((wk_buf[slot] << sh) & jnp.uint32(_HI))
            for t in range(ND_T):
                wk_s[t] = wk[:, t * _T:(t + 1) * _T].astype(BF16)
            wvT = _as_f32((wv_buf[slot] << sh) & jnp.uint32(_HI)).T.astype(BF16)
            for t in range(NC_T):
                wvT_s[t] = wvT[:, t * _T:(t + 1) * _T]
            tri = (lax.broadcasted_iota(I32, (_T, _T), 0) <= lax.broadcasted_iota(I32, (_T, _T), 1))
            G, NG, q_u = _G, _NG, qc_s.bitcast(U32)
            lane_t = lax.broadcasted_iota(I32, (_T, _T), 1)
            row_g = lax.broadcasted_iota(I32, (G, _T), 0)
            lane_g = lax.broadcasted_iota(I32, (G, _T), 1)
            qn = _ld(qc_s, h, NS_T - 1).astype(F32).T
            for t in range(ND_T):
                qn_s[t] = qn[:, t * _T:(t + 1) * _T].astype(BF16)

            def c_rows(r0, n):
                return _cat([_ld(c_s, t, rows=(r0, n)) for t in range(NC_T)])

            def k_rows(r0, n):
                return _cat([_ld(k_s, t, rows=(r0, n)) for t in range(ND_T)])

            def proj_k(j, t):
                w = wk[:, t * _T:(t + 1) * _T] if j == 0 else _ld(wk_s, t)
                k_s[t, j * _B:(j + 1) * _B, :] = _mm(c_rows(j * _B, _B), w).astype(BF16)

            def proj_v(j, t):
                w = wvT if (j, t) == (0, 0) else _cat([_ld(wvT_s, u) for u in range(NC_T)])
                vT_s[2 * j + t] = _mm_nt(w, c_rows(j * _B + t * _T, _T)).astype(BF16)

            done = set()

            def piece(fn, j, t):
                if j < NB and (fn, j, t) not in done:
                    done.add((fn, j, t))
                    fn(j, t)

            items = [(j, c) for j in range(NB) for c in range(j + 1)]
            state, cmax = {}, {}

            def qk(i):
                j, c = items[i]
                for t in range(2):
                    piece(proj_k, c, t)
                k0, st = c * _B, s_s[i % _NS]
                q0u, q1u = q_u[h, 2 * j], q_u[h, 2 * j + 1]
                q0, q1 = pltpu.bitcast(q0u, BF16), pltpu.bitcast(q1u, BF16)
                q = _cat([q0, q1])

                def diag(r0, qu, g):
                    w = jnp.where(lane_t < g * G, q_u[h, NS_T - 1], qu) if g else qu
                    return _mm(k_rows(k0 + r0 + g * G, G), pltpu.bitcast(w, BF16))

                def z_parts():
                    u = c // 2
                    assert (proj_k, 2 * u + 1, 1) in done
                    for g in (1,) if c % 2 == 0 else (2, 3):
                        kg = _cat([k_rows((NG * u + p) * _T + g * G, G) for p in range(NG)], axis=0)
                        qg = _cat([_ld(qn_s, t, rows=(g * G, _T - g * G)) for t in range(ND_T)])
                        z_s[u, g - 1, g * G:, :] = _mm_nt(qg, kg)

                if c < j < NB - 1:
                    s = _mm(k_rows(k0, _B), q)
                    st[0] = s
                    cmax[i] = _colmax(s)
                elif c < j:
                    n1 = (_B + 5 * G) // 2
                    sa = _mm(k_rows(k0, n1), q0)
                    z_parts()
                    sb = _mm(k_rows(k0 + n1, _B - n1), q0)
                    su = _mm(_cat([k_rows(k0, G), k_rows(k0 + _T, G)], axis=0), q1)
                    s0 = _cat([sa, sb], axis=0)
                    st[0, :, 0:_T] = s0
                    st[0, 0:G, _T:] = su[:G]
                    st[0, _T:_T + G, _T:] = su[G:]
                    cmax[i] = _cat([_colmax(s0), _colmax(su)])
                elif j < NB - 1:
                    sab = _mm(k_rows(k0, _T), q1)
                    sa = [diag(0, q0u, g) for g in range(NG)]
                    sb = [diag(_T, q1u, g) for g in range(NG)]
                    for g in range(1, NG):
                        side_s[2 * j, g - 1] = sa[g]
                        side_s[2 * j + 1, g - 1] = sb[g]
                    s = _cat([jnp.where(tri, _cat(sa, axis=0), _NEG), sab])
                    s2 = jnp.where(tri, _cat(sb, axis=0), _NEG)
                    st[0, 0:_T, :] = s
                    st[0, _T:, _T:] = s2
                    m = _colmax(s)
                    cmax[i] = _cat([m[:, :_T], jnp.maximum(m[:, _T:], _colmax(s2))])
                else:
                    z_parts()
                    sa = [diag(0, q0u, 1)]
                    s_a0 = _mm(k_rows(k0, G), q)
                    sa += [diag(0, q0u, g) for g in range(2, NG)]
                    s_b0 = _cat([_mm(k_rows(k0 + _T + r, G // 2), q1) for r in (0, G // 2)], axis=0)
                    for g in range(1, NG):
                        side_s[2 * j, g - 1] = sa[g - 1]
                    s0 = jnp.where(tri, _cat([s_a0[:, :_T]] + sa, axis=0), _NEG)
                    s_b0 = jnp.where(row_g <= lane_g, s_b0, _NEG)
                    st[0, 0:_T, 0:_T] = s0
                    st[0, 0:G, _T:] = s_a0[:, _T:]
                    st[0, _T:_T + G, _T:] = s_b0
                    cmax[i] = _cat([_colmax(s0), jnp.maximum(_colmax(s_a0[:, _T:]), _colmax(s_b0))])

            def pv(i):
                j, c = items[i]
                for t in range(2):
                    piece(proj_v, c, t)
                st, m = s_s[i % _NS], cmax.pop(i)
                if j == NB - 1:
                    fix = []
                    for g in range(1, NG):
                        if c % 2 == 0:
                            zt = z_s[c // 2, g - 1].T
                            zt_s[g - 1] = zt[2 * G:]
                        else:
                            zt = zt_s[g - 1]
                        for r in range(2):
                            zr = zt[r * G:(r + 1) * G]
                            if 2 * c + r < NS_T - 1:
                                x = jnp.where(lane_g < g * G, side_s[2 * c + r, g - 1], zr)
                            else:
                                x = jnp.where(row_g + g * G <= lane_g, zr, _NEG)
                            st[0, r * _T + g * G:r * _T + (g + 1) * G, _T:] = x
                            fix.append(x)
                    m = _cat([m[:, :_T], jnp.maximum(m[:, _T:], _colmax(_cat(fix, axis=0)))])
                if c > 0:
                    m0, l0, o0 = state[j]
                    m = jnp.maximum(m0, m)
                    alpha = jnp.exp2(m0 - m)
                if c < j:
                    p = jnp.exp2(st[0] - m)
                    l = jnp.sum(p, axis=0, keepdims=True)
                    o = _mm(_cat([_ld(vT_s, 2 * c), _ld(vT_s, 2 * c + 1)]), p.astype(BF16))
                else:
                    p = jnp.exp2(st[0, 0:_T, :] - m)
                    p2 = jnp.exp2(st[0, _T:, _T:] - m[:, _T:])
                    l = jnp.sum(p, axis=0, keepdims=True)
                    l = _cat([l[:, :_T], l[:, _T:] + jnp.sum(p2, axis=0, keepdims=True)])
                    p, p2 = p.astype(BF16), p2.astype(BF16)
                    o = _cat([_mm(_ld(vT_s, 2 * c, rows=(r, D // 2)), p)
                              for r in range(0, D, D // 2)], axis=0)
                    o2 = _cat([_mm(_ld(vT_s, 2 * c + 1, rows=(r, D // 4)), p2)
                               for r in range(0, D, D // 4)], axis=0)
                    o = _cat([o[:, :_T], o[:, _T:] + o2])
                l = jnp.where(o[0:1] != o[0:1], o[0:1], l)
                if c > 0:
                    l = l0 * alpha + l
                    o = o0 * alpha + o
                state[j] = (m, l, o)
                if c == j:
                    ctx = o * (1.0 / l)
                    for t in range(2):
                        qc_s[h, 2 * j + t] = ctx[:, t * _T:(t + 1) * _T].astype(BF16)

            for i in range(len(items) + _LAG):
                if i < len(items):
                    qk(i)
                    j, c = items[i]
                    fill = [(proj_v, j, 0), (proj_k, j + 1, 0), (proj_v, j, 1), (proj_k, j + 1, 1)]
                    if j < NB - 1:
                        for pc in fill[len(fill) * c // (j + 1):len(fill) * (c + 1) // (j + 1)]:
                            piece(*pc)
                elif i - len(items) in (0, 3):
                    piece(proj_v, NB - 1, (i - len(items)) // 3)
                if i >= _LAG:
                    pv(i - _LAG)

            return carry

        def run_heads():
            lax.fori_loop(0, H, head, 0)
            wait(group('wo'))

        def phase_o(j, carry):
            pl.when(j >= 2)(lambda: wait(o_cp(j - 2)))
            c0 = pl.multiple_of(j * _B, _B)
            a = None
            for hh in range(0, H, 2):
                w2 = _cat([_ld(woT_s, t, hh + u) for u in range(2) for t in range(ND_T)])
                x2 = _cat([_cat([_ld(qc_s, hh + u, 2 * j), _ld(qc_s, hh + u, 2 * j + 1)])
                           for u in range(2)], axis=0)
                part = _mm(w2, x2)
                a = part if a is None else a + part
            g = g_s[:, pl.ds(c0, _B)]
            rs = _sigmoid(r_s[:, pl.ds(c0, _B)])
            col = lax.broadcasted_iota(I32, (1, _B), 1) + j * _B
            upd = jnp.where(col == idx_s[0], _cat([y_s[0], y_s[0]]),
                            jnp.where(col == idx_s[1], _cat([y_s[1], y_s[1]]), 0.0))
            b = _cat([xT_s[2 * j], xT_s[2 * j + 1]]).astype(F32) + upd * rs
            o_s[j & 1] = (g * a + (1.0 - g) * b).astype(BF16)
            start(o_cp(j))
            return carry

        def run_o():
            lax.fori_loop(0, NB, phase_o, 0)

        def stage(k, carry):
            for i, fn in enumerate((run_pre, run_heads, run_o)):
                pl.when(k == i)(fn)
            return carry

        lax.fori_loop(0, 3, stage, 0)
        wait(o_cp(NB - 2) + o_cp(NB - 1))

    return kernel


@jax.jit
def pallas_gated_mix__compressed_kv_cla__moe_arch_mod__prompt_kernel(
    A_x: jax.Array,
    A_c_kv: jax.Array,
    A_w_q: jax.Array,
    A_w_uk: jax.Array,
    A_w_uv: jax.Array,
    A_w_o: jax.Array,
    B_x: jax.Array,
    B_w_r: jax.Array,
    B_w_gate: jax.Array,
    B_w_up: jax.Array,
    B_w_down: jax.Array,
    gate_w: jax.Array,
):
    _, S, M = A_x.shape
    C = A_c_kv.shape[2]
    H, D = A_w_q.shape[1], A_w_q.shape[2]
    FF = B_w_gate.shape[1]
    xT = A_x[0].T
    woT = jnp.transpose(A_w_o, (0, 2, 1))
    wdT = B_w_down.T
    any_spec = pl.BlockSpec(memory_space=pl.ANY)
    V = pltpu.VMEM
    outT = pl.pallas_call(
        _make_kernel(S, M, C, H, D, FF),
        in_specs=[any_spec] * 11,
        out_specs=any_spec,
        out_shape=jax.ShapeDtypeStruct((M, S), BF16),
        scratch_shapes=[
            V((H, S // _T, D, _T), BF16),
            V((H // 2, M, D), U32), V((H // 2, C, D), U32), V((H // 2, C, D), U32),
            V((S // _T, M, _T), BF16), V((2, M, _B), BF16),
            V((C // _T, S, _T), BF16), V((D // _T, H, M, _T), BF16),
            V((M, FF), BF16), V((M, FF), BF16), V((M, FF), BF16),
            [V((pl.cdiv(M, _T), 2 * D, _T), BF16)] * 2, V((D // _T, C, _T), BF16),
            V((C // _T, D, _T), BF16),
            V((D // _T, S, _T), BF16), V((S // _T, D, _T), BF16), V((2, M, _T), F32),
            [V((1, _B, _B), F32)] * _NS,
            V((S // _T // _NG, _NG - 1, _T, _T), F32), V((_NG - 1, 2 * _G, _T), F32),
            V((S // _T, _NG - 1, _G, _T), F32), V((D // _T, _T, _T), BF16),
            V((2, M, _T), F32),
            V((1, S), F32), V((1, S), F32), V((M,), BF16), V((M,), BF16),
            pltpu.SMEM((3,), I32),
            pltpu.SemaphoreType.DMA((7,)), pltpu.SemaphoreType.DMA((H // 2,)),
            pltpu.SemaphoreType.DMA(()), pltpu.SemaphoreType.DMA((2,)),
        ],
        compiler_params=pltpu.CompilerParams(vmem_limit_bytes=100 << 20),
    )(xT, A_c_kv[0], A_w_q, A_w_uk, A_w_uv, woT, B_w_r, gate_w, B_w_gate, B_w_up, wdT)
    return outT.T[None]
```

```python
import math

import jax
import jax.numpy as jnp
from jax import lax
import jax.experimental.pallas as pl
import jax.experimental.pallas.tpu as pltpu

F32, BF16, U32, I32 = jnp.float32, jnp.bfloat16, jnp.uint32, jnp.int32
_NT = (((1,), (1,)), ((), ()))
_NEG = -1e30
_HI = 0xFFFF0000
_T = 128
_B = 256
_LAG = 5
_NS = 7
_NG = 4
_G = _T // _NG
_XA, _XB = 2, 7


def _mm(a, b):
    return jnp.dot(a, b, preferred_element_type=F32)


def _mm_nt(a, b):
    return lax.dot_general(a, b, _NT, preferred_element_type=F32)


def _sigmoid(x):
    return 1.0 / (1.0 + jnp.exp(-x))


def _as_f32(u):
    return lax.bitcast_convert_type(u, F32)


def _cat(parts, axis=1):
    return parts[0] if len(parts) == 1 else jnp.concatenate(parts, axis=axis)


def _colmax(x):
    return jnp.max(x, axis=0, keepdims=True)


def _ld(ref, *lead, rows=None):
    u = ref.bitcast(U32)
    idx = lead if rows is None else lead + (slice(rows[0] // 2, (rows[0] + rows[1]) // 2),)
    return pltpu.bitcast(u[idx], BF16)


def _make_kernel(S, M, C, H, D, FF):
    NB, NP = S // _B, H // 2
    NS_T, NC_T, ND_T, NF_T = S // _T, C // _T, D // _T, FF // _T
    MF, MR = M // _T, M % _T
    assert ND_T == 2 and MR > 0 and _NS > _LAG >= 1 and _NG == 4 and NB % 2 == 0
    q_scale = math.log2(math.e) * (D ** -0.5)

    def kernel(xT_hbm, c_hbm, wq_hbm, wk_hbm, wv_hbm, woT_hbm, wr_hbm, gw_hbm,
               wg_hbm, wu_hbm, wdT_hbm, o_hbm,
               qc_s, wq_buf, wk_buf, wv_buf, xT_s, o_s, c_s, woT_s, wg_s, wu_s, wdT_s,
               wqT_s, wk_s, wvT_s, k_s, vT_s, y_s, s_s, z_s, zt_s, side_s, qn_s, wc_s,
               g_s, r_s, wr_s, gw_s, idx_s,
               sem, q_sem, kv_sem, o_sem):
        def tiled(src, dst, n):
            return [(src.at[..., t * _T:(t + 1) * _T], dst.at[t]) for t in range(n)]

        xt = tiled(xT_hbm, xT_s, NS_T)
        groups = dict(w=[(wr_hbm, wr_s), (gw_hbm, gw_s)], xa=xt[:_XA], xb=xt[_XA:_XB], xc=xt[_XB:],
                      ffn=[(wg_hbm, wg_s), (wu_hbm, wu_s), (wdT_hbm, wdT_s)],
                      c=tiled(c_hbm, c_s, NC_T), wo=tiled(woT_hbm, woT_s, ND_T))

        def group(name):
            s = sem.at[list(groups).index(name)]
            return [pltpu.make_async_copy(src, dst, s) for src, dst in groups[name]]

        def q_cp(p):
            return [pltpu.make_async_copy(wq_hbm.bitcast(U32).at[:, p, :], wq_buf.at[p], q_sem.at[p])]

        def kv_cp(p):
            return [pltpu.make_async_copy(src.bitcast(U32).at[:, p, :], dst.at[p], kv_sem.at[jnp.minimum(p, 1)])
                    for src, dst in ((wk_hbm, wk_buf), (wv_hbm, wv_buf))]

        def o_cp(j):
            c0 = pl.multiple_of(j * _B, _B)
            return [pltpu.make_async_copy(o_s.at[j & 1], o_hbm.at[:, pl.ds(c0, _B)], o_sem.at[j & 1])]

        def start(cps):
            for d in cps:
                d.start()

        def wait(cps):
            for d in cps:
                d.wait()

        def prep_q(p, b):
            w = wq_buf[p].T
            for half, u in enumerate((w << 16, w & jnp.uint32(_HI))):
                wb = _as_f32(u)
                for t in range(MF):
                    wqT_s[b][t, half * D:(half + 1) * D, :] = wb[:, t * _T:(t + 1) * _T].astype(BF16)
                wqT_s[b][MF, half * D:(half + 1) * D, 0:MR] = wb[:, MF * _T:].astype(BF16)

        def q_tile(p, t, b):
            wqT = _cat([_ld(wqT_s[b], u) for u in range(MF)] + [_ld(wqT_s[b], MF)[:, 0:MR]])
            q = _mm(wqT, _ld(xT_s, t)) * q_scale
            qc_s[2 * p, t] = q[:D].astype(BF16)
            qc_s[2 * p + 1, t] = q[D:].astype(BF16)

        def q_first(t0, t1):
            for t in range(t0, t1):
                q_tile(0, t, 0)
                xf = xT_s[t].astype(F32)
                r0, r1 = [jnp.sum(xf * wc_s[n], axis=0, keepdims=True) for n in range(2)]
                r_s[:, t * _T:(t + 1) * _T] = r0.astype(BF16).astype(F32)
                g_s[:, t * _T:(t + 1) * _T] = _sigmoid(r1)

        def prep_wk0(hh):
            sh = jnp.asarray((1 - (hh & 1)) * 16).astype(U32)
            wk_s[0][0] = _as_f32((wk_buf[hh >> 1, :, 0:_T] << sh) & jnp.uint32(_HI)).astype(BF16)

        def run_pre():
            start(group('w') + q_cp(0) + group('xa') + group('xb') + group('xc'))
            pl.loop(1, NP)(lambda p: start(q_cp(p)))
            start(group('ffn') + group('c'))
            pl.loop(0, NP)(lambda p: start(kv_cp(p)))
            start(group('wo'))
            for b in range(2):
                wqT_s[b][MF] = jnp.zeros((2 * D, _T), BF16)
            idx_s[2] = 0
            wait(group('w'))
            for n, ref in enumerate((wr_s, gw_s)):
                wc_s[n] = jnp.broadcast_to(ref[...].astype(F32).reshape(1, M), (_T, M)).T
            wait(q_cp(0))
            prep_q(0, 0)
            wait(group('xa'))
            q_first(0, _XA)
            wait(group('xb'))
            q_first(_XA, _XB)
            wait(group('xc') + q_cp(1))
            prep_q(1, 1)
            q_first(_XB, NS_T)
            wait(q_cp(2) + q_cp(3))

            def phase_q(i, carry):
                p = 2 * i + 1
                prep_q(p + 1, 0)
                for t in range(NS_T):
                    q_tile(p, t, 1)
                prep_q(p + 2, 1)
                for t in range(NS_T):
                    q_tile(p + 1, t, 0)
                pl.when(p + 4 < NP)(lambda: wait(q_cp(p + 3) + q_cp(p + 4)))
                return carry

            lax.fori_loop(0, (NP - 2) // 2, phase_q, 0)
            wait(group('ffn') + kv_cp(0))

            lane = lax.broadcasted_iota(I32, (1, S), 1)
            idxs, cur = [], r_s[...]
            for n in range(2):
                mx = jnp.max(cur, axis=1, keepdims=True)
                ii = jnp.min(jnp.where(cur == mx, lane, S - 1))
                idxs.append(ii)
                idx_s[n] = ii
                cur = jnp.where(lane == ii, -jnp.inf, cur)
            ffn = {}

            def ffn_select(n):
                row16 = lax.broadcasted_iota(I32, (16, _T), 0)
                lane16 = lax.broadcasted_iota(I32, (16, _T), 1)
                oh = jnp.logical_and(row16 == n, lane16 == (idxs[n] & (_T - 1)))
                xr = _mm_nt(jnp.where(oh, 1.0, 0.0).astype(BF16), _ld(xT_s, idxs[n] // _T))
                ffn['x'] = xr if n == 0 else (ffn['x'] + xr).astype(BF16)

            def ffn_gate(f):
                ffn['g', f] = _mm(ffn['x'], wg_s[:, f * _T:(f + 1) * _T])

            def ffn_up(f):
                gt = ffn['g', f]
                ffn[f] = (gt * _sigmoid(gt) * _mm(ffn['x'], wu_s[:, f * _T:(f + 1) * _T])).astype(BF16)

            def ffn_down(f):
                y = _mm_nt(ffn[f], wdT_s[:, f * _T:(f + 1) * _T])
                ffn['y'] = y if 'y' not in ffn else ffn['y'] + y

            plain = [(fn, f) for f in range(NF_T) for fn in (ffn_gate, ffn_up)]
            after = {5: [(ffn_select, 0)], 6: [(ffn_select, 1)]}
            gap, nd, ready = 7, 0, {}
            while plain or nd < NF_T:
                slot = []
                if nd < NF_T and ready.get(nd, gap) < gap:
                    slot.append((ffn_down, nd))
                    nd += 1
                while len(slot) < 2 and plain:
                    fn, f = plain.pop(0)
                    slot.append((fn, f))
                    if fn is ffn_up:
                        ready[f] = gap
                after[gap] = slot
                gap += 1
            assert gap <= 2 * NS_T - 1, gap
            for t in range(NS_T):
                if 2 * t in after:
                    for half in range(2):
                        w = _cat([_ld(wqT_s[1], u, rows=(half * D, D)) for u in range(MF)]
                                 + [_ld(wqT_s[1], MF, rows=(half * D, D))[:, 0:MR]])
                        qc_s[2 * (NP - 1) + half, t] = (_mm(w, _ld(xT_s, t)) * q_scale).astype(BF16)
                        for fn, f in after.get(2 * t + half, []):
                            fn(f)
                else:
                    q_tile(NP - 1, t, 1)
                    for fn, f in after.get(2 * t + 1, []):
                        fn(f)
            yp = jnp.concatenate([ffn['y'], jnp.zeros((16, (MF + 1) * _T - M), F32)], axis=1)
            yT = jnp.concatenate([yp, jnp.zeros((_T - 16, (MF + 1) * _T), F32)], axis=0).T[:M]
            for n in range(2):
                y_s[n] = jnp.broadcast_to(yT[:, n:n + 1], (M, _T))

            prep_wk0(0)

            zero = idx_s[2]
            for ref in s_s:
                ref[zero, 0:8, :] = jnp.zeros((8, _B), F32)
            z_s[...] = jnp.zeros(z_s.shape, F32)
            z_s[zero, 0, 0:8, :] = jnp.zeros((8, _T), F32)
            side_s[zero, 0, 0:8, :] = jnp.zeros((8, _T), F32)
            zt_s[zero, 0:8, :] = jnp.zeros((8, _T), F32)
            wait(group('c'))
            pl.loop(1, NP)(lambda p: wait(kv_cp(p)))

        def head(h, carry):
            slot = h >> 1
            sh = ((1 - (h & 1)) * 16).astype(U32)
            wk = _as_f32((wk_buf[slot, :, _T:] << sh) & jnp.uint32(_HI))
            wk_s[1][0] = wk.astype(BF16)
            wvT = _as_f32((wv_buf[slot] << sh) & jnp.uint32(_HI)).T.astype(BF16)
            for t in range(NC_T):
                wvT_s[t] = wvT[:, t * _T:(t + 1) * _T]
            tri = (lax.broadcasted_iota(I32, (_T, _T), 0) <= lax.broadcasted_iota(I32, (_T, _T), 1))
            G, NG, q_u = _G, _NG, qc_s.bitcast(U32)
            lane_t = lax.broadcasted_iota(I32, (_T, _T), 1)
            row_g = lax.broadcasted_iota(I32, (G, _T), 0)
            lane_g = lax.broadcasted_iota(I32, (G, _T), 1)
            qn = _ld(qc_s, h, NS_T - 1).astype(F32).T
            for t in range(ND_T):
                qn_s[t] = qn[:, t * _T:(t + 1) * _T].astype(BF16)

            def c_rows(r0, n):
                return _cat([_ld(c_s, t, rows=(r0, n)) for t in range(NC_T)])

            def k_rows(r0, n):
                return _cat([_ld(k_s, t, rows=(r0, n)) for t in range(ND_T)])

            def proj_k(j, t):
                w = wk if (j, t) == (0, 1) else _ld(wk_s[t], 0)
                k_s[t, j * _B:(j + 1) * _B, :] = _mm(c_rows(j * _B, _B), w).astype(BF16)

            def proj_v(j, t):
                w = wvT if (j, t) == (0, 0) else _cat([_ld(wvT_s, u) for u in range(NC_T)])
                vT_s[2 * j + t] = _mm_nt(w, c_rows(j * _B + t * _T, _T)).astype(BF16)

            done = set()

            def piece(fn, j, t):
                if j < NB and (fn, j, t) not in done:
                    done.add((fn, j, t))
                    fn(j, t)

            items = [(j, c) for j in range(NB) for c in range(j + 1)]
            state, cmax = {}, {}

            def qk(i):
                j, c = items[i]
                for t in range(2):
                    piece(proj_k, c, t)
                k0, st = c * _B, s_s[i % _NS]
                q0u, q1u = q_u[h, 2 * j], q_u[h, 2 * j + 1]
                q0, q1 = pltpu.bitcast(q0u, BF16), pltpu.bitcast(q1u, BF16)
                q = _cat([q0, q1])

                def diag(r0, qu, g):
                    w = jnp.where(lane_t < g * G, q_u[h, NS_T - 1], qu) if g else qu
                    return _mm(k_rows(k0 + r0 + g * G, G), pltpu.bitcast(w, BF16))

                def z_parts():
                    u = c // 2
                    assert (proj_k, 2 * u + 1, 1) in done
                    for g in (1,) if c % 2 == 0 else (2, 3):
                        kg = _cat([k_rows((NG * u + p) * _T + g * G, G) for p in range(NG)], axis=0)
                        qg = _cat([_ld(qn_s, t, rows=(g * G, _T - g * G)) for t in range(ND_T)])
                        z_s[u, g - 1, g * G:, :] = _mm_nt(qg, kg)

                if c < j < NB - 1:
                    s = _mm(k_rows(k0, _B), q)
                    st[0] = s
                    cmax[i] = _colmax(s)
                elif c < j:
                    n1 = (_B + 5 * G) // 2
                    sa = _mm(k_rows(k0, n1), q0)
                    z_parts()
                    sb = _mm(k_rows(k0 + n1, _B - n1), q0)
                    su = _mm(_cat([k_rows(k0, G), k_rows(k0 + _T, G)], axis=0), q1)
                    s0 = _cat([sa, sb], axis=0)
                    st[0, :, 0:_T] = s0
                    st[0, 0:G, _T:] = su[:G]
                    st[0, _T:_T + G, _T:] = su[G:]
                    cmax[i] = _cat([_colmax(s0), _colmax(su)])
                elif j < NB - 1:
                    sab = _mm(k_rows(k0, _T), q1)
                    sa = [diag(0, q0u, g) for g in range(NG)]
                    sb = [diag(_T, q1u, g) for g in range(NG)]
                    for g in range(1, NG):
                        side_s[2 * j, g - 1] = sa[g]
                        side_s[2 * j + 1, g - 1] = sb[g]
                    s = _cat([jnp.where(tri, _cat(sa, axis=0), _NEG), sab])
                    s2 = jnp.where(tri, _cat(sb, axis=0), _NEG)
                    st[0, 0:_T, :] = s
                    st[0, _T:, _T:] = s2
                    m = _colmax(s)
                    cmax[i] = _cat([m[:, :_T], jnp.maximum(m[:, _T:], _colmax(s2))])
                else:
                    z_parts()
                    sa = [diag(0, q0u, 1)]
                    s_a0 = _mm(k_rows(k0, G), q)
                    sa += [diag(0, q0u, g) for g in range(2, NG)]
                    s_b0 = _cat([_mm(k_rows(k0 + _T + r, G // 2), q1) for r in (0, G // 2)], axis=0)
                    for g in range(1, NG):
                        side_s[2 * j, g - 1] = sa[g - 1]
                    s0 = jnp.where(tri, _cat([s_a0[:, :_T]] + sa, axis=0), _NEG)
                    s_b0 = jnp.where(row_g <= lane_g, s_b0, _NEG)
                    st[0, 0:_T, 0:_T] = s0
                    st[0, 0:G, _T:] = s_a0[:, _T:]
                    st[0, _T:_T + G, _T:] = s_b0
                    cmax[i] = _cat([_colmax(s0), jnp.maximum(_colmax(s_a0[:, _T:]), _colmax(s_b0))])

            def pv(i):
                j, c = items[i]
                for t in range(2):
                    piece(proj_v, c, t)
                st, m = s_s[i % _NS], cmax.pop(i)
                if j == NB - 1:
                    fix = []
                    for g in range(1, NG):
                        if c % 2 == 0:
                            zt = z_s[c // 2, g - 1].T
                            zt_s[g - 1] = zt[2 * G:]
                        else:
                            zt = zt_s[g - 1]
                        for r in range(2):
                            zr = zt[r * G:(r + 1) * G]
                            if 2 * c + r < NS_T - 1:
                                x = jnp.where(lane_g < g * G, side_s[2 * c + r, g - 1], zr)
                            else:
                                x = jnp.where(row_g + g * G <= lane_g, zr, _NEG)
                            st[0, r * _T + g * G:r * _T + (g + 1) * G, _T:] = x
                            fix.append(x)
                    m = _cat([m[:, :_T], jnp.maximum(m[:, _T:], _colmax(_cat(fix, axis=0)))])
                if c > 0:
                    m0, l0, o0 = state[j]
                    m = jnp.maximum(m0, m)
                    alpha = jnp.exp2(m0 - m)
                if c < j:
                    p = jnp.exp2(st[0] - m)
                    l = jnp.sum(p, axis=0, keepdims=True)
                    o = _mm(_cat([_ld(vT_s, 2 * c), _ld(vT_s, 2 * c + 1)]), p.astype(BF16))
                else:
                    p = jnp.exp2(st[0, 0:_T, :] - m)
                    p2 = jnp.exp2(st[0, _T:, _T:] - m[:, _T:])
                    l = jnp.sum(p, axis=0, keepdims=True)
                    l = _cat([l[:, :_T], l[:, _T:] + jnp.sum(p2, axis=0, keepdims=True)])
                    p, p2 = p.astype(BF16), p2.astype(BF16)
                    o = _cat([_mm(_ld(vT_s, 2 * c, rows=(r, D // 2)), p)
                              for r in range(0, D, D // 2)], axis=0)
                    o2 = _cat([_mm(_ld(vT_s, 2 * c + 1, rows=(r, D // 4)), p2)
                               for r in range(0, D, D // 4)], axis=0)
                    o = _cat([o[:, :_T], o[:, _T:] + o2])
                l = jnp.where(o[0:1] != o[0:1], o[0:1], l)
                if c > 0:
                    l = l0 * alpha + l
                    o = o0 * alpha + o
                state[j] = (m, l, o)
                if c == j:
                    ctx = o * (1.0 / l)
                    for t in range(2):
                        qc_s[h, 2 * j + t] = ctx[:, t * _T:(t + 1) * _T].astype(BF16)

            for i in range(len(items) + _LAG):
                if i < len(items):
                    qk(i)
                    j, c = items[i]
                    fill = [(proj_v, j, 0), (proj_k, j + 1, 0), (proj_v, j, 1), (proj_k, j + 1, 1)]
                    if j < NB - 1:
                        for pc in fill[len(fill) * c // (j + 1):len(fill) * (c + 1) // (j + 1)]:
                            piece(*pc)
                elif i - len(items) in (0, 3):
                    piece(proj_v, NB - 1, (i - len(items)) // 3)
                if i >= _LAG:
                    pv(i - _LAG)
            prep_wk0(jnp.minimum(h + 1, H - 1))
            return carry

        def run_heads():
            lax.fori_loop(0, H, head, 0)
            wait(group('wo'))

        def phase_o(j, carry):
            pl.when(j >= 2)(lambda: wait(o_cp(j - 2)))
            c0 = pl.multiple_of(j * _B, _B)
            a = None
            for hh in range(0, H, 2):
                w2 = _cat([_ld(woT_s, t, hh + u) for u in range(2) for t in range(ND_T)])
                x2 = _cat([_cat([_ld(qc_s, hh + u, 2 * j), _ld(qc_s, hh + u, 2 * j + 1)])
                           for u in range(2)], axis=0)
                part = _mm(w2, x2)
                a = part if a is None else a + part
            g = g_s[:, pl.ds(c0, _B)]
            rs = _sigmoid(r_s[:, pl.ds(c0, _B)])
            col = lax.broadcasted_iota(I32, (1, _B), 1) + j * _B
            upd = jnp.where(col == idx_s[0], _cat([y_s[0], y_s[0]]),
                            jnp.where(col == idx_s[1], _cat([y_s[1], y_s[1]]), 0.0))
            b = _cat([xT_s[2 * j], xT_s[2 * j + 1]]).astype(F32) + upd * rs
            o_s[j & 1] = (g * a + (1.0 - g) * b).astype(BF16)
            start(o_cp(j))
            return carry

        def run_o():
            lax.fori_loop(0, NB, phase_o, 0)

        def stage(k, carry):
            for i, fn in enumerate((run_pre, run_heads, run_o)):
                pl.when(k == i)(fn)
            return carry

        lax.fori_loop(0, 3, stage, 0)
        wait(o_cp(NB - 2) + o_cp(NB - 1))

    return kernel


@jax.jit
def pallas_gated_mix__compressed_kv_cla__moe_arch_mod__prompt_kernel(
    A_x: jax.Array,
    A_c_kv: jax.Array,
    A_w_q: jax.Array,
    A_w_uk: jax.Array,
    A_w_uv: jax.Array,
    A_w_o: jax.Array,
    B_x: jax.Array,
    B_w_r: jax.Array,
    B_w_gate: jax.Array,
    B_w_up: jax.Array,
    B_w_down: jax.Array,
    gate_w: jax.Array,
):
    _, S, M = A_x.shape
    C = A_c_kv.shape[2]
    H, D = A_w_q.shape[1], A_w_q.shape[2]
    FF = B_w_gate.shape[1]
    xT = A_x[0].T
    woT = jnp.transpose(A_w_o, (0, 2, 1))
    wdT = B_w_down.T
    any_spec = pl.BlockSpec(memory_space=pl.ANY)
    V = pltpu.VMEM
    outT = pl.pallas_call(
        _make_kernel(S, M, C, H, D, FF),
        in_specs=[any_spec] * 11,
        out_specs=any_spec,
        out_shape=jax.ShapeDtypeStruct((M, S), BF16),
        scratch_shapes=[
            V((H, S // _T, D, _T), BF16),
            V((H // 2, M, D), U32), V((H // 2, C, D), U32), V((H // 2, C, D), U32),
            V((S // _T, M, _T), BF16), V((2, M, _B), BF16),
            V((C // _T, S, _T), BF16), V((D // _T, H, M, _T), BF16),
            V((M, FF), BF16), V((M, FF), BF16), V((M, FF), BF16),
            [V((pl.cdiv(M, _T), 2 * D, _T), BF16)] * 2, [V((1, C, _T), BF16)] * 2,
            V((C // _T, D, _T), BF16),
            V((D // _T, S, _T), BF16), V((S // _T, D, _T), BF16), V((2, M, _T), F32),
            [V((1, _B, _B), F32)] * _NS,
            V((S // _T // _NG, _NG - 1, _T, _T), F32), V((_NG - 1, 2 * _G, _T), F32),
            V((S // _T, _NG - 1, _G, _T), F32), V((D // _T, _T, _T), BF16),
            V((2, M, _T), F32),
            V((1, S), F32), V((1, S), F32), V((M,), BF16), V((M,), BF16),
            pltpu.SMEM((3,), I32),
            pltpu.SemaphoreType.DMA((7,)), pltpu.SemaphoreType.DMA((H // 2,)),
            pltpu.SemaphoreType.DMA((2,)), pltpu.SemaphoreType.DMA((2,)),
        ],
        compiler_params=pltpu.CompilerParams(vmem_limit_bytes=100 << 20),
    )(xT, A_c_kv[0], A_w_q, A_w_uk, A_w_uv, woT, B_w_r, gate_w, B_w_gate, B_w_up, wdT)
    return outT.T[None]
```

```python
import math

import jax
import jax.numpy as jnp
from jax import lax
import jax.experimental.pallas as pl
import jax.experimental.pallas.tpu as pltpu

F32, BF16, U32, I32 = jnp.float32, jnp.bfloat16, jnp.uint32, jnp.int32
_NT = (((1,), (1,)), ((), ()))
_NEG = -1e30
_HI = 0xFFFF0000
_T = 128
_B = 256
_LAG = 5
_NS = 7
_NG = 4
_G = _T // _NG
_XA, _XB = 2, 7


def _mm(a, b):
    return jnp.dot(a, b, preferred_element_type=F32)


def _mm_nt(a, b):
    return lax.dot_general(a, b, _NT, preferred_element_type=F32)


def _sigmoid(x):
    return 1.0 / (1.0 + jnp.exp(-x))


def _as_f32(u):
    return lax.bitcast_convert_type(u, F32)


def _cat(parts, axis=1):
    return parts[0] if len(parts) == 1 else jnp.concatenate(parts, axis=axis)


def _colmax(x):
    return jnp.max(x, axis=0, keepdims=True)


def _ld(ref, *lead, rows=None):
    u = ref.bitcast(U32)
    idx = lead if rows is None else lead + (slice(rows[0] // 2, (rows[0] + rows[1]) // 2),)
    return pltpu.bitcast(u[idx], BF16)


def _make_kernel(S, M, C, H, D, FF):
    NB, NP = S // _B, H // 2
    NS_T, NC_T, ND_T, NF_T = S // _T, C // _T, D // _T, FF // _T
    MF, MR = M // _T, M % _T
    assert ND_T == 2 and MR > 0 and _NS > _LAG >= 1 and _NG == 4 and NB % 2 == 0
    q_scale = math.log2(math.e) * (D ** -0.5)

    def kernel(xT_hbm, c_hbm, wq_hbm, wk_hbm, wv_hbm, woT_hbm, wr_hbm, gw_hbm,
               wg_hbm, wu_hbm, wdT_hbm, o_hbm,
               qc_s, wq_buf, wk_buf, wv_buf, xT_s, o_s, c_s, woT_s, wg_s, wu_s, wdT_s,
               wqT_s, wk_s, wvT_s, k_s, vT_s, y_s, s_s, z_s, zt_s, side_s, qn_s, wc_s,
               g_s, r_s, wr_s, gw_s, idx_s,
               sem, q_sem, kv_sem, o_sem):
        def tiled(src, dst, n):
            return [(src.at[..., t * _T:(t + 1) * _T], dst.at[t]) for t in range(n)]

        xt = tiled(xT_hbm, xT_s, NS_T)
        groups = dict(w=[(wr_hbm, wr_s), (gw_hbm, gw_s)], xa=xt[:_XA], xb=xt[_XA:_XB], xc=xt[_XB:],
                      ffn=[(wg_hbm, wg_s), (wu_hbm, wu_s), (wdT_hbm, wdT_s)],
                      c=tiled(c_hbm, c_s, NC_T), wo=tiled(woT_hbm, woT_s, ND_T))

        def group(name):
            s = sem.at[list(groups).index(name)]
            return [pltpu.make_async_copy(src, dst, s) for src, dst in groups[name]]

        def q_cp(p):
            return [pltpu.make_async_copy(wq_hbm.bitcast(U32).at[:, p, :], wq_buf.at[p], q_sem.at[p])]

        def kv_cp(p):
            return [pltpu.make_async_copy(src.bitcast(U32).at[:, p, :], dst.at[p], kv_sem.at[jnp.minimum(p, 1)])
                    for src, dst in ((wk_hbm, wk_buf), (wv_hbm, wv_buf))]

        def o_cp(j):
            c0 = pl.multiple_of(j * _B, _B)
            return [pltpu.make_async_copy(o_s.at[j & 1], o_hbm.at[:, pl.ds(c0, _B)], o_sem.at[j & 1])]

        def start(cps):
            for d in cps:
                d.start()

        def wait(cps):
            for d in cps:
                d.wait()

        def prep_q(p, b):
            w = wq_buf[p].T
            for half, u in enumerate((w << 16, w & jnp.uint32(_HI))):
                wb = _as_f32(u)
                for t in range(MF):
                    wqT_s[b][t, half * D:(half + 1) * D, :] = wb[:, t * _T:(t + 1) * _T].astype(BF16)
                wqT_s[b][MF, half * D:(half + 1) * D, 0:MR] = wb[:, MF * _T:].astype(BF16)

        def q_tile(p, t, b):
            wqT = _cat([_ld(wqT_s[b], u) for u in range(MF)] + [_ld(wqT_s[b], MF)[:, 0:MR]])
            q = _mm(wqT, _ld(xT_s, t)) * q_scale
            qc_s[2 * p, t] = q[:D].astype(BF16)
            qc_s[2 * p + 1, t] = q[D:].astype(BF16)

        def q_first(t0, t1):
            for t in range(t0, t1):
                q_tile(0, t, 0)
                xf = xT_s[t].astype(F32)
                r0, r1 = [jnp.sum(xf * wc_s[n], axis=0, keepdims=True) for n in range(2)]
                r_s[:, t * _T:(t + 1) * _T] = r0.astype(BF16).astype(F32)
                g_s[:, t * _T:(t + 1) * _T] = _sigmoid(r1)

        def prep_wk0(hh):
            sh = jnp.asarray((1 - (hh & 1)) * 16).astype(U32)
            wk_s[0][0] = _as_f32((wk_buf[hh >> 1, :, 0:_T] << sh) & jnp.uint32(_HI)).astype(BF16)

        def run_pre():
            start(group('w') + q_cp(0) + group('xa') + group('xb') + group('xc'))
            pl.loop(1, NP)(lambda p: start(q_cp(p)))
            start(group('ffn') + group('c'))
            pl.loop(0, NP)(lambda p: start(kv_cp(p)))
            start(group('wo'))
            for b in range(2):
                wqT_s[b][MF] = jnp.zeros((2 * D, _T), BF16)
            idx_s[2] = 0
            wait(group('w'))
            for n, ref in enumerate((wr_s, gw_s)):
                wc_s[n] = jnp.broadcast_to(ref[...].astype(F32).reshape(1, M), (_T, M)).T
            wait(q_cp(0))
            prep_q(0, 0)
            wait(group('xa'))
            q_first(0, _XA)
            wait(group('xb'))
            q_first(_XA, _XB)
            wait(group('xc') + q_cp(1))
            prep_q(1, 1)
            q_first(_XB, NS_T)
            wait(q_cp(2) + q_cp(3))

            def phase_q(i, carry):
                p = 2 * i + 1
                prep_q(p + 1, 0)
                for t in range(NS_T):
                    q_tile(p, t, 1)
                prep_q(p + 2, 1)
                for t in range(NS_T):
                    q_tile(p + 1, t, 0)
                pl.when(p + 4 < NP)(lambda: wait(q_cp(p + 3) + q_cp(p + 4)))
                return carry

            lax.fori_loop(0, (NP - 2) // 2, phase_q, 0)
            wait(group('ffn') + kv_cp(0))

            lane = lax.broadcasted_iota(I32, (1, S), 1)
            idxs, cur = [], r_s[...]
            for n in range(2):
                mx = jnp.max(cur, axis=1, keepdims=True)
                ii = jnp.min(jnp.where(cur == mx, lane, S - 1))
                idxs.append(ii)
                idx_s[n] = ii
                cur = jnp.where(lane == ii, -jnp.inf, cur)
            ffn = {}

            def ffn_select(n):
                row16 = lax.broadcasted_iota(I32, (16, _T), 0)
                lane16 = lax.broadcasted_iota(I32, (16, _T), 1)
                oh = jnp.logical_and(row16 == n, lane16 == (idxs[n] & (_T - 1)))
                xr = _mm_nt(jnp.where(oh, 1.0, 0.0).astype(BF16), _ld(xT_s, jnp.clip(idxs[n] // _T, 0, NS_T - 1)))
                ffn['x'] = xr if n == 0 else (ffn['x'] + xr).astype(BF16)

            def ffn_gate(f):
                ffn['g', f] = _mm(ffn['x'], wg_s[:, f * _T:(f + 1) * _T])

            def ffn_up(f):
                gt = ffn['g', f]
                ffn[f] = (gt * _sigmoid(gt) * _mm(ffn['x'], wu_s[:, f * _T:(f + 1) * _T])).astype(BF16)

            def ffn_down(f):
                y = _mm_nt(ffn[f], wdT_s[:, f * _T:(f + 1) * _T])
                ffn['y'] = y if 'y' not in ffn else ffn['y'] + y

            plain = [(fn, f) for f in range(NF_T) for fn in (ffn_gate, ffn_up)]
            after = {5: [(ffn_select, 0)], 6: [(ffn_select, 1)]}
            gap, nd, ready = 7, 0, {}
            while plain or nd < NF_T:
                slot = []
                if nd < NF_T and ready.get(nd, gap) < gap:
                    slot.append((ffn_down, nd))
                    nd += 1
                while len(slot) < 2 and plain:
                    fn, f = plain.pop(0)
                    slot.append((fn, f))
                    if fn is ffn_up:
                        ready[f] = gap
                after[gap] = slot
                gap += 1
            assert gap <= 2 * NS_T - 1, gap
            for t in range(NS_T):
                if 2 * t in after:
                    for half in range(2):
                        w = _cat([_ld(wqT_s[1], u, rows=(half * D, D)) for u in range(MF)]
                                 + [_ld(wqT_s[1], MF, rows=(half * D, D))[:, 0:MR]])
                        qc_s[2 * (NP - 1) + half, t] = (_mm(w, _ld(xT_s, t)) * q_scale).astype(BF16)
                        for fn, f in after.get(2 * t + half, []):
                            fn(f)
                else:
                    q_tile(NP - 1, t, 1)
                    for fn, f in after.get(2 * t + 1, []):
                        fn(f)
            yp = jnp.concatenate([ffn['y'], jnp.zeros((16, (MF + 1) * _T - M), F32)], axis=1)
            yT = jnp.concatenate([yp, jnp.zeros((_T - 16, (MF + 1) * _T), F32)], axis=0).T[:M]
            for n in range(2):
                y_s[n] = jnp.broadcast_to(yT[:, n:n + 1], (M, _T))

            prep_wk0(0)

            rows = pl.ds(pl.multiple_of(jnp.clip(idx_s[2], 0, 1) * 8, 8), 8)
            z_s[...] = jnp.zeros(z_s.shape, F32)
            for ref in list(s_s) + [z_s.at[0], side_s.at[0], zt_s]:
                ref[0, rows, :] = jnp.zeros((8, ref.shape[-1]), F32)
            wait(group('c'))
            pl.loop(1, NP)(lambda p: wait(kv_cp(p)))

        def head(h, carry):
            slot = h >> 1
            sh = ((1 - (h & 1)) * 16).astype(U32)
            wk = _as_f32((wk_buf[slot, :, _T:] << sh) & jnp.uint32(_HI))
            wk_s[1][0] = wk.astype(BF16)
            wvT = _as_f32((wv_buf[slot] << sh) & jnp.uint32(_HI)).T.astype(BF16)
            for t in range(NC_T):
                wvT_s[t] = wvT[:, t * _T:(t + 1) * _T]
            tri = (lax.broadcasted_iota(I32, (_T, _T), 0) <= lax.broadcasted_iota(I32, (_T, _T), 1))
            G, NG, q_u = _G, _NG, qc_s.bitcast(U32)
            lane_t = lax.broadcasted_iota(I32, (_T, _T), 1)
            row_g = lax.broadcasted_iota(I32, (G, _T), 0)
            lane_g = lax.broadcasted_iota(I32, (G, _T), 1)
            qn = _ld(qc_s, h, NS_T - 1).astype(F32).T
            for t in range(ND_T):
                qn_s[t] = qn[:, t * _T:(t + 1) * _T].astype(BF16)

            def c_rows(r0, n):
                return _cat([_ld(c_s, t, rows=(r0, n)) for t in range(NC_T)])

            def k_rows(r0, n):
                return _cat([_ld(k_s, t, rows=(r0, n)) for t in range(ND_T)])

            def proj_k(j, t):
                w = wk if (j, t) == (0, 1) else _ld(wk_s[t], 0)
                k_s[t, j * _B:(j + 1) * _B, :] = _mm(c_rows(j * _B, _B), w).astype(BF16)

            def proj_v(j, t):
                w = wvT if (j, t) == (0, 0) else _cat([_ld(wvT_s, u) for u in range(NC_T)])
                vT_s[2 * j + t] = _mm_nt(w, c_rows(j * _B + t * _T, _T)).astype(BF16)

            done = set()

            def piece(fn, j, t):
                if j < NB and (fn, j, t) not in done:
                    done.add((fn, j, t))
                    fn(j, t)

            items = [(j, c) for j in range(NB) for c in range(j + 1)]
            state, cmax = {}, {}

            def qk(i):
                j, c = items[i]
                for t in range(2):
                    piece(proj_k, c, t)
                k0, st = c * _B, s_s[i % _NS]
                q0u, q1u = q_u[h, 2 * j], q_u[h, 2 * j + 1]
                q0, q1 = pltpu.bitcast(q0u, BF16), pltpu.bitcast(q1u, BF16)
                q = _cat([q0, q1])

                def diag(r0, qu, g):
                    w = jnp.where(lane_t < g * G, q_u[h, NS_T - 1], qu) if g else qu
                    return _mm(k_rows(k0 + r0 + g * G, G), pltpu.bitcast(w, BF16))

                def z_parts():
                    u = c // 2
                    assert (proj_k, 2 * u + 1, 1) in done
                    for g in (1,) if c % 2 == 0 else (2, 3):
                        kg = _cat([k_rows((NG * u + p) * _T + g * G, G) for p in range(NG)], axis=0)
                        qg = _cat([_ld(qn_s, t, rows=(g * G, _T - g * G)) for t in range(ND_T)])
                        z_s[u, g - 1, g * G:, :] = _mm_nt(qg, kg)

                if c < j < NB - 1:
                    s = _mm(k_rows(k0, _B), q)
                    st[0] = s
                    cmax[i] = _colmax(s)
                elif c < j:
                    n1 = (_B + 5 * G) // 2
                    sa = _mm(k_rows(k0, n1), q0)
                    z_parts()
                    sb = _mm(k_rows(k0 + n1, _B - n1), q0)
                    su = _mm(_cat([k_rows(k0, G), k_rows(k0 + _T, G)], axis=0), q1)
                    s0 = _cat([sa, sb], axis=0)
                    st[0, :, 0:_T] = s0
                    st[0, 0:G, _T:] = su[:G]
                    st[0, _T:_T + G, _T:] = su[G:]
                    cmax[i] = _cat([_colmax(s0), _colmax(su)])
                elif j < NB - 1:
                    sab = _mm(k_rows(k0, _T), q1)
                    sa = [diag(0, q0u, g) for g in range(NG)]
                    sb = [diag(_T, q1u, g) for g in range(NG)]
                    for g in range(1, NG):
                        side_s[2 * j, g - 1] = sa[g]
                        side_s[2 * j + 1, g - 1] = sb[g]
                    s = _cat([jnp.where(tri, _cat(sa, axis=0), _NEG), sab])
                    s2 = jnp.where(tri, _cat(sb, axis=0), _NEG)
                    st[0, 0:_T, :] = s
                    st[0, _T:, _T:] = s2
                    m = _colmax(s)
                    cmax[i] = _cat([m[:, :_T], jnp.maximum(m[:, _T:], _colmax(s2))])
                else:
                    z_parts()
                    sa = [diag(0, q0u, 1)]
                    s_a0 = _mm(k_rows(k0, G), q)
                    sa += [diag(0, q0u, g) for g in range(2, NG)]
                    s_b0 = _cat([_mm(k_rows(k0 + _T + r, G // 2), q1) for r in (0, G // 2)], axis=0)
                    for g in range(1, NG):
                        side_s[2 * j, g - 1] = sa[g - 1]
                    s0 = jnp.where(tri, _cat([s_a0[:, :_T]] + sa, axis=0), _NEG)
                    s_b0 = jnp.where(row_g <= lane_g, s_b0, _NEG)
                    st[0, 0:_T, 0:_T] = s0
                    st[0, 0:G, _T:] = s_a0[:, _T:]
                    st[0, _T:_T + G, _T:] = s_b0
                    cmax[i] = _cat([_colmax(s0), jnp.maximum(_colmax(s_a0[:, _T:]), _colmax(s_b0))])

            def pv(i):
                j, c = items[i]
                for t in range(2):
                    piece(proj_v, c, t)
                st, m = s_s[i % _NS], cmax.pop(i)
                if j == NB - 1:
                    fix = []
                    for g in range(1, NG):
                        if c % 2 == 0:
                            zt = z_s[c // 2, g - 1].T
                            zt_s[g - 1] = zt[2 * G:]
                        else:
                            zt = zt_s[g - 1]
                        for r in range(2):
                            zr = zt[r * G:(r + 1) * G]
                            if 2 * c + r < NS_T - 1:
                                x = jnp.where(lane_g < g * G, side_s[2 * c + r, g - 1], zr)
                            else:
                                x = jnp.where(row_g + g * G <= lane_g, zr, _NEG)
                            st[0, r * _T + g * G:r * _T + (g + 1) * G, _T:] = x
                            fix.append(x)
                    m = _cat([m[:, :_T], jnp.maximum(m[:, _T:], _colmax(_cat(fix, axis=0)))])
                if c > 0:
                    m0, l0, o0 = state[j]
                    m = jnp.maximum(m0, m)
                    alpha = jnp.exp2(m0 - m)
                if c < j:
                    p = jnp.exp2(st[0] - m)
                    l = jnp.sum(p, axis=0, keepdims=True)
                    o = _mm(_cat([_ld(vT_s, 2 * c), _ld(vT_s, 2 * c + 1)]), p.astype(BF16))
                else:
                    p = jnp.exp2(st[0, 0:_T, :] - m)
                    p2 = jnp.exp2(st[0, _T:, _T:] - m[:, _T:])
                    l = jnp.sum(p, axis=0, keepdims=True)
                    l = _cat([l[:, :_T], l[:, _T:] + jnp.sum(p2, axis=0, keepdims=True)])
                    p, p2 = p.astype(BF16), p2.astype(BF16)
                    o = _cat([_mm(_ld(vT_s, 2 * c, rows=(r, D // 2)), p)
                              for r in range(0, D, D // 2)], axis=0)
                    o2 = _cat([_mm(_ld(vT_s, 2 * c + 1, rows=(r, D // 4)), p2)
                               for r in range(0, D, D // 4)], axis=0)
                    o = _cat([o[:, :_T], o[:, _T:] + o2])
                l = jnp.where(o[0:1] != o[0:1], o[0:1], l)
                if c > 0:
                    l = l0 * alpha + l
                    o = o0 * alpha + o
                state[j] = (m, l, o)
                if c == j:
                    ctx = o * (1.0 / l)
                    for t in range(2):
                        qc_s[h, 2 * j + t] = ctx[:, t * _T:(t + 1) * _T].astype(BF16)

            for i in range(len(items) + _LAG):
                if i < len(items):
                    qk(i)
                    j, c = items[i]
                    fill = [(proj_v, j, 0), (proj_k, j + 1, 0), (proj_v, j, 1), (proj_k, j + 1, 1)]
                    if j < NB - 1:
                        for pc in fill[len(fill) * c // (j + 1):len(fill) * (c + 1) // (j + 1)]:
                            piece(*pc)
                elif i - len(items) in (0, 3):
                    piece(proj_v, NB - 1, (i - len(items)) // 3)
                if i >= _LAG:
                    pv(i - _LAG)
            prep_wk0(jnp.minimum(h + 1, H - 1))
            return carry

        def run_heads():
            lax.fori_loop(0, H, head, 0)
            wait(group('wo'))

        def phase_o(j, carry):
            pl.when(j >= 2)(lambda: wait(o_cp(j - 2)))
            c0 = pl.multiple_of(j * _B, _B)
            a = None
            for hh in range(0, H, 2):
                w2 = _cat([_ld(woT_s, t, hh + u) for u in range(2) for t in range(ND_T)])
                x2 = _cat([_cat([_ld(qc_s, hh + u, 2 * j), _ld(qc_s, hh + u, 2 * j + 1)])
                           for u in range(2)], axis=0)
                part = _mm(w2, x2)
                a = part if a is None else a + part
            g = g_s[:, pl.ds(c0, _B)]
            rs = _sigmoid(r_s[:, pl.ds(c0, _B)])
            col = lax.broadcasted_iota(I32, (1, _B), 1) + j * _B
            upd = jnp.where(col == idx_s[0], _cat([y_s[0], y_s[0]]),
                            jnp.where(col == idx_s[1], _cat([y_s[1], y_s[1]]), 0.0))
            b = _cat([xT_s[2 * j], xT_s[2 * j + 1]]).astype(F32) + upd * rs
            o_s[j & 1] = (g * a + (1.0 - g) * b).astype(BF16)
            start(o_cp(j))
            return carry

        def run_o():
            lax.fori_loop(0, NB, phase_o, 0)

        def stage(k, carry):
            for i, fn in enumerate((run_pre, run_heads, run_o)):
                pl.when(k == i)(fn)
            return carry

        lax.fori_loop(0, 3, stage, 0)
        wait(o_cp(NB - 2) + o_cp(NB - 1))

    return kernel


@jax.jit
def pallas_gated_mix__compressed_kv_cla__moe_arch_mod__prompt_kernel(
    A_x: jax.Array,
    A_c_kv: jax.Array,
    A_w_q: jax.Array,
    A_w_uk: jax.Array,
    A_w_uv: jax.Array,
    A_w_o: jax.Array,
    B_x: jax.Array,
    B_w_r: jax.Array,
    B_w_gate: jax.Array,
    B_w_up: jax.Array,
    B_w_down: jax.Array,
    gate_w: jax.Array,
):
    _, S, M = A_x.shape
    C = A_c_kv.shape[2]
    H, D = A_w_q.shape[1], A_w_q.shape[2]
    FF = B_w_gate.shape[1]
    xT = A_x[0].T
    woT = jnp.transpose(A_w_o, (0, 2, 1))
    wdT = B_w_down.T
    any_spec = pl.BlockSpec(memory_space=pl.ANY)
    V = pltpu.VMEM
    outT = pl.pallas_call(
        _make_kernel(S, M, C, H, D, FF),
        in_specs=[any_spec] * 11,
        out_specs=any_spec,
        out_shape=jax.ShapeDtypeStruct((M, S), BF16),
        scratch_shapes=[
            V((H, S // _T, D, _T), BF16),
            V((H // 2, M, D), U32), V((H // 2, C, D), U32), V((H // 2, C, D), U32),
            V((S // _T, M, _T), BF16), V((2, M, _B), BF16),
            V((C // _T, S, _T), BF16), V((D // _T, H, M, _T), BF16),
            V((M, FF), BF16), V((M, FF), BF16), V((M, FF), BF16),
            [V((pl.cdiv(M, _T), 2 * D, _T), BF16)] * 2, [V((1, C, _T), BF16)] * 2,
            V((C // _T, D, _T), BF16),
            V((D // _T, S, _T), BF16), V((S // _T, D, _T), BF16), V((2, M, _T), F32),
            [V((1, _B, _B), F32)] * _NS,
            V((S // _T // _NG, _NG - 1, _T, _T), F32), V((_NG - 1, 2 * _G, _T), F32),
            V((S // _T, _NG - 1, _G, _T), F32), V((D // _T, _T, _T), BF16),
            V((2, M, _T), F32),
            V((1, S), F32), V((1, S), F32), V((M,), BF16), V((M,), BF16),
            pltpu.SMEM((3,), I32),
            pltpu.SemaphoreType.DMA((7,)), pltpu.SemaphoreType.DMA((H // 2,)),
            pltpu.SemaphoreType.DMA((2,)), pltpu.SemaphoreType.DMA((2,)),
        ],
        compiler_params=pltpu.CompilerParams(vmem_limit_bytes=100 << 20),
    )(xT, A_c_kv[0], A_w_q, A_w_uk, A_w_uv, woT, B_w_r, gate_w, B_w_gate, B_w_up, wdT)
    return outT.T[None]
```

```python
import math

import jax
import jax.numpy as jnp
from jax import lax
import jax.experimental.pallas as pl
import jax.experimental.pallas.tpu as pltpu

F32, BF16, U32, I32 = jnp.float32, jnp.bfloat16, jnp.uint32, jnp.int32
_NT = (((1,), (1,)), ((), ()))
_NEG = -1e30
_HI = 0xFFFF0000
_T = 128
_B = 256
_LAG = 5
_NS = 7
_NG = 4
_G = _T // _NG
_XA, _XB = 2, 7


def _mm(a, b):
    return jnp.dot(a, b, preferred_element_type=F32)


def _mm_nt(a, b):
    return lax.dot_general(a, b, _NT, preferred_element_type=F32)


def _sigmoid(x):
    return 1.0 / (1.0 + jnp.exp(-x))


def _as_f32(u):
    return lax.bitcast_convert_type(u, F32)


def _cat(parts, axis=1):
    return parts[0] if len(parts) == 1 else jnp.concatenate(parts, axis=axis)


def _colmax(x):
    return jnp.max(x, axis=0, keepdims=True)


def _ld(ref, *lead, rows=None):
    u = ref.bitcast(U32)
    idx = lead if rows is None else lead + (slice(rows[0] // 2, (rows[0] + rows[1]) // 2),)
    return pltpu.bitcast(u[idx], BF16)


def _make_kernel(S, M, C, H, D, FF):
    NB, NP = S // _B, H // 2
    NS_T, NC_T, ND_T, NF_T = S // _T, C // _T, D // _T, FF // _T
    MF, MR = M // _T, M % _T
    assert ND_T == 2 and MR > 0 and _NS > _LAG >= 1 and _NG == 4 and NB % 2 == 0
    q_scale = math.log2(math.e) * (D ** -0.5)

    def kernel(xT_hbm, c_hbm, wq_hbm, wk_hbm, wv_hbm, woT_hbm, wr_hbm, gw_hbm,
               wg_hbm, wu_hbm, wdT_hbm, o_hbm,
               qc_s, wq_buf, wk_buf, wv_buf, xT_s, o_s, c_s, woT_s, wg_s, wu_s, wdT_s,
               wqT_s, wk_s, wvT_s, k_s, vT_s, y_s, s_s, z_s, zt_s, side_s, qn_s, wc_s,
               g_s, r_s, wr_s, gw_s, idx_s,
               sem, q_sem, kv_sem, o_sem):
        def tiled(src, dst, n):
            return [(src.at[..., t * _T:(t + 1) * _T], dst.at[t]) for t in range(n)]

        xt = tiled(xT_hbm, xT_s, NS_T)
        groups = dict(w=[(wr_hbm, wr_s), (gw_hbm, gw_s)], xa=xt[:_XA], xb=xt[_XA:_XB], xc=xt[_XB:],
                      ffn=[(wg_hbm, wg_s), (wu_hbm, wu_s), (wdT_hbm, wdT_s)],
                      c=tiled(c_hbm, c_s, NC_T), wo=tiled(woT_hbm, woT_s, ND_T))

        def group(name):
            s = sem.at[list(groups).index(name)]
            return [pltpu.make_async_copy(src, dst, s) for src, dst in groups[name]]

        def q_cp(p):
            return [pltpu.make_async_copy(wq_hbm.bitcast(U32).at[:, p, :], wq_buf.at[p], q_sem.at[p])]

        def kv_cp(p):
            return [pltpu.make_async_copy(src.bitcast(U32).at[:, p, :], dst.at[p], kv_sem.at[jnp.minimum(p, 1)])
                    for src, dst in ((wk_hbm, wk_buf), (wv_hbm, wv_buf))]

        def o_cp(j):
            c0 = pl.multiple_of(j * _B, _B)
            return [pltpu.make_async_copy(o_s.at[j & 1], o_hbm.at[:, pl.ds(c0, _B)], o_sem.at[j & 1])]

        def start(cps):
            for d in cps:
                d.start()

        def wait(cps):
            for d in cps:
                d.wait()

        def prep_q(p, b):
            w = wq_buf[p].T
            for half, u in enumerate((w << 16, w & jnp.uint32(_HI))):
                wb = _as_f32(u)
                for t in range(MF):
                    wqT_s[b][t, half * D:(half + 1) * D, :] = wb[:, t * _T:(t + 1) * _T].astype(BF16)
                wqT_s[b][MF, half * D:(half + 1) * D, 0:MR] = wb[:, MF * _T:].astype(BF16)

        def q_tile(p, t, b):
            wqT = _cat([_ld(wqT_s[b], u) for u in range(MF)] + [_ld(wqT_s[b], MF)[:, 0:MR]])
            q = _mm(wqT, _ld(xT_s, t)) * q_scale
            qc_s[2 * p, t] = q[:D].astype(BF16)
            qc_s[2 * p + 1, t] = q[D:].astype(BF16)

        def q_first(t0, t1):
            for t in range(t0, t1):
                q_tile(0, t, 0)
                xf = xT_s[t].astype(F32)
                r0, r1 = [jnp.sum(xf * wc_s[n], axis=0, keepdims=True) for n in range(2)]
                r_s[:, t * _T:(t + 1) * _T] = r0.astype(BF16).astype(F32)
                g_s[:, t * _T:(t + 1) * _T] = _sigmoid(r1)

        def prep_wk0(hh):
            sh = jnp.asarray((1 - (hh & 1)) * 16).astype(U32)
            wk_s[0][0] = _as_f32((wk_buf[hh >> 1, :, 0:_T] << sh) & jnp.uint32(_HI)).astype(BF16)

        def run_pre():
            start(group('w') + q_cp(0) + group('xa') + group('xb') + group('xc'))
            pl.loop(1, NP)(lambda p: start(q_cp(p)))
            start(group('ffn') + group('c'))
            pl.loop(0, NP)(lambda p: start(kv_cp(p)))
            start(group('wo'))
            for b in range(2):
                wqT_s[b][MF] = jnp.zeros((2 * D, _T), BF16)
            idx_s[2] = 0
            wait(group('w'))
            for n, ref in enumerate((wr_s, gw_s)):
                wc_s[n] = jnp.broadcast_to(ref[...].astype(F32).reshape(1, M), (_T, M)).T
            wait(q_cp(0))
            prep_q(0, 0)
            wait(group('xa'))
            q_first(0, _XA)
            wait(group('xb'))
            q_first(_XA, _XB)
            wait(group('xc') + q_cp(1))
            prep_q(1, 1)
            q_first(_XB, NS_T)
            wait(q_cp(2) + q_cp(3))

            def phase_q(i, carry):
                p = 2 * i + 1
                prep_q(p + 1, 0)
                for t in range(NS_T):
                    q_tile(p, t, 1)
                prep_q(p + 2, 1)
                for t in range(NS_T):
                    q_tile(p + 1, t, 0)
                pl.when(p + 4 < NP)(lambda: wait(q_cp(p + 3) + q_cp(p + 4)))
                return carry

            lax.fori_loop(0, (NP - 2) // 2, phase_q, 0)
            wait(group('ffn') + kv_cp(0))

            lane = lax.broadcasted_iota(I32, (1, S), 1)
            idxs, cur = [], r_s[...]
            for n in range(2):
                mx = jnp.max(cur, axis=1, keepdims=True)
                ii = jnp.min(jnp.where(cur == mx, lane, S - 1))
                idxs.append(ii)
                idx_s[n] = ii
                cur = jnp.where(lane == ii, -jnp.inf, cur)
            ffn = {}

            def ffn_select(n):
                row16 = lax.broadcasted_iota(I32, (16, _T), 0)
                lane16 = lax.broadcasted_iota(I32, (16, _T), 1)
                oh = jnp.logical_and(row16 == n, lane16 == (idxs[n] & (_T - 1)))
                xr = _mm_nt(jnp.where(oh, 1.0, 0.0).astype(BF16), _ld(xT_s, jnp.clip(idxs[n] // _T, 0, NS_T - 1)))
                ffn['x'] = xr if n == 0 else (ffn['x'] + xr).astype(BF16)

            def ffn_gate(f):
                ffn['g', f] = _mm(ffn['x'], wg_s[:, f * _T:(f + 1) * _T])

            def ffn_up(f):
                gt = ffn['g', f]
                ffn[f] = (gt * _sigmoid(gt) * _mm(ffn['x'], wu_s[:, f * _T:(f + 1) * _T])).astype(BF16)

            def ffn_down(f):
                y = _mm_nt(ffn[f], wdT_s[:, f * _T:(f + 1) * _T])
                ffn['y'] = y if 'y' not in ffn else ffn['y'] + y

            plain = [(fn, f) for f in range(NF_T) for fn in (ffn_gate, ffn_up)]
            after = {5: [(ffn_select, 0)], 6: [(ffn_select, 1)]}
            gap, nd, ready = 7, 0, {}
            while plain or nd < NF_T:
                slot = []
                if nd < NF_T and ready.get(nd, gap) < gap:
                    slot.append((ffn_down, nd))
                    nd += 1
                while len(slot) < 2 and plain:
                    fn, f = plain.pop(0)
                    slot.append((fn, f))
                    if fn is ffn_up:
                        ready[f] = gap
                after[gap] = slot
                gap += 1
            assert gap <= 2 * NS_T - 1, gap
            for t in range(NS_T):
                if 2 * t in after:
                    for half in range(2):
                        w = _cat([_ld(wqT_s[1], u, rows=(half * D, D)) for u in range(MF)]
                                 + [_ld(wqT_s[1], MF, rows=(half * D, D))[:, 0:MR]])
                        qc_s[2 * (NP - 1) + half, t] = (_mm(w, _ld(xT_s, t)) * q_scale).astype(BF16)
                        for fn, f in after.get(2 * t + half, []):
                            fn(f)
                else:
                    q_tile(NP - 1, t, 1)
                    for fn, f in after.get(2 * t + 1, []):
                        fn(f)
            yp = jnp.concatenate([ffn['y'], jnp.zeros((16, (MF + 1) * _T - M), F32)], axis=1)
            yT = jnp.concatenate([yp, jnp.zeros((_T - 16, (MF + 1) * _T), F32)], axis=0).T[:M]
            for n in range(2):
                y_s[n] = jnp.broadcast_to(yT[:, n:n + 1], (M, _T))

            prep_wk0(0)

            rows = pl.ds(pl.multiple_of(jnp.clip(idx_s[2], 0, 1) * 8, 8), 8)
            z_s[...] = jnp.zeros(z_s.shape, F32)
            for ref in list(s_s) + [z_s.at[0], side_s.at[0], zt_s]:
                ref[0, rows, :] = jnp.zeros((8, ref.shape[-1]), F32)
            wait(group('c'))
            pl.loop(1, NP)(lambda p: wait(kv_cp(p)))

        def head(h, carry):
            slot = h >> 1
            sh = ((1 - (h & 1)) * 16).astype(U32)
            wk = _as_f32((wk_buf[slot, :, _T:] << sh) & jnp.uint32(_HI))
            wk_s[1][0] = wk.astype(BF16)
            wvT = _as_f32((wv_buf[slot] << sh) & jnp.uint32(_HI)).T.astype(BF16)
            for t in range(NC_T):
                wvT_s[t] = wvT[:, t * _T:(t + 1) * _T]
            tri = (lax.broadcasted_iota(I32, (_T, _T), 0) <= lax.broadcasted_iota(I32, (_T, _T), 1))
            G, NG, q_u = _G, _NG, qc_s.bitcast(U32)
            lane_t = lax.broadcasted_iota(I32, (_T, _T), 1)
            row_g = lax.broadcasted_iota(I32, (G, _T), 0)
            lane_g = lax.broadcasted_iota(I32, (G, _T), 1)
            qn = _ld(qc_s, h, NS_T - 1).astype(F32).T
            for t in range(ND_T):
                qn_s[t] = qn[:, t * _T:(t + 1) * _T].astype(BF16)

            def c_rows(r0, n):
                return _cat([_ld(c_s, t, rows=(r0, n)) for t in range(NC_T)])

            def k_rows(r0, n):
                return _cat([_ld(k_s, t, rows=(r0, n)) for t in range(ND_T)])

            def proj_k(j, t):
                w = wk if (j, t) == (0, 1) else _ld(wk_s[t], 0)
                k_s[t, j * _B:(j + 1) * _B, :] = _mm(c_rows(j * _B, _B), w).astype(BF16)

            def proj_v(j, t):
                w = wvT if (j, t) == (0, 0) else _cat([_ld(wvT_s, u) for u in range(NC_T)])
                vT_s[2 * j + t] = _mm_nt(w, c_rows(j * _B + t * _T, _T)).astype(BF16)

            done = set()

            def piece(fn, j, t):
                if j < NB and (fn, j, t) not in done:
                    done.add((fn, j, t))
                    fn(j, t)

            items = [(j, c) for j in range(NB) for c in range(j + 1)]
            state, cmax = {}, {}

            def qk(i):
                j, c = items[i]
                for t in range(2):
                    piece(proj_k, c, t)
                k0, st = c * _B, s_s[i % _NS]
                q0u, q1u = q_u[h, 2 * j], q_u[h, 2 * j + 1]
                q0, q1 = pltpu.bitcast(q0u, BF16), pltpu.bitcast(q1u, BF16)
                q = _cat([q0, q1])

                def diag(r0, qu, g):
                    w = jnp.where(lane_t < g * G, q_u[h, NS_T - 1], qu) if g else qu
                    return _mm(k_rows(k0 + r0 + g * G, G), pltpu.bitcast(w, BF16))

                def z_parts():
                    u = c // 2
                    assert (proj_k, 2 * u + 1, 1) in done
                    for g in (1,) if c % 2 == 0 else (2, 3):
                        kg = _cat([k_rows((NG * u + p) * _T + g * G, G) for p in range(NG)], axis=0)
                        qg = _cat([_ld(qn_s, t, rows=(g * G, _T - g * G)) for t in range(ND_T)])
                        z_s[u, g - 1, g * G:, :] = _mm_nt(qg, kg)

                if c < j < NB - 1:
                    s = _mm(k_rows(k0, _B), q)
                    st[0] = s
                    cmax[i] = _colmax(s)
                elif c < j:
                    n1 = (_B + 5 * G) // 2
                    sa = _mm(k_rows(k0, n1), q0)
                    z_parts()
                    sb = _mm(k_rows(k0 + n1, _B - n1), q0)
                    su = _mm(_cat([k_rows(k0, G), k_rows(k0 + _T, G)], axis=0), q1)
                    s0 = _cat([sa, sb], axis=0)
                    st[0, :, 0:_T] = s0
                    st[0, 0:G, _T:] = su[:G]
                    st[0, _T:_T + G, _T:] = su[G:]
                    cmax[i] = _cat([_colmax(s0), _colmax(su)])
                elif j < NB - 1:
                    sab = _mm(k_rows(k0, _T), q1)
                    sa = [diag(0, q0u, g) for g in range(NG)]
                    sb = [diag(_T, q1u, g) for g in range(NG)]
                    for g in range(1, NG):
                        side_s[2 * j, g - 1] = sa[g]
                        side_s[2 * j + 1, g - 1] = sb[g]
                    s = _cat([jnp.where(tri, _cat(sa, axis=0), _NEG), sab])
                    s2 = jnp.where(tri, _cat(sb, axis=0), _NEG)
                    st[0, 0:_T, :] = s
                    st[0, _T:, _T:] = s2
                    m = _colmax(s)
                    cmax[i] = _cat([m[:, :_T], jnp.maximum(m[:, _T:], _colmax(s2))])
                else:
                    z_parts()
                    sa = [diag(0, q0u, 1)]
                    s_a0 = _mm(k_rows(k0, G), q)
                    sa += [diag(0, q0u, g) for g in range(2, NG)]
                    s_b0 = _cat([_mm(k_rows(k0 + _T + r, G // 2), q1) for r in (0, G // 2)], axis=0)
                    for g in range(1, NG):
                        side_s[2 * j, g - 1] = sa[g - 1]
                    s0 = jnp.where(tri, _cat([s_a0[:, :_T]] + sa, axis=0), _NEG)
                    s_b0 = jnp.where(row_g <= lane_g, s_b0, _NEG)
                    st[0, 0:_T, 0:_T] = s0
                    st[0, 0:G, _T:] = s_a0[:, _T:]
                    st[0, _T:_T + G, _T:] = s_b0
                    cmax[i] = _cat([_colmax(s0), jnp.maximum(_colmax(s_a0[:, _T:]), _colmax(s_b0))])

            def pv(i):
                j, c = items[i]
                for t in range(2):
                    piece(proj_v, c, t)
                st, m = s_s[i % _NS], cmax.pop(i)
                if j == NB - 1:
                    fix = []
                    for g in range(1, NG):
                        if c % 2 == 0:
                            zt = z_s[c // 2, g - 1].T
                            zt_s[g - 1] = zt[2 * G:]
                        else:
                            zt = zt_s[g - 1]
                        for r in range(2):
                            zr = zt[r * G:(r + 1) * G]
                            if 2 * c + r < NS_T - 1:
                                x = jnp.where(lane_g < g * G, side_s[2 * c + r, g - 1], zr)
                            else:
                                x = jnp.where(row_g + g * G <= lane_g, zr, _NEG)
                            st[0, r * _T + g * G:r * _T + (g + 1) * G, _T:] = x
                            fix.append(x)
                    m = _cat([m[:, :_T], jnp.maximum(m[:, _T:], _colmax(_cat(fix, axis=0)))])
                if c > 0:
                    m0, l0, o0 = state[j]
                    m = jnp.maximum(m0, m)
                    alpha = jnp.exp2(m0 - m)
                if c < j:
                    p = jnp.exp2(st[0] - m)
                    l = jnp.sum(p, axis=0, keepdims=True)
                    o = _mm(_cat([_ld(vT_s, 2 * c), _ld(vT_s, 2 * c + 1)]), p.astype(BF16))
                else:
                    p = jnp.exp2(st[0, 0:_T, :] - m)
                    p2 = jnp.exp2(st[0, _T:, _T:] - m[:, _T:])
                    l = jnp.sum(p, axis=0, keepdims=True)
                    l = _cat([l[:, :_T], l[:, _T:] + jnp.sum(p2, axis=0, keepdims=True)])
                    p, p2 = p.astype(BF16), p2.astype(BF16)
                    o = _cat([_mm(_ld(vT_s, 2 * c, rows=(r, D // 2)), p)
                              for r in range(0, D, D // 2)], axis=0)
                    o2 = _cat([_mm(_ld(vT_s, 2 * c + 1, rows=(r, D // 4)), p2)
                               for r in range(0, D, D // 4)], axis=0)
                    o = _cat([o[:, :_T], o[:, _T:] + o2])
                l = jnp.where(o[0:1] != o[0:1], o[0:1], l)
                if c > 0:
                    l = l0 * alpha + l
                    o = o0 * alpha + o
                state[j] = (m, l, o)
                if c == j:
                    ctx = o * (1.0 / l)
                    for t in range(2):
                        qc_s[h, 2 * j + t] = ctx[:, t * _T:(t + 1) * _T].astype(BF16)

            for i in range(len(items) + _LAG):
                if i < len(items):
                    qk(i)
                    j, c = items[i]
                    fill = [(proj_v, j, 0), (proj_k, j + 1, 0), (proj_v, j, 1), (proj_k, j + 1, 1)]
                    if j < NB - 1:
                        for pc in fill[len(fill) * c // (j + 1):len(fill) * (c + 1) // (j + 1)]:
                            piece(*pc)
                elif i - len(items) in (0, 3):
                    piece(proj_v, NB - 1, (i - len(items)) // 3)
                if i >= _LAG:
                    pv(i - _LAG)
            prep_wk0(jnp.minimum(h + 1, H - 1))
            return carry

        def run_heads():
            lax.fori_loop(0, H, head, 0)
            wait(group('wo'))

        def phase_o(j, carry):
            pl.when(j >= 2)(lambda: wait(o_cp(j - 2)))
            c0 = pl.multiple_of(j * _B, _B)
            a = None
            for hh in range(0, H, 2):
                w2 = _cat([_ld(woT_s, t, hh + u) for u in range(2) for t in range(ND_T)])
                x2 = _cat([_cat([_ld(qc_s, hh + u, 2 * j), _ld(qc_s, hh + u, 2 * j + 1)])
                           for u in range(2)], axis=0)
                part = _mm(w2, x2)
                a = part if a is None else a + part
            g = g_s[:, pl.ds(c0, _B)]
            rs = _sigmoid(r_s[:, pl.ds(c0, _B)])
            col = lax.broadcasted_iota(I32, (1, _B), 1) + j * _B
            upd = jnp.where(col == idx_s[0], _cat([y_s[0], y_s[0]]),
                            jnp.where(col == idx_s[1], _cat([y_s[1], y_s[1]]), 0.0))
            b = _cat([xT_s[2 * j], xT_s[2 * j + 1]]).astype(F32) + upd * rs
            o_s[j & 1] = (g * a + (1.0 - g) * b).astype(BF16)
            start(o_cp(j))
            return carry

        def run_o():
            lax.fori_loop(0, NB, phase_o, 0)

        run_pre()

        def stage(k, carry):
            pl.when(k == 0)(run_heads)
            pl.when(k == 1)(run_o)
            return carry

        lax.fori_loop(0, 2, stage, 0)
        wait(o_cp(NB - 2) + o_cp(NB - 1))

    return kernel


@jax.jit
def pallas_gated_mix__compressed_kv_cla__moe_arch_mod__prompt_kernel(
    A_x: jax.Array,
    A_c_kv: jax.Array,
    A_w_q: jax.Array,
    A_w_uk: jax.Array,
    A_w_uv: jax.Array,
    A_w_o: jax.Array,
    B_x: jax.Array,
    B_w_r: jax.Array,
    B_w_gate: jax.Array,
    B_w_up: jax.Array,
    B_w_down: jax.Array,
    gate_w: jax.Array,
):
    _, S, M = A_x.shape
    C = A_c_kv.shape[2]
    H, D = A_w_q.shape[1], A_w_q.shape[2]
    FF = B_w_gate.shape[1]
    xT = A_x[0].T
    woT = jnp.transpose(A_w_o, (0, 2, 1))
    wdT = B_w_down.T
    any_spec = pl.BlockSpec(memory_space=pl.ANY)
    V = pltpu.VMEM
    outT = pl.pallas_call(
        _make_kernel(S, M, C, H, D, FF),
        in_specs=[any_spec] * 11,
        out_specs=any_spec,
        out_shape=jax.ShapeDtypeStruct((M, S), BF16),
        scratch_shapes=[
            V((H, S // _T, D, _T), BF16),
            V((H // 2, M, D), U32), V((H // 2, C, D), U32), V((H // 2, C, D), U32),
            V((S // _T, M, _T), BF16), V((2, M, _B), BF16),
            V((C // _T, S, _T), BF16), V((D // _T, H, M, _T), BF16),
            V((M, FF), BF16), V((M, FF), BF16), V((M, FF), BF16),
            [V((pl.cdiv(M, _T), 2 * D, _T), BF16)] * 2, [V((1, C, _T), BF16)] * 2,
            V((C // _T, D, _T), BF16),
            V((D // _T, S, _T), BF16), V((S // _T, D, _T), BF16), V((2, M, _T), F32),
            [V((1, _B, _B), F32)] * _NS,
            V((S // _T // _NG, _NG - 1, _T, _T), F32), V((_NG - 1, 2 * _G, _T), F32),
            V((S // _T, _NG - 1, _G, _T), F32), V((D // _T, _T, _T), BF16),
            V((2, M, _T), F32),
            V((1, S), F32), V((1, S), F32), V((M,), BF16), V((M,), BF16),
            pltpu.SMEM((3,), I32),
            pltpu.SemaphoreType.DMA((7,)), pltpu.SemaphoreType.DMA((H // 2,)),
            pltpu.SemaphoreType.DMA((2,)), pltpu.SemaphoreType.DMA((2,)),
        ],
        compiler_params=pltpu.CompilerParams(vmem_limit_bytes=100 << 20),
    )(xT, A_c_kv[0], A_w_q, A_w_uk, A_w_uv, woT, B_w_r, gate_w, B_w_gate, B_w_up, wdT)
    return outT.T[None]
```
